```python
import jax
import jax.numpy as jnp

def _softmax(x, axis=-1):
    return jax.nn.softmax(x, axis=axis)

def _gelu(x):
    return jax.nn.gelu(x, approximate=True)

def _silu(x):
    return jax.nn.silu(x)

def _sigmoid(x):
    return jax.nn.sigmoid(x)

def _layernorm(x, axis=-1, eps=1e-05):
    m = jnp.mean(x, axis=axis, keepdims=True)
    v = jnp.var(x, axis=axis, keepdims=True)
    return (x - m) / jnp.sqrt(v + eps)

def _scatter_add(tgt, idx, src, axis=0):
    return tgt.at[idx].add(src)

def _segment_sum(src, seg, n):
    return jax.ops.segment_sum(src, seg, n)

class _Rng:

    def __init__(self, key):
        self._k = key

    def _next(self):
        self._k, sub = jax.random.split(self._k)
        return sub

    def normal(self, shape):
        return jax.random.normal(self._next(), shape, dtype=jnp.bfloat16)

    def randint(self, lo, hi, shape):
        return jax.random.randint(self._next(), shape, lo, hi, dtype=jnp.int32)

    def uniform(self, shape, lo=0.0, hi=1.0):
        return jax.random.uniform(self._next(), shape, jnp.bfloat16, lo, hi)

    def permutation(self, n):
        return jax.random.permutation(self._next(), n)
kernel_name = 'interleave_layers__memory_aug_recurrent_mem_tr__glu_gated_geglu__prompt'

def setup_inputs():
    _rng = _Rng(jax.random.key(int.from_bytes(__import__("os").urandom(4), "little")))
    _w = lambda a: (lambda t: t.astype(jnp.bfloat16) if jnp.issubdtype(t.dtype, jnp.floating) else t)(jnp.asarray(a))

    def _A_setup():
        B, S, Dm = (1, 2048, 1024)
        H, Dh = (32, 128)
        M, seg = (8, 32)
        seg = min(seg, S)
        S = S // seg * seg
        return {'x': _w((lambda *s: _rng.normal(s) * 0.05)(B, S, Dm)), 'mem0': _w((lambda *s: _rng.normal(s) * 0.05)(B, M, Dm)), 'Wq': _w((lambda *s: _rng.normal(s) * 0.05)(Dm, H, Dh) * Dm ** (-0.5)), 'Wk': _w((lambda *s: _rng.normal(s) * 0.05)(Dm, H, Dh) * Dm ** (-0.5)), 'Wv': _w((lambda *s: _rng.normal(s) * 0.05)(Dm, H, Dh) * Dm ** (-0.5)), 'Wo': _w((lambda *s: _rng.normal(s) * 0.05)(H, Dh, Dm) * (H * Dh) ** (-0.5)), 'seg_len': seg}
    _A_in = _A_setup()

    def _B_setup():
        B, S, Dm, Df = (1, 2048, 1024, 3584)
        return {'x': _w((lambda *s: _rng.normal(s) * 0.05)(B, S, Dm)), 'w_gate': _w((lambda *s: _rng.normal(s) * 0.05)(Dm, Df) * Dm ** (-0.5)), 'w_up': _w((lambda *s: _rng.normal(s) * 0.05)(Dm, Df) * Dm ** (-0.5)), 'w_down': _w((lambda *s: _rng.normal(s) * 0.05)(Df, Dm) * Df ** (-0.5))}
    _B_in = _B_setup()
    return {'A_x': _A_in['x'], 'A_mem0': _A_in['mem0'], 'A_Wq': _A_in['Wq'], 'A_Wk': _A_in['Wk'], 'A_Wv': _A_in['Wv'], 'A_Wo': _A_in['Wo'], 'A_seg_len': _A_in['seg_len'], 'B_x': _B_in['x'], 'B_w_gate': _B_in['w_gate'], 'B_w_up': _B_in['w_up'], 'B_w_down': _B_in['w_down']}

def reference(A_x, A_mem0, A_Wq, A_Wk, A_Wv, A_Wo, A_seg_len, B_x, B_w_gate, B_w_up, B_w_down):

    def _A_ref(x, mem0, Wq, Wk, Wv, Wo, seg_len):
        B, S, Dm = x.shape
        H, Dh = (Wq.shape[1], Wq.shape[2])
        M = mem0.shape[1]
        scale = Dh ** (-0.5)
        n_seg = S // seg_len
        L = M + seg_len
        idx = jnp.arange(L)
        mask = (idx[:, None] < M) | (idx[:, None] >= idx[None, :])
        mem = mem0
        outs = []
        for s in range(n_seg):
            xs = x[:, s * seg_len:(s + 1) * seg_len, :].copy()
            h = jnp.concatenate([mem, xs], axis=1)
            q = jnp.einsum('btd,dhe->bhte', h, Wq)
            k = jnp.einsum('btd,dhe->bhte', h, Wk)
            v = jnp.einsum('btd,dhe->bhte', h, Wv)
            scores = jnp.einsum('bhqe,bhke->bhqk', q, k) * scale
            scores = jnp.where(mask[None, None], scores, -1000000000.0)
            p = _softmax(scores, axis=-1)
            o = jnp.einsum('bhqk,bhke->bhqe', p, v)
            o = jnp.einsum('bhte,hed->btd', o, Wo)
            mem = o[:, :M, :].copy()
            outs.append(o[:, M:, :])
        return jnp.concatenate(outs, axis=1)

    def _B_ref(x, w_gate, w_up, w_down):
        g = jnp.einsum('bsd,df->bsf', x, w_gate)
        u = jnp.einsum('bsd,df->bsf', x, w_up)
        h = _gelu(g) * u
        return jnp.einsum('bsf,fd->bsd', h, w_down)
    x = A_x
    x = x + _A_ref(_layernorm(x, axis=-1), A_mem0, A_Wq, A_Wk, A_Wv, A_Wo, A_seg_len)
    x = x + _B_ref(_layernorm(x, axis=-1), B_w_gate, B_w_up, B_w_down)
    x = x + _A_ref(_layernorm(x, axis=-1), A_mem0, A_Wq, A_Wk, A_Wv, A_Wo, A_seg_len)
    x = x + _B_ref(_layernorm(x, axis=-1), B_w_gate, B_w_up, B_w_down)
    return x
```

```python
import functools
import math

import jax
import jax.numpy as jnp
import numpy as np
from jax import lax
from jax.experimental import pallas as pl
from jax.experimental.pallas import tpu as pltpu

F32 = jnp.float32
BF16 = jnp.bfloat16

HG = 4
FC = 512
RB = 128


def _layernorm(x):
    m = jnp.mean(x, axis=-1, keepdims=True)
    c = x - m
    v = jnp.mean(c * c, axis=-1, keepdims=True)
    return c * lax.rsqrt(v + 1e-5)


def _gelu(x):
    c0 = math.sqrt(2.0 / math.pi)
    inner = x * (c0 + (c0 * 0.044715) * (x * x))
    return (0.5 * x) * (1.0 + jnp.tanh(inner))


def _dot(a, b):
    return jnp.dot(a, b, preferred_element_type=F32)


def _kernel(x_hbm, mem0_ref, wq_hbm, wk_hbm, wv_hbm, wo_hbm, wg_hbm, wu_hbm, wd_hbm,
            out_hbm,
            x_v, o_v, raw_v, wqkv_v, wo_v, wg_v, wu_v, wd_v,
            lhs_a, res_a, acc_o, lhs_f, res_f, acc_f, fill_v,
            raw_sem, w_sem, out_sem,
            *, S, D, H, Dh, M, SEG, DF):
    n_seg = S // SEG
    MM = 2 * M
    n_grp = H // HG
    n_fc = DF // FC
    GW = HG * Dh
    scale = Dh ** -0.5
    exp_c = scale * math.log2(math.e)

    n_rb = D // RB
    raw_srcs = (wq_hbm, wk_hbm, wv_hbm)

    def raw_copy(m, r):
        return pltpu.make_async_copy(
            raw_srcs[m].at[pl.ds(r * RB * H, RB * H)],
            raw_v.at[pl.ds((m * D + r * RB) * H, RB * H)],
            raw_sem.at[m * n_rb + r])

    plain = [pltpu.make_async_copy(s, d, w_sem.at[i]) for i, (s, d) in enumerate(
        ((x_hbm, x_v), (wo_hbm, wo_v), (wg_hbm, wg_v), (wu_hbm, wu_v), (wd_hbm, wd_v)))]
    plain[0].start()
    for m in range(3):
        for r in range(n_rb):
            raw_copy(m, r).start()
    for c in plain[1:]:
        c.start()

    R = MM + 2 * SEG
    row = lax.broadcasted_iota(jnp.int32, (R, 128), 0)
    col = lax.broadcasted_iota(jnp.int32, (R, 128), 1)

    def layer_of(i):
        return jnp.where(i < M, 0, jnp.where(i < MM, 1, jnp.where(i < MM + SEG, 0, jnp.where(i < R, 1, 2))))

    same = layer_of(row) == layer_of(col)
    keep = (row < MM) | (row >= col)
    fill_v[...] = jnp.where(same, jnp.where(keep, 0.0, -1e9 / scale), -jnp.inf).astype(F32)

    raw32 = raw_v.bitcast(jnp.int32)
    HP = H // 2
    for m in range(3):
        for r in range(n_rb):
            raw_copy(m, r).wait()
            base = (m * D + r * RB) * HP
            for j in range(HP):
                ev = raw32[pl.ds(base + j, RB // 2, stride=2 * HP), :]
                od = raw32[pl.ds(base + HP + j, RB // 2, stride=2 * HP), :]
                lo = (ev & 0xFFFF) | (od << 16)
                hi = lax.shift_right_logical(ev, 16) | (od & -65536)
                g, i = divmod(2 * j, HG)
                c0 = m * GW + i * Dh
                wqkv_v[g, pl.ds(r * RB, RB), pl.ds(c0, Dh)] = pltpu.bitcast(lo, BF16)
                wqkv_v[g, pl.ds(r * RB, RB), pl.ds(c0 + Dh, Dh)] = pltpu.bitcast(hi, BF16)

    plain[0].wait()
    mem0 = mem0_ref[...].astype(F32)
    zeros = jnp.zeros((SEG, D), F32)
    x_first = x_v[pl.ds(0, SEG), :].astype(F32)
    lhs_a[pl.ds(0, MM), :] = jnp.concatenate([mem0, mem0], axis=0).astype(BF16)
    lhs_a[pl.ds(MM, SEG), :] = _layernorm(x_first).astype(BF16)
    lhs_a[pl.ds(MM + SEG, SEG), :] = zeros.astype(BF16)
    res_a[pl.ds(0, SEG), :] = x_first
    res_a[pl.ds(SEG, SEG), :] = zeros
    lhs_f[...] = jnp.zeros(lhs_f.shape, BF16)
    res_f[...] = jnp.zeros(res_f.shape, F32)
    for c in plain[1:]:
        c.wait()

    def qkv(g):
        return _dot(lhs_a[...], wqkv_v[g]).astype(BF16)

    def scores(p):
        out = []
        for i in range(HG):
            q = p[:, i * Dh:(i + 1) * Dh]
            k = p[:, GW + i * Dh:GW + (i + 1) * Dh]
            k = jnp.concatenate([k, jnp.zeros((128 - R, Dh), BF16)], axis=0)
            out.append(lax.dot_general(q, k, (((1,), (1,)), ((), ())),
                                       preferred_element_type=F32))
        return out

    def attend(p, ss):
        out = []
        for i in range(HG):
            fill = fill_v[...]
            s = jnp.where(fill == 0.0, ss[i], fill)
            e = jnp.exp2((s - jnp.max(s, axis=-1, keepdims=True)) * exp_c)
            inv = 1.0 / jnp.sum(e, axis=-1, keepdims=True)
            v = p[:, 2 * GW + i * Dh:2 * GW + (i + 1) * Dh]
            v = jnp.concatenate([v, jnp.zeros((128 - R, Dh), BF16)], axis=0)
            out.append((_dot(e.astype(BF16), v) * inv).astype(BF16))
        return jnp.concatenate(out, axis=1)

    def project(g, o):
        y = _dot(o, wo_v[pl.ds(g * GW, GW), :])
        if g == 0:
            acc_o[...] = y
        else:
            acc_o[...] += y

    def ffn_up(c):
        h = lhs_f[...]
        gate = _dot(h, wg_v[:, pl.ds(c * FC, FC)])
        up = _dot(h, wu_v[:, pl.ds(c * FC, FC)])
        return (_gelu(gate) * up).astype(BF16)

    def ffn_down(c, a):
        y = _dot(a, wd_v[pl.ds(c * FC, FC), :])
        if c == 0:
            acc_f[...] = res_f[...] + y
        else:
            acc_f[...] += y

    def out_copy(s):
        rows = pl.ds(pl.multiple_of(s * SEG, SEG), SEG)
        return pltpu.make_async_copy(o_v.at[rows], out_hbm.at[rows], out_sem)

    def step(t, carry):
        p, ss, o, a = {}, {}, {}, {}
        p[0] = qkv(0)
        for g in range(n_grp):
            ss[g] = scores(p[g])
            if g + 1 < n_grp:
                p[g + 1] = qkv(g + 1)
            if g < n_fc:
                a[g] = ffn_up(g)
            if 1 <= g <= n_fc:
                ffn_down(g - 1, a[g - 1])
            o[g] = attend(p[g], ss[g])
            if g >= 1:
                project(g - 1, o[g - 1])
        x2 = acc_f[pl.ds(0, SEG), :]
        s_out = jnp.maximum(t - 3, 0)
        o_v[pl.ds(pl.multiple_of(s_out * SEG, SEG), SEG), :] = acc_f[pl.ds(SEG, SEG), :].astype(BF16)
        s_in = jnp.minimum(t + 1, n_seg - 1)
        x0 = x_v[pl.ds(pl.multiple_of(s_in * SEG, SEG), SEG), :].astype(F32)
        lhs_a[pl.ds(MM, SEG), :] = _layernorm(x0).astype(BF16)
        lhs_a[pl.ds(MM + SEG, SEG), :] = _layernorm(x2).astype(BF16)
        project(n_grp - 1, o[n_grp - 1])
        mem = acc_o[pl.ds(0, MM), :]
        is2 = lax.broadcasted_iota(jnp.int32, (MM, D), 0) >= M
        restart = jnp.where(t < 2, 1, 0)
        mem = jnp.where(jnp.where(is2, restart, 0) == 1,
                        jnp.concatenate([mem0, mem0], axis=0), mem)
        lhs_a[pl.ds(0, MM), :] = mem.astype(BF16)
        xa = res_a[...] + acc_o[pl.ds(MM, 2 * SEG), :]
        res_f[...] = xa
        lhs_f[...] = _layernorm(xa).astype(BF16)
        res_a[pl.ds(0, SEG), :] = x0
        res_a[pl.ds(SEG, SEG), :] = x2

        @pl.when(t >= 3)
        def _():
            out_copy(t - 3).start()

        return carry

    lax.fori_loop(0, n_seg + 3, step, 0)
    pltpu.make_async_copy(o_v, out_hbm, out_sem).wait()


@functools.partial(jax.jit, static_argnames=("A_seg_len",))
def pallas_interleave_layers__memory_aug_recurrent_mem_tr__glu_gated_geglu__prompt_kernel(
    A_x, A_mem0, A_Wq, A_Wk, A_Wv, A_Wo, A_seg_len, B_x, B_w_gate, B_w_up, B_w_down,
):
    del B_x
    B, S, D = A_x.shape
    _, H, Dh = A_Wq.shape
    M = A_mem0.shape[1]
    SEG = int(A_seg_len)
    DF = B_w_gate.shape[1]
    assert B == 1 and S % SEG == 0 and Dh == 128 and 2 * (M + SEG) <= 128
    R = 2 * (M + SEG)
    hbm = pl.BlockSpec(memory_space=pl.ANY)
    out = pl.pallas_call(
        functools.partial(_kernel, S=S, D=D, H=H, Dh=Dh, M=M, SEG=SEG, DF=DF),
        out_shape=jax.ShapeDtypeStruct((S, D), A_x.dtype),
        in_specs=[hbm, pl.BlockSpec(memory_space=pltpu.VMEM)] + [hbm] * 7,
        out_specs=hbm,
        scratch_shapes=[
            pltpu.VMEM((S, D), BF16),
            pltpu.VMEM((S, D), BF16),
            pltpu.VMEM((3 * D * H, Dh), BF16),
            pltpu.VMEM((H // HG, D, 3 * HG * Dh), BF16),
            pltpu.VMEM((H * Dh, D), BF16),
            pltpu.VMEM((D, DF), BF16),
            pltpu.VMEM((D, DF), BF16),
            pltpu.VMEM((DF, D), BF16),
            pltpu.VMEM((R, D), BF16),
            pltpu.VMEM((2 * SEG, D), F32),
            pltpu.VMEM((R, D), F32),
            pltpu.VMEM((2 * SEG, D), BF16),
            pltpu.VMEM((2 * SEG, D), F32),
            pltpu.VMEM((2 * SEG, D), F32),
            pltpu.VMEM((R, 128), F32),
            pltpu.SemaphoreType.DMA((3 * (D // RB),)),
            pltpu.SemaphoreType.DMA((5,)),
            pltpu.SemaphoreType.DMA(()),
        ],
        compiler_params=pltpu.CompilerParams(vmem_limit_bytes=120 * 2**20),
    )(A_x.reshape(S, D), A_mem0.reshape(M, D),
      A_Wq.reshape(D * H, Dh), A_Wk.reshape(D * H, Dh), A_Wv.reshape(D * H, Dh),
      A_Wo.reshape(H * Dh, D), B_w_gate, B_w_up, B_w_down)
    return out.reshape(B, S, D)
```

```python
import functools
import math

import jax
import jax.numpy as jnp
import numpy as np
from jax import lax
from jax.experimental import pallas as pl
from jax.experimental.pallas import tpu as pltpu

F32 = jnp.float32
BF16 = jnp.bfloat16

HG = 4
FC = 512
LAG = 4
WINDOW = 3
RING = 8
RB = 128


def _layernorm(x):
    m = jnp.mean(x, axis=-1, keepdims=True)
    c = x - m
    v = jnp.mean(c * c, axis=-1, keepdims=True)
    return c * lax.rsqrt(v + 1e-5)


def _gelu(x):
    c0 = math.sqrt(2.0 / math.pi)
    inner = x * (c0 + (c0 * 0.044715) * (x * x))
    return (0.5 * x) * (1.0 + jnp.tanh(inner))


def _dot(a, b):
    return jnp.dot(a, b, preferred_element_type=F32)


def _kernel(x_hbm, mem0_ref, wq_hbm, wk_hbm, wv_hbm, wo_hbm, wg_hbm, wu_hbm, wd_hbm,
            out_hbm,
            x_v, o_v, raw_v, wqkv_v, wo_v, wg_v, wu_v, wd_v,
            res_v, lhs_a, acc_o, lhs_f, acc_f, fill_v, fill_s,
            raw_sem, w_sem, out_sem,
            *, S, D, H, Dh, M, SEG, DF):
    n_seg = S // SEG
    MM = 2 * M
    R2 = MM + 2 * SEG
    R1 = MM + SEG
    n_grp = H // HG
    n_fc = DF // FC
    GW = HG * Dh
    scale = Dh ** -0.5
    exp_c = scale * math.log2(math.e)

    n_rb = D // RB
    queued = ((wq_hbm, raw_v, 0), (wk_hbm, raw_v, 1), (wv_hbm, raw_v, 2), (wo_hbm, wo_v, 0))

    def queued_copy(m, r):
        src, dst, first = queued[m]
        n = src.shape[0] // n_rb
        return pltpu.make_async_copy(
            src.at[pl.ds(pl.multiple_of(r * n, n), n)],
            dst.at[pl.ds(pl.multiple_of((first * n_rb + r) * n, n), n)],
            raw_sem.at[m * n_rb + r])

    head_rows = (LAG + 1) * SEG
    x_head, wg_copy, wu_copy, wd_copy, x_rest = [
        pltpu.make_async_copy(s, d, w_sem.at[i]) for i, (s, d) in enumerate((
            (x_hbm.at[pl.ds(0, head_rows)], x_v.at[pl.ds(0, head_rows)]),
            (wg_hbm, wg_v), (wu_hbm, wu_v), (wd_hbm, wd_v),
            (x_hbm.at[pl.ds(head_rows, S - head_rows)],
             x_v.at[pl.ds(head_rows, S - head_rows)])))]
    x_head.start()
    for r in range(WINDOW):
        queued_copy(0, r).start()

    def wait_queued(m, r):
        queued_copy(m, r).wait()

        @pl.when(r + WINDOW < n_rb)
        def _():
            queued_copy(m, r + WINDOW).start()

        if m + 1 < len(queued):
            @pl.when(r + WINDOW >= n_rb)
            def _():
                queued_copy(m + 1, r + WINDOW - n_rb).start()

    def make_fill(rows, layer_of):
        row = lax.broadcasted_iota(jnp.int32, (rows, 128), 0)
        col = lax.broadcasted_iota(jnp.int32, (rows, 128), 1)
        same = layer_of(row) == layer_of(col)
        keep = (row < MM) | (row >= col)
        return jnp.where(same, jnp.where(keep, 0.0, -1e9 / scale), -jnp.inf).astype(F32)

    fill_v[...] = make_fill(R2, lambda i: jnp.where(
        i < M, 0, jnp.where(i < MM, 1, jnp.where(i < R1, 0, jnp.where(i < R2, 1, 2)))))
    for layer in range(2):
        fill_s[layer] = make_fill(R1, lambda i: jnp.where(
            i < M, 0, jnp.where(i < MM, 1, jnp.where(i < R1, layer, 2))))

    HP = H // 2

    def relayout(m, r, carry):
        wait_queued(m, r)
        base = pl.multiple_of((m * n_rb + r) * (RB * H), RB * H)
        raw32 = raw_v.at[pl.ds(base, RB * H)].bitcast(jnp.int32)
        rows = pl.ds(pl.multiple_of(r * RB, RB), RB)
        for j in range(HP):
            ev = raw32[pl.ds(j, RB // 2, stride=2 * HP), :]
            od = raw32[pl.ds(HP + j, RB // 2, stride=2 * HP), :]
            lo = (ev & 0xFFFF) | (od << 16)
            hi = lax.shift_right_logical(ev, 16) | (od & -65536)
            g, i = divmod(2 * j, HG)
            c0 = m * GW + i * Dh
            wqkv_v[g, rows, pl.ds(c0, Dh)] = pltpu.bitcast(lo, BF16)
            wqkv_v[g, rows, pl.ds(c0 + Dh, Dh)] = pltpu.bitcast(hi, BF16)
        return carry

    for m in range(3):
        lax.fori_loop(0, n_rb, functools.partial(relayout, m), 0)

    def seg_rows(s):
        return pl.ds(pl.multiple_of(s * SEG, SEG), SEG)

    def slot(s):
        return s & (RING - 1)

    def load_segment(s):
        x0 = x_v[seg_rows(s), :].astype(F32)
        res_v[slot(s)] = x0
        return x0

    x_head.wait()
    mem0 = mem0_ref[...].astype(F32)
    lhs_a[pl.ds(0, MM), :] = jnp.concatenate([mem0, mem0], axis=0).astype(BF16)
    for s in range(LAG + 1):
        load_segment(s)

    def wait_wo(r, carry):
        wait_queued(3, r)

        @pl.when(r == n_rb - 2)
        def _():
            wg_copy.start()

        return carry

    lax.fori_loop(0, n_rb, wait_wo, 0)
    wu_copy.start()
    wd_copy.start()

    def qkv(g, rows):
        return _dot(lhs_a[pl.ds(0, rows), :], wqkv_v[g]).astype(BF16)

    def padded(a):
        return jnp.concatenate([a, jnp.zeros((128 - a.shape[0], Dh), BF16)], axis=0)

    def scores(p):
        return [lax.dot_general(p[:, i * Dh:(i + 1) * Dh],
                                padded(p[:, GW + i * Dh:GW + (i + 1) * Dh]),
                                (((1,), (1,)), ((), ())), preferred_element_type=F32)
                for i in range(HG)]

    def attend(p, ss, fill_ref):
        out = []
        for i in range(HG):
            fill = fill_ref[...]
            s = jnp.where(fill == 0.0, ss[i], fill)
            e = jnp.exp2((s - jnp.max(s, axis=-1, keepdims=True)) * exp_c)
            inv = 1.0 / jnp.sum(e, axis=-1, keepdims=True)
            v = padded(p[:, 2 * GW + i * Dh:2 * GW + (i + 1) * Dh])
            out.append((_dot(e.astype(BF16), v) * inv).astype(BF16))
        return jnp.concatenate(out, axis=1)

    def project(g, o, segs):
        rows = o.shape[0]
        y = _dot(o, wo_v[pl.ds(g * GW, GW), :])
        if g == 0:
            acc_o[pl.ds(0, MM), :] = y[:MM]
            for n, s in enumerate(segs):
                lo = MM + n * SEG
                acc_o[pl.ds(lo, SEG), :] = res_v[slot(s)] + y[lo:lo + SEG]
        elif g < n_grp - 1:
            acc_o[pl.ds(0, rows), :] += y
        else:
            y = acc_o[pl.ds(0, rows), :] + y
            for n, s in enumerate(segs):
                lo = MM + n * SEG
                res_v[slot(s)] = y[lo:lo + SEG]
            return y[:MM]

    def ffn_input(segs):
        for n, s in enumerate(segs):
            x = res_v[slot(s)]
            acc_f[pl.ds(n * SEG, SEG), :] = x
            lhs_f[pl.ds(n * SEG, SEG), :] = _layernorm(x).astype(BF16)

    def ffn_up(c):
        h = lhs_f[...]
        gate = _dot(h, wg_v[:, pl.ds(c * FC, FC)])
        up = _dot(h, wu_v[:, pl.ds(c * FC, FC)])
        return (_gelu(gate) * up).astype(BF16)

    def ffn_down(c, a, segs):
        y = _dot(a, wd_v[pl.ds(c * FC, FC), :])
        if c < n_fc - 1:
            acc_f[...] += y
        else:
            y = acc_f[...] + y
            for n, s in enumerate(segs):
                r = y[n * SEG:(n + 1) * SEG]
                res_v[slot(s)] = r
                o_v[seg_rows(s), :] = r.astype(BF16)

    def out_copy(s):
        return pltpu.make_async_copy(o_v.at[seg_rows(s)], out_hbm.at[seg_rows(s)], out_sem)

    def attention_input(n, x):
        lhs_a[pl.ds(MM + n * SEG, SEG), :] = _layernorm(x).astype(BF16)

    def single_attention(layer, s):
        attention_input(0, res_v[slot(s)])
        p, ss, o = {}, {}, {}
        p[0] = qkv(0, R1)
        for g in range(n_grp):
            if g + 1 < n_grp:
                p[g + 1] = qkv(g + 1, R1)
            ss[g] = scores(p[g])
            if g >= 1:
                project(g - 1, o[g - 1], (s,))
            o[g] = attend(p[g], ss[g], fill_s.at[layer])
        mem = project(n_grp - 1, o[n_grp - 1], (s,))
        own = jnp.where(lax.broadcasted_iota(jnp.int32, (MM, D), 0) < M, 0, 1) == layer
        lhs_a[pl.ds(0, MM), :] = jnp.where(
            own, mem, lhs_a[pl.ds(0, MM), :].astype(F32)).astype(BF16)

    def single_ffn(segs):
        ffn_input(segs)
        a = {0: ffn_up(0)}
        for c in range(n_fc):
            if c + 1 < n_fc:
                a[c + 1] = ffn_up(c + 1)
            ffn_down(c, a[c], segs)

    def paired_step(t, carry):
        att = (t, t - LAG)
        ffn = (t - 1, jnp.where(t == LAG, t - 2, t - LAG - 1))
        p, ss, o, a = {}, {}, {}, {}
        p[0] = qkv(0, R2)
        ffn_input(ffn)
        for g in range(n_grp):
            if g + 1 < n_grp:
                p[g + 1] = qkv(g + 1, R2)
            ss[g] = scores(p[g])
            if g < n_fc:
                a[g] = ffn_up(g)
            if g + 1 == n_grp:
                attention_input(0, load_segment(jnp.minimum(t + 1, n_seg - 1)))
                attention_input(1, res_v[slot(t + 1 - LAG)])
            if g >= 1:
                project(g - 1, o[g - 1], att)
            o[g] = attend(p[g], ss[g], fill_v)
            if 1 <= g < n_fc:
                ffn_down(g - 1, a[g - 1], ffn)
        mem = project(n_grp - 1, o[n_grp - 1], att)
        lhs_a[pl.ds(0, MM), :] = mem.astype(BF16)
        ffn_down(n_fc - 1, a[n_fc - 1], ffn)

        @pl.when(t > LAG)
        def _():
            out_copy(t - LAG - 1).start()

        return carry

    def single_op(phase, i):
        is_head = phase == 0
        j = i - 1
        tail_ffn = lax.rem(i, 3) == 0
        is_ffn = jnp.where(is_head, i == LAG, tail_ffn)
        first = n_seg - LAG + 2 * lax.div(jnp.maximum(j, 0), 3)

        @pl.when(jnp.logical_not(is_ffn))
        def _():
            single_attention(phase, jnp.where(is_head, i, first + lax.rem(j, 3)))

        @pl.when(is_ffn)
        def _():
            @pl.when(is_head)
            def _():
                for c in (wg_copy, wu_copy, wd_copy):
                    c.wait()
                x_rest.start()

            s0 = jnp.where(is_head, 0, jnp.where(i == 0, n_seg - 1, first))
            s1 = jnp.where(is_head, 1, jnp.where(i == 0, n_seg - LAG - 1, first + 1))
            single_ffn((s0, s1))

            @pl.when(jnp.logical_not(is_head))
            def _():
                out_copy(s1).start()

                @pl.when(i > 0)
                def _():
                    out_copy(s0).start()

    def phase_body(phase, carry):
        n_ops = jnp.where(phase == 0, LAG + 1, 1 + 3 * (LAG // 2))
        lax.fori_loop(0, n_ops, lambda i, c: (single_op(phase, i), c)[1], 0)

        @pl.when(phase == 0)
        def _():
            x_rest.wait()
            attention_input(0, res_v[slot(LAG)])
            attention_input(1, res_v[slot(0)])
            lax.fori_loop(LAG, n_seg, paired_step, 0)

        return carry

    lax.fori_loop(0, 2, phase_body, 0)
    pltpu.make_async_copy(o_v, out_hbm, out_sem).wait()


@functools.partial(jax.jit, static_argnames=("A_seg_len",))
def pallas_interleave_layers__memory_aug_recurrent_mem_tr__glu_gated_geglu__prompt_kernel(
    A_x, A_mem0, A_Wq, A_Wk, A_Wv, A_Wo, A_seg_len, B_x, B_w_gate, B_w_up, B_w_down,
):
    del B_x
    B, S, D = A_x.shape
    _, H, Dh = A_Wq.shape
    M = A_mem0.shape[1]
    SEG = int(A_seg_len)
    DF = B_w_gate.shape[1]
    assert B == 1 and S % SEG == 0 and Dh == 128 and 2 * (M + SEG) <= 128
    R = 2 * (M + SEG)
    hbm = pl.BlockSpec(memory_space=pl.ANY)
    out = pl.pallas_call(
        functools.partial(_kernel, S=S, D=D, H=H, Dh=Dh, M=M, SEG=SEG, DF=DF),
        out_shape=jax.ShapeDtypeStruct((S, D), A_x.dtype),
        in_specs=[hbm, pl.BlockSpec(memory_space=pltpu.VMEM)] + [hbm] * 7,
        out_specs=hbm,
        scratch_shapes=[
            pltpu.VMEM((S, D), BF16),
            pltpu.VMEM((S, D), BF16),
            pltpu.VMEM((3 * D * H, Dh), BF16),
            pltpu.VMEM((H // HG, D, 3 * HG * Dh), BF16),
            pltpu.VMEM((H * Dh, D), BF16),
            pltpu.VMEM((D, DF), BF16),
            pltpu.VMEM((D, DF), BF16),
            pltpu.VMEM((DF, D), BF16),
            pltpu.VMEM((RING, SEG, D), F32),
            pltpu.VMEM((R, D), BF16),
            pltpu.VMEM((R, D), F32),
            pltpu.VMEM((2 * SEG, D), BF16),
            pltpu.VMEM((2 * SEG, D), F32),
            pltpu.VMEM((R, 128), F32),
            pltpu.VMEM((2, R - SEG, 128), F32),
            pltpu.SemaphoreType.DMA((4 * (D // RB),)),
            pltpu.SemaphoreType.DMA((5,)),
            pltpu.SemaphoreType.DMA(()),
        ],
        compiler_params=pltpu.CompilerParams(vmem_limit_bytes=120 * 2**20),
    )(A_x.reshape(S, D), A_mem0.reshape(M, D),
      A_Wq.reshape(D * H, Dh), A_Wk.reshape(D * H, Dh), A_Wv.reshape(D * H, Dh),
      A_Wo.reshape(H * Dh, D), B_w_gate, B_w_up, B_w_down)
    return out.reshape(B, S, D)
```

```python
import functools
import math

import jax
import jax.numpy as jnp
import numpy as np
from jax import lax
from jax.experimental import pallas as pl
from jax.experimental.pallas import tpu as pltpu

F32 = jnp.float32
BF16 = jnp.bfloat16

HG = 2
FC = 512
LAG = 4
WINDOW = 3
PRE = 7
PRE_PARTS = 4
ATT_PARTS = 2
FFN_PARTS = 2
RING = 8
RB = 128


def _step_order(n_grp, n_fc):
    at = [(c * (n_grp - 1)) // n_fc for c in range(n_fc)]
    order = [("q", 0), ("i", 0), ("q", 1), ("s", 0)]
    for g in range(n_grp):
        last = g == n_grp - 1
        if g + 2 < n_grp:
            order.append(("q", g + 2))
        if not last:
            order.append(("s", g + 1))
        if g + 2 == n_grp:
            order.append(("n", 0))
        order.append(("a", g))
        if g >= 1:
            order.append(("o", g - 1))
        order += [("u", c) for c in range(n_fc) if at[c] == g]
        order += [("d", c) for c in range(n_fc - 1) if at[c] + 1 == g]
    return order + [("o", n_grp - 1), ("d", n_fc - 1)]


def _layernorm(x):
    m = jnp.mean(x, axis=-1, keepdims=True)
    c = x - m
    v = jnp.mean(c * c, axis=-1, keepdims=True)
    return c * lax.rsqrt(v + 1e-5)


def _gelu(x):
    c0 = math.sqrt(2.0 / math.pi)
    inner = x * (c0 + (c0 * 0.044715) * (x * x))
    return (0.5 * x) * (1.0 + jnp.tanh(inner))


def _dot(a, b):
    return jnp.dot(a, b, preferred_element_type=F32)


def _kernel(x_hbm, mem0_ref, wq_hbm, wk_hbm, wv_hbm, wo_hbm, wg_hbm, wu_hbm, wd_hbm,
            out_hbm,
            x_v, o_v, raw_v, wqkv_v, wo_v, wg_v, wu_v, wd_v,
            res_v, lhs_a, acc_o, lhs_f, acc_f, fill_v, fill_s, pre_in, pre_v,
            raw_sem, w_sem, out_sem,
            *, S, D, H, Dh, M, SEG, DF):
    n_seg = S // SEG
    MM = 2 * M
    R2 = MM + 2 * SEG
    R1 = MM + SEG
    n_grp = H // HG
    n_fc = DF // FC
    GW = HG * Dh
    scale = Dh ** -0.5
    exp_c = scale * math.log2(math.e)

    n_rb = D // RB
    queued = ((wq_hbm, raw_v, 0), (wk_hbm, raw_v, 1), (wv_hbm, raw_v, 2), (wo_hbm, wo_v, 0))

    def queued_copy(m, r):
        src, dst, first = queued[m]
        n = src.shape[0] // n_rb
        return pltpu.make_async_copy(
            src.at[pl.ds(pl.multiple_of(r * n, n), n)],
            dst.at[pl.ds(pl.multiple_of((first * n_rb + r) * n, n), n)],
            raw_sem.at[m * n_rb + r])

    head_rows = (LAG + PRE) * SEG
    x_head, wg_copy, wu_copy, wd_copy, x_rest = [
        pltpu.make_async_copy(s, d, w_sem.at[i]) for i, (s, d) in enumerate((
            (x_hbm.at[pl.ds(0, head_rows)], x_v.at[pl.ds(0, head_rows)]),
            (wg_hbm, wg_v), (wu_hbm, wu_v), (wd_hbm, wd_v),
            (x_hbm.at[pl.ds(head_rows, S - head_rows)],
             x_v.at[pl.ds(head_rows, S - head_rows)])))]
    x_head.start()
    for r in range(WINDOW):
        queued_copy(0, r).start()

    def wait_queued(m, r):
        queued_copy(m, r).wait()

        @pl.when(r + WINDOW < n_rb)
        def _():
            queued_copy(m, r + WINDOW).start()

        if m + 1 < len(queued):
            @pl.when(r + WINDOW >= n_rb)
            def _():
                queued_copy(m + 1, r + WINDOW - n_rb).start()

    def make_fill(rows, mem_lo, layer_of):
        row = lax.broadcasted_iota(jnp.int32, (rows, 128), 0)
        col = lax.broadcasted_iota(jnp.int32, (rows, 128), 1)

        def is_mem(i):
            return (i >= mem_lo) & (i < mem_lo + MM)

        keep = is_mem(row) | is_mem(col) | (row >= col)
        return jnp.where(layer_of(row) == layer_of(col),
                         jnp.where(keep, 0.0, -1e9 / scale), -jnp.inf).astype(F32)

    fill_v[...] = make_fill(
        R2, SEG, lambda i: jnp.where(i < SEG + M, 0, jnp.where(i < R2, 1, 2)))
    for layer in range(2):
        fill_s[layer] = make_fill(R1, 0, lambda i: jnp.where(
            i < M, 0, jnp.where(i < MM, 1, jnp.where(i < R1, layer, 2))))

    HP = H // 2

    def relayout(m, r):
        base = pl.multiple_of((m * n_rb + r) * (RB * H), RB * H)
        raw32 = raw_v.at[pl.ds(base, RB * H)].bitcast(jnp.int32)
        rows = pl.ds(pl.multiple_of(r * (RB // 2), RB // 2), RB // 2)
        for j in range(HP):
            ev = raw32[pl.ds(j, RB // 2, stride=2 * HP), :]
            od = raw32[pl.ds(HP + j, RB // 2, stride=2 * HP), :]
            lo = (ev & 0xFFFF) | (od << 16)
            hi = lax.shift_right_logical(ev, 16) | (od & -65536)
            g, i = divmod(2 * j, HG)
            c0 = m * GW + i * Dh
            wqkv_v[g, rows, pl.ds(c0, Dh)] = lo
            wqkv_v[g, rows, pl.ds(c0 + Dh, Dh)] = hi

    def precompute(m, r):
        for j in range(n_grp // n_rb):
            g = r * (n_grp // n_rb) + j
            w = pltpu.bitcast(wqkv_v[g, :, pl.ds(m * GW, GW)], BF16)
            pre_v[g, :, pl.ds(m * GW, GW)] = _dot(pre_in[...], w).astype(BF16)

    x_head.wait()
    for s in range(LAG, LAG + PRE):
        x0 = x_v[pl.ds(s * SEG, SEG), :].astype(F32)
        pre_in[pl.ds((s - LAG) * SEG, SEG), :] = _layernorm(x0).astype(BF16)

    def load_body(m, r, carry):
        wait_queued(m, r)
        if m == 3:
            @pl.when(r == n_rb - 2)
            def _():
                wg_copy.start()
        if m >= 1:
            precompute(m - 1, r)
        if m < 3:
            relayout(m, r)
        return carry

    for m in range(4):
        lax.fori_loop(0, n_rb, functools.partial(load_body, m), 0)
    wu_copy.start()
    wd_copy.start()

    def seg_rows(s):
        return pl.ds(pl.multiple_of(s * SEG, SEG), SEG)

    def slot(s):
        return s & (RING - 1)

    def load_segment(s):
        x0 = x_v[seg_rows(s), :].astype(F32)
        res_v[slot(s)] = x0
        return x0

    mem0 = mem0_ref[...].astype(F32)
    lhs_a[pl.ds(SEG, MM), :] = jnp.concatenate([mem0, mem0], axis=0).astype(BF16)
    for s in range(LAG + 1):
        load_segment(s)

    def qkv(g, rows):
        return _dot(lhs_a[pl.ds(R2 - rows, rows), :], pltpu.bitcast(wqkv_v[g], BF16)).astype(BF16)

    def padded(a):
        return jnp.concatenate([a, jnp.zeros((128 - a.shape[0], Dh), BF16)], axis=0)

    def scores(p):
        return [lax.dot_general(p[:, i * Dh:(i + 1) * Dh],
                                padded(p[:, GW + i * Dh:GW + (i + 1) * Dh]),
                                (((1,), (1,)), ((), ())), preferred_element_type=F32)
                for i in range(HG)]

    def attend(p, ss, fill_ref):
        out = []
        for i in range(HG):
            fill = fill_ref[...]
            s = jnp.where(fill == 0.0, ss[i], fill)
            e = jnp.exp2((s - jnp.max(s, axis=-1, keepdims=True)) * exp_c)
            inv = 1.0 / jnp.sum(e, axis=-1, keepdims=True)
            v = padded(p[:, 2 * GW + i * Dh:2 * GW + (i + 1) * Dh])
            out.append((_dot(e.astype(BF16), v) * inv).astype(BF16))
        return jnp.concatenate(out, axis=1)

    def project(g, o, segs):
        rows = o.shape[0]
        y = _dot(o, wo_v[pl.ds(g * GW, GW), :])
        blocks = (0, SEG + MM) if len(segs) == 2 else (MM,)
        mem_lo = rows - R1
        if g == 0:
            acc_o[pl.ds(mem_lo, MM), :] = y[mem_lo:mem_lo + MM]
            for lo, s in zip(blocks, segs):
                acc_o[pl.ds(lo, SEG), :] = res_v[slot(s)] + y[lo:lo + SEG]
        elif g < n_grp - 1:
            acc_o[pl.ds(0, rows), :] += y
        else:
            y = acc_o[pl.ds(0, rows), :] + y
            for lo, s in zip(blocks, segs):
                res_v[slot(s)] = y[lo:lo + SEG]
            return y[mem_lo:mem_lo + MM]

    def ffn_input(segs):
        for n, s in enumerate(segs):
            x = res_v[slot(s)]
            acc_f[pl.ds(n * SEG, SEG), :] = x
            lhs_f[pl.ds(n * SEG, SEG), :] = _layernorm(x).astype(BF16)

    def ffn_up(c):
        h = lhs_f[...]
        gate = _dot(h, wg_v[:, pl.ds(c * FC, FC)])
        up = _dot(h, wu_v[:, pl.ds(c * FC, FC)])
        return (_gelu(gate) * up).astype(BF16)

    def ffn_down(c, a, segs):
        y = _dot(a, wd_v[pl.ds(c * FC, FC), :])
        if c < n_fc - 1:
            acc_f[...] += y
        else:
            y = acc_f[...] + y
            for n, s in enumerate(segs):
                r = y[n * SEG:(n + 1) * SEG]
                res_v[slot(s)] = r
                o_v[seg_rows(s), :] = r.astype(BF16)

    def out_copy(s):
        return pltpu.make_async_copy(o_v.at[seg_rows(s)], out_hbm.at[seg_rows(s)], out_sem)

    def attention_input(n, x):
        lhs_a[pl.ds(n * (SEG + MM), SEG), :] = _layernorm(x).astype(BF16)

    def ffn_cuts(parts):
        width = DF // parts
        cuts = list(range(0, width, FC)) + [width]
        return [(width, lo, hi - lo) for lo, hi in zip(cuts, cuts[1:])]

    def ffn_piece(op, k, cut, act):
        width, lo, n = cut
        cols = pl.ds(pl.multiple_of(k * width + lo, 128), n)
        if op == "u":
            h = lhs_f[...]
            return (_gelu(_dot(h, wg_v[:, cols])) * _dot(h, wu_v[:, cols])).astype(BF16)
        acc_f[...] += _dot(act, wd_v[cols, :])

    def project_piece(g, o):
        acc_o[pl.ds(0, o.shape[0]), :] += _dot(
            o, wo_v[pl.ds(pl.multiple_of(g * GW, GW), GW), :])

    def ffn_output(segs):
        for n, s in enumerate(segs):
            r = acc_f[pl.ds(n * SEG, SEG), :]
            res_v[slot(s)] = r
            o_v[seg_rows(s), :] = r.astype(BF16)

    def single_attention(layer, s):
        attention_input(1, res_v[slot(s)])
        acc_o[pl.ds(0, MM), :] = jnp.zeros((MM, D), F32)
        acc_o[pl.ds(MM, SEG), :] = res_v[slot(s)]
        gs = n_grp // ATT_PARTS

        def part(k, c):
            p, ss, o = {}, {}, {}
            for op, n in _step_order(gs, 1):
                g = k * gs + n
                if op == "q":
                    p[n] = qkv(g, R1)
                elif op == "s":
                    ss[n] = scores(p[n])
                elif op == "a":
                    o[n] = attend(p[n], ss[n], fill_s.at[layer])
                elif op == "o":
                    project_piece(g, o[n])
            return c

        lax.fori_loop(0, ATT_PARTS, part, 0)
        res_v[slot(s)] = acc_o[pl.ds(MM, SEG), :]
        own = jnp.where(lax.broadcasted_iota(jnp.int32, (MM, D), 0) < M, 0, 1) == layer
        lhs_a[pl.ds(SEG, MM), :] = jnp.where(
            own, acc_o[pl.ds(0, MM), :], lhs_a[pl.ds(SEG, MM), :].astype(F32)).astype(BF16)

    def single_ffn(segs):
        ffn_input(segs)
        cuts = ffn_cuts(FFN_PARTS)

        def part(k, c):
            a = {0: ffn_piece("u", k, cuts[0], None)}
            for n, cut in enumerate(cuts):
                if n + 1 < len(cuts):
                    a[n + 1] = ffn_piece("u", k, cuts[n + 1], None)
                ffn_piece("d", k, cut, a[n])
            return c

        lax.fori_loop(0, FFN_PARTS, part, 0)
        ffn_output(segs)

    def step_segments(t):
        return (t, t - LAG), (t - 1, jnp.where(t == LAG, t - 2, t - LAG - 1))

    def next_attention_input(t):
        attention_input(0, load_segment(jnp.minimum(t + 1, n_seg - 1)))
        attention_input(1, res_v[slot(t + 1 - LAG)])

    def write_out(t):
        @pl.when(t > LAG)
        def _():
            out_copy(t - LAG - 1).start()

    def paired_step(t, carry):
        att, ffn = step_segments(t)
        p, ss, o, a = {}, {}, {}, {}
        for op, n in _step_order(n_grp, n_fc):
            if op == "q":
                p[n] = qkv(n, R2)
            elif op == "s":
                ss[n] = scores(p[n])
            elif op == "a":
                o[n] = attend(p[n], ss[n], fill_v)
            elif op == "o":
                mem = project(n, o[n], att)
                if n == n_grp - 1:
                    lhs_a[pl.ds(SEG, MM), :] = mem.astype(BF16)
            elif op == "i":
                ffn_input(ffn)
            elif op == "u":
                a[n] = ffn_up(n)
            elif op == "d":
                ffn_down(n, a[n], ffn)
            else:
                next_attention_input(t)
        write_out(t)
        return carry

    def precomputed_step(t, carry):
        att, ffn = step_segments(t)
        pre_rows = pl.ds(pl.multiple_of((t - LAG) * SEG, SEG), SEG)
        gs, cuts = n_grp // PRE_PARTS, ffn_cuts(PRE_PARTS)
        acc_o[pl.ds(0, SEG), :] = res_v[slot(att[0])]
        acc_o[pl.ds(SEG, MM), :] = jnp.zeros((MM, D), F32)
        acc_o[pl.ds(SEG + MM, SEG), :] = res_v[slot(att[1])]
        for n, s in enumerate(ffn):
            acc_f[pl.ds(n * SEG, SEG), :] = res_v[slot(s)]

        def part(k, c):
            p, ss, o, a = {}, {}, {}, {}
            for op, n in _step_order(gs, len(cuts)):
                g = k * gs + n
                if op == "q":
                    p[n] = jnp.concatenate([pre_v[g, pre_rows, :], qkv(g, R1)], axis=0)
                elif op == "s":
                    ss[n] = scores(p[n])
                elif op == "a":
                    o[n] = attend(p[n], ss[n], fill_v)
                elif op == "o":
                    project_piece(g, o[n])
                elif op == "i":
                    for j, s in enumerate(ffn):
                        lhs_f[pl.ds(j * SEG, SEG), :] = _layernorm(res_v[slot(s)]).astype(BF16)
                elif op in "ud":
                    a[n] = ffn_piece(op, k, cuts[n], a.get(n))
            return c

        lax.fori_loop(0, PRE_PARTS, part, 0)
        res_v[slot(att[0])] = acc_o[pl.ds(0, SEG), :]
        lhs_a[pl.ds(SEG, MM), :] = acc_o[pl.ds(SEG, MM), :].astype(BF16)
        res_v[slot(att[1])] = acc_o[pl.ds(SEG + MM, SEG), :]
        ffn_output(ffn)
        next_attention_input(t)
        write_out(t)
        return carry

    def single_op(phase, i):
        is_head = phase == 0
        j = i - 1
        tail_ffn = lax.rem(i, 3) == 0
        is_ffn = jnp.where(is_head, i == LAG, tail_ffn)
        first = n_seg - LAG + 2 * lax.div(jnp.maximum(j, 0), 3)

        @pl.when(jnp.logical_not(is_ffn))
        def _():
            single_attention(phase, jnp.where(is_head, i, first + lax.rem(j, 3)))

        @pl.when(is_ffn)
        def _():
            @pl.when(is_head)
            def _():
                for c in (wg_copy, wu_copy, wd_copy):
                    c.wait()
                x_rest.start()

            s0 = jnp.where(is_head, 0, jnp.where(i == 0, n_seg - 1, first))
            s1 = jnp.where(is_head, 1, jnp.where(i == 0, n_seg - LAG - 1, first + 1))
            single_ffn((s0, s1))

            @pl.when(jnp.logical_not(is_head))
            def _():
                out_copy(s1).start()

                @pl.when(i > 0)
                def _():
                    out_copy(s0).start()

    def phase_body(phase, carry):
        n_ops = jnp.where(phase == 0, LAG + 1, 1 + 3 * (LAG // 2))
        lax.fori_loop(0, n_ops, lambda i, c: (single_op(phase, i), c)[1], 0)

        @pl.when(phase == 0)
        def _():
            x_rest.wait()
            attention_input(1, res_v[slot(0)])
            lax.fori_loop(LAG, LAG + PRE, precomputed_step, 0)
            lax.fori_loop(LAG + PRE, n_seg, paired_step, 0)

        return carry

    lax.fori_loop(0, 2, phase_body, 0)
    pltpu.make_async_copy(o_v, out_hbm, out_sem).wait()


@functools.partial(jax.jit, static_argnames=("A_seg_len",))
def pallas_interleave_layers__memory_aug_recurrent_mem_tr__glu_gated_geglu__prompt_kernel(
    A_x, A_mem0, A_Wq, A_Wk, A_Wv, A_Wo, A_seg_len, B_x, B_w_gate, B_w_up, B_w_down,
):
    del B_x
    B, S, D = A_x.shape
    _, H, Dh = A_Wq.shape
    M = A_mem0.shape[1]
    SEG = int(A_seg_len)
    DF = B_w_gate.shape[1]
    assert B == 1 and S % SEG == 0 and Dh == 128 and 2 * (M + SEG) <= 128
    R = 2 * (M + SEG)
    hbm = pl.BlockSpec(memory_space=pl.ANY)
    out = pl.pallas_call(
        functools.partial(_kernel, S=S, D=D, H=H, Dh=Dh, M=M, SEG=SEG, DF=DF),
        out_shape=jax.ShapeDtypeStruct((S, D), A_x.dtype),
        in_specs=[hbm, pl.BlockSpec(memory_space=pltpu.VMEM)] + [hbm] * 7,
        out_specs=hbm,
        scratch_shapes=[
            pltpu.VMEM((S, D), BF16),
            pltpu.VMEM((S, D), BF16),
            pltpu.VMEM((3 * D * H, Dh), BF16),
            pltpu.VMEM((H // HG, D // 2, 3 * HG * Dh), jnp.int32),
            pltpu.VMEM((H * Dh, D), BF16),
            pltpu.VMEM((D, DF), BF16),
            pltpu.VMEM((D, DF), BF16),
            pltpu.VMEM((DF, D), BF16),
            pltpu.VMEM((RING, SEG, D), F32),
            pltpu.VMEM((R, D), BF16),
            pltpu.VMEM((R, D), F32),
            pltpu.VMEM((2 * SEG, D), BF16),
            pltpu.VMEM((2 * SEG, D), F32),
            pltpu.VMEM((R, 128), F32),
            pltpu.VMEM((2, R - SEG, 128), F32),
            pltpu.VMEM((PRE * SEG, D), BF16),
            pltpu.VMEM((H // HG, PRE * SEG, 3 * HG * Dh), BF16),
            pltpu.SemaphoreType.DMA((4 * (D // RB),)),
            pltpu.SemaphoreType.DMA((5,)),
            pltpu.SemaphoreType.DMA(()),
        ],
        compiler_params=pltpu.CompilerParams(vmem_limit_bytes=120 * 2**20),
    )(A_x.reshape(S, D), A_mem0.reshape(M, D),
      A_Wq.reshape(D * H, Dh), A_Wk.reshape(D * H, Dh), A_Wv.reshape(D * H, Dh),
      A_Wo.reshape(H * Dh, D), B_w_gate, B_w_up, B_w_down)
    return out.reshape(B, S, D)
```

```python
import functools
import math

import jax
import jax.numpy as jnp
import numpy as np
from jax import lax
from jax.experimental import pallas as pl
from jax.experimental.pallas import tpu as pltpu

F32 = jnp.float32
BF16 = jnp.bfloat16

HG = 2
FC = 512
LAG = 4
WINDOW = 4
PRE = 7
PRE_PARTS = 4
ATT_PARTS = 2
FFN_PARTS = 2
RING = 8
RB = 256
PRE_ROWS = 112
FFN_START = 24


def _step_order(n_grp, n_fc):
    at = [(c * (n_grp - 1)) // n_fc for c in range(n_fc)]
    order = [("q", 0), ("i", 0), ("q", 1), ("s", 0)]
    for g in range(n_grp):
        last = g == n_grp - 1
        if g + 2 < n_grp:
            order.append(("q", g + 2))
        if not last:
            order.append(("s", g + 1))
        if g + 2 == n_grp:
            order.append(("n", 0))
        order.append(("a", g))
        if g >= 1:
            order.append(("o", g - 1))
        order += [("u", c) for c in range(n_fc) if at[c] == g]
        order += [("d", c) for c in range(n_fc - 1) if at[c] + 1 == g]
    return order + [("o", n_grp - 1), ("d", n_fc - 1)]


def _layernorm(x):
    m = jnp.mean(x, axis=-1, keepdims=True)
    c = x - m
    v = jnp.mean(c * c, axis=-1, keepdims=True)
    return c * lax.rsqrt(v + 1e-5)


def _gelu(x):
    c0 = math.sqrt(2.0 / math.pi)
    inner = x * (c0 + (c0 * 0.044715) * (x * x))
    return (0.5 * x) * (1.0 + jnp.tanh(inner))


def _dot(a, b):
    return jnp.dot(a, b, preferred_element_type=F32)


def _kernel(x_hbm, mem0_ref, wq_hbm, wk_hbm, wv_hbm, wo_hbm, wg_hbm, wu_hbm, wd_hbm,
            out_hbm,
            x_v, o_v, raw_v, wqkv_v, wo_v, wg_v, wu_v, wd_v,
            res_v, lhs_a, acc_o, lhs_f, acc_f, fill_v, fill_s, pre_in, pre_v,
            chunk_sem, w_sem, out_sem,
            *, S, D, H, Dh, M, SEG, DF):
    n_seg = S // SEG
    MM = 2 * M
    R2 = MM + 2 * SEG
    R1 = MM + SEG
    n_grp = H // HG
    n_fc = DF // FC
    GW = HG * Dh
    scale = Dh ** -0.5
    exp_c = scale * math.log2(math.e)

    n_rb = D // RB
    n_raw = 6 * n_rb
    n_chunk = 8 * n_rb
    HH = H // 2

    def raw_copy(w_hbm, i):
        unit, r = lax.div(i, n_rb), lax.rem(i, n_rb)
        heads = pl.ds(pl.multiple_of(lax.div(unit, 3) * HH, HH), HH)
        return pltpu.make_async_copy(
            w_hbm.at[pl.ds(pl.multiple_of(r * RB, RB), RB), heads],
            raw_v.at[pl.ds(pl.multiple_of(i * RB, RB), RB)], chunk_sem.at[i])

    def wo_copy(i):
        n = H * Dh // (2 * n_rb)
        rows = pl.ds(pl.multiple_of((i - n_raw) * n, n), n)
        return pltpu.make_async_copy(wo_hbm.at[rows], wo_v.at[rows], chunk_sem.at[i])

    def start_chunk(i, carry=None):
        for m, w_hbm in enumerate((wq_hbm, wk_hbm, wv_hbm)):
            @pl.when(jnp.logical_and(i < n_raw, lax.rem(lax.div(i, n_rb), 3) == m))
            def _():
                raw_copy(w_hbm, i).start()

        @pl.when(i >= n_raw)
        def _():
            wo_copy(i).start()

        return carry

    head_rows = (LAG + PRE) * SEG
    x_head, wg_copy, wu_copy, wd_copy, x_rest = [
        pltpu.make_async_copy(s, d, w_sem.at[i]) for i, (s, d) in enumerate((
            (x_hbm.at[pl.ds(0, head_rows)], x_v.at[pl.ds(0, head_rows)]),
            (wg_hbm, wg_v), (wu_hbm, wu_v), (wd_hbm, wd_v),
            (x_hbm.at[pl.ds(head_rows, S - head_rows)],
             x_v.at[pl.ds(head_rows, S - head_rows)])))]
    x_head.start()
    lax.fori_loop(0, WINDOW, start_chunk, None)

    def make_fill(rows, mem_lo, layer_of):
        row = lax.broadcasted_iota(jnp.int32, (rows, 128), 0)
        col = lax.broadcasted_iota(jnp.int32, (rows, 128), 1)

        def is_mem(i):
            return (i >= mem_lo) & (i < mem_lo + MM)

        keep = is_mem(row) | is_mem(col) | (row >= col)
        return jnp.where(layer_of(row) == layer_of(col),
                         jnp.where(keep, 0.0, -1e9 / scale), -jnp.inf).astype(F32)

    fill_v[...] = make_fill(
        R2, SEG, lambda i: jnp.where(i < SEG + M, 0, jnp.where(i < R2, 1, 2)))
    for layer in range(2):
        fill_s[layer] = make_fill(R1, 0, lambda i: jnp.where(
            i < M, 0, jnp.where(i < MM, 1, jnp.where(i < R1, layer, 2))))

    grp_half = n_grp // 2

    def relayout(i):
        unit, r = lax.div(i, n_rb), lax.rem(i, n_rb)
        half, m = lax.div(unit, 3), lax.rem(unit, 3)
        for t in range(RB // 16):
            x = raw_v[pl.ds(pl.multiple_of(i * RB + t * 16, 16), 16)].reshape(16 * HH, Dh)
            x = pltpu.bitcast(x, jnp.int32).reshape(8, 2, HH // 2, Dh)
            ev, od = x[:, 0], x[:, 1]
            lo = jnp.swapaxes((ev & 0xFFFF) | (od << 16), 0, 1)
            hi = jnp.swapaxes(lax.shift_right_logical(ev, 16) | (od & -65536), 0, 1)
            rows = pl.ds(pl.multiple_of(r * (RB // 2) + t * 8, 8), 8)
            for j in range(HH // 2):
                g, c = divmod(2 * j, HG)
                wqkv_v[m, half * grp_half + g, rows, pl.ds(c * Dh, Dh)] = lo[j]
                wqkv_v[m, half * grp_half + g, rows, pl.ds((c + 1) * Dh, Dh)] = hi[j]

    def precompute(i):
        unit, r = lax.div(i, n_rb), lax.rem(i, n_rb)
        half, m = lax.div(unit, 3), lax.rem(unit, 3)
        for j in range(grp_half // n_rb):
            g = half * grp_half + r * (grp_half // n_rb) + j
            w = pltpu.bitcast(wqkv_v[m, g], BF16)
            for lo in range(0, PRE * SEG, PRE_ROWS):
                rows = pl.ds(lo, min(PRE_ROWS, PRE * SEG - lo))
                pre_v[m, g, rows, :] = _dot(pre_in[rows, :], w).astype(BF16)

    x_head.wait()
    for s in range(LAG, LAG + PRE):
        x0 = x_v[pl.ds(s * SEG, SEG), :].astype(F32)
        pre_in[pl.ds((s - LAG) * SEG, SEG), :] = _layernorm(x0).astype(BF16)

    def load_body(i, carry):
        @pl.when(i < n_raw)
        def _():
            raw_copy(wq_hbm, i).wait()
            relayout(i)

        @pl.when(i >= n_raw)
        def _():
            wo_copy(i).wait()

        def started(n):
            return jnp.minimum(WINDOW + n + lax.div(jnp.maximum(n - n_rb, 0), 3), n_chunk)

        lax.fori_loop(started(i), started(i + 1), start_chunk, None)

        @pl.when(i == FFN_START)
        def _():
            wg_copy.start()

        @pl.when(jnp.logical_and(i >= n_rb, i < n_raw + n_rb))
        def _():
            precompute(i - n_rb)

        return carry

    lax.fori_loop(0, n_chunk, load_body, 0)
    wu_copy.start()
    wd_copy.start()

    def seg_rows(s):
        return pl.ds(pl.multiple_of(s * SEG, SEG), SEG)

    def slot(s):
        return s & (RING - 1)

    def load_segment(s):
        x0 = x_v[seg_rows(s), :].astype(F32)
        res_v[slot(s)] = x0
        return x0

    mem0 = mem0_ref[...].astype(F32)
    lhs_a[pl.ds(SEG, MM), :] = jnp.concatenate([mem0, mem0], axis=0).astype(BF16)
    for s in range(LAG + 1):
        load_segment(s)

    def qkv(g, rows):
        h = lhs_a[pl.ds(R2 - rows, rows), :]
        return jnp.concatenate(
            [_dot(h, pltpu.bitcast(wqkv_v[m, g], BF16)).astype(BF16) for m in range(3)],
            axis=1)

    def padded(a):
        return jnp.concatenate([a, jnp.zeros((128 - a.shape[0], Dh), BF16)], axis=0)

    def scores(p):
        return [lax.dot_general(p[:, i * Dh:(i + 1) * Dh],
                                padded(p[:, GW + i * Dh:GW + (i + 1) * Dh]),
                                (((1,), (1,)), ((), ())), preferred_element_type=F32)
                for i in range(HG)]

    def attend(p, ss, fill_ref):
        out = []
        for i in range(HG):
            fill = fill_ref[...]
            s = jnp.where(fill == 0.0, ss[i], fill)
            e = jnp.exp2((s - jnp.max(s, axis=-1, keepdims=True)) * exp_c)
            inv = 1.0 / jnp.sum(e, axis=-1, keepdims=True)
            v = padded(p[:, 2 * GW + i * Dh:2 * GW + (i + 1) * Dh])
            out.append((_dot(e.astype(BF16), v) * inv).astype(BF16))
        return jnp.concatenate(out, axis=1)

    def project(g, o, segs):
        rows = o.shape[0]
        y = _dot(o, wo_v[pl.ds(g * GW, GW), :])
        blocks = (0, SEG + MM) if len(segs) == 2 else (MM,)
        mem_lo = rows - R1
        if g == 0:
            acc_o[pl.ds(mem_lo, MM), :] = y[mem_lo:mem_lo + MM]
            for lo, s in zip(blocks, segs):
                acc_o[pl.ds(lo, SEG), :] = res_v[slot(s)] + y[lo:lo + SEG]
        elif g < n_grp - 1:
            acc_o[pl.ds(0, rows), :] += y
        else:
            y = acc_o[pl.ds(0, rows), :] + y
            for lo, s in zip(blocks, segs):
                res_v[slot(s)] = y[lo:lo + SEG]
            return y[mem_lo:mem_lo + MM]

    def ffn_input(segs):
        for n, s in enumerate(segs):
            x = res_v[slot(s)]
            acc_f[pl.ds(n * SEG, SEG), :] = x
            lhs_f[pl.ds(n * SEG, SEG), :] = _layernorm(x).astype(BF16)

    def ffn_up(c):
        h = lhs_f[...]
        gate = _dot(h, wg_v[:, pl.ds(c * FC, FC)])
        up = _dot(h, wu_v[:, pl.ds(c * FC, FC)])
        return (_gelu(gate) * up).astype(BF16)

    def ffn_down(c, a, segs):
        y = _dot(a, wd_v[pl.ds(c * FC, FC), :])
        if c < n_fc - 1:
            acc_f[...] += y
        else:
            y = acc_f[...] + y
            for n, s in enumerate(segs):
                r = y[n * SEG:(n + 1) * SEG]
                res_v[slot(s)] = r
                o_v[seg_rows(s), :] = r.astype(BF16)

    def out_copy(s):
        return pltpu.make_async_copy(o_v.at[seg_rows(s)], out_hbm.at[seg_rows(s)], out_sem)

    def attention_input(n, x):
        lhs_a[pl.ds(n * (SEG + MM), SEG), :] = _layernorm(x).astype(BF16)

    def ffn_cuts(parts):
        width = DF // parts
        cuts = list(range(0, width, FC)) + [width]
        return [(width, lo, hi - lo) for lo, hi in zip(cuts, cuts[1:])]

    def ffn_piece(op, k, cut, act):
        width, lo, n = cut
        cols = pl.ds(pl.multiple_of(k * width + lo, 128), n)
        if op == "u":
            h = lhs_f[...]
            return (_gelu(_dot(h, wg_v[:, cols])) * _dot(h, wu_v[:, cols])).astype(BF16)
        acc_f[...] += _dot(act, wd_v[cols, :])

    def project_piece(g, o):
        acc_o[pl.ds(0, o.shape[0]), :] += _dot(
            o, wo_v[pl.ds(pl.multiple_of(g * GW, GW), GW), :])

    def ffn_output(segs):
        for n, s in enumerate(segs):
            r = acc_f[pl.ds(n * SEG, SEG), :]
            res_v[slot(s)] = r
            o_v[seg_rows(s), :] = r.astype(BF16)

    def single_attention(layer, s):
        attention_input(1, res_v[slot(s)])
        acc_o[pl.ds(0, MM), :] = jnp.zeros((MM, D), F32)
        acc_o[pl.ds(MM, SEG), :] = res_v[slot(s)]
        gs = n_grp // ATT_PARTS

        def part(k, c):
            p, ss, o = {}, {}, {}
            for op, n in _step_order(gs, 1):
                g = k * gs + n
                if op == "q":
                    p[n] = qkv(g, R1)
                elif op == "s":
                    ss[n] = scores(p[n])
                elif op == "a":
                    o[n] = attend(p[n], ss[n], fill_s.at[layer])
                elif op == "o":
                    project_piece(g, o[n])
            return c

        lax.fori_loop(0, ATT_PARTS, part, 0)
        res_v[slot(s)] = acc_o[pl.ds(MM, SEG), :]
        own = jnp.where(lax.broadcasted_iota(jnp.int32, (MM, D), 0) < M, 0, 1) == layer
        lhs_a[pl.ds(SEG, MM), :] = jnp.where(
            own, acc_o[pl.ds(0, MM), :], lhs_a[pl.ds(SEG, MM), :].astype(F32)).astype(BF16)

    def single_ffn(segs):
        ffn_input(segs)
        cuts = ffn_cuts(FFN_PARTS)

        def part(k, c):
            a = {0: ffn_piece("u", k, cuts[0], None)}
            for n, cut in enumerate(cuts):
                if n + 1 < len(cuts):
                    a[n + 1] = ffn_piece("u", k, cuts[n + 1], None)
                ffn_piece("d", k, cut, a[n])
            return c

        lax.fori_loop(0, FFN_PARTS, part, 0)
        ffn_output(segs)

    def step_segments(t):
        return (t, t - LAG), (t - 1, jnp.where(t == LAG, t - 2, t - LAG - 1))

    def next_attention_input(t):
        attention_input(0, load_segment(jnp.minimum(t + 1, n_seg - 1)))
        attention_input(1, res_v[slot(t + 1 - LAG)])

    def write_out(t):
        @pl.when(t > LAG)
        def _():
            out_copy(t - LAG - 1).start()

    def paired_step(t, carry):
        att, ffn = step_segments(t)
        p, ss, o, a = {}, {}, {}, {}
        for op, n in _step_order(n_grp, n_fc):
            if op == "q":
                p[n] = qkv(n, R2)
            elif op == "s":
                ss[n] = scores(p[n])
            elif op == "a":
                o[n] = attend(p[n], ss[n], fill_v)
            elif op == "o":
                mem = project(n, o[n], att)
                if n == n_grp - 1:
                    lhs_a[pl.ds(SEG, MM), :] = mem.astype(BF16)
            elif op == "i":
                ffn_input(ffn)
            elif op == "u":
                a[n] = ffn_up(n)
            elif op == "d":
                ffn_down(n, a[n], ffn)
            else:
                next_attention_input(t)
        write_out(t)
        return carry

    def precomputed_step(t, carry):
        att, ffn = step_segments(t)
        pre_rows = pl.ds(pl.multiple_of((t - LAG) * SEG, SEG), SEG)
        gs, cuts = n_grp // PRE_PARTS, ffn_cuts(PRE_PARTS)
        acc_o[pl.ds(0, SEG), :] = res_v[slot(att[0])]
        acc_o[pl.ds(SEG, MM), :] = jnp.zeros((MM, D), F32)
        acc_o[pl.ds(SEG + MM, SEG), :] = res_v[slot(att[1])]
        for n, s in enumerate(ffn):
            acc_f[pl.ds(n * SEG, SEG), :] = res_v[slot(s)]

        def part(k, c):
            p, ss, o, a = {}, {}, {}, {}
            for op, n in _step_order(gs, len(cuts)):
                g = k * gs + n
                if op == "q":
                    p[n] = jnp.concatenate(
                        [jnp.concatenate([pre_v[m, g, pre_rows, :] for m in range(3)], axis=1),
                         qkv(g, R1)], axis=0)
                elif op == "s":
                    ss[n] = scores(p[n])
                elif op == "a":
                    o[n] = attend(p[n], ss[n], fill_v)
                elif op == "o":
                    project_piece(g, o[n])
                elif op == "i":
                    for j, s in enumerate(ffn):
                        lhs_f[pl.ds(j * SEG, SEG), :] = _layernorm(res_v[slot(s)]).astype(BF16)
                elif op in "ud":
                    a[n] = ffn_piece(op, k, cuts[n], a.get(n))
            return c

        lax.fori_loop(0, PRE_PARTS, part, 0)
        res_v[slot(att[0])] = acc_o[pl.ds(0, SEG), :]
        lhs_a[pl.ds(SEG, MM), :] = acc_o[pl.ds(SEG, MM), :].astype(BF16)
        res_v[slot(att[1])] = acc_o[pl.ds(SEG + MM, SEG), :]
        ffn_output(ffn)
        next_attention_input(t)
        write_out(t)
        return carry

    def single_op(phase, i):
        is_head = phase == 0
        j = i - 1
        tail_ffn = lax.rem(i, 3) == 0
        is_ffn = jnp.where(is_head, i == LAG, tail_ffn)
        first = n_seg - LAG + 2 * lax.div(jnp.maximum(j, 0), 3)

        @pl.when(jnp.logical_not(is_ffn))
        def _():
            single_attention(phase, jnp.where(is_head, i, first + lax.rem(j, 3)))

        @pl.when(is_ffn)
        def _():
            @pl.when(is_head)
            def _():
                for c in (wg_copy, wu_copy, wd_copy):
                    c.wait()
                x_rest.start()

            s0 = jnp.where(is_head, 0, jnp.where(i == 0, n_seg - 1, first))
            s1 = jnp.where(is_head, 1, jnp.where(i == 0, n_seg - LAG - 1, first + 1))
            single_ffn((s0, s1))

            @pl.when(jnp.logical_not(is_head))
            def _():
                out_copy(s1).start()

                @pl.when(i > 0)
                def _():
                    out_copy(s0).start()

    def phase_body(phase, carry):
        n_ops = jnp.where(phase == 0, LAG + 1, 1 + 3 * (LAG // 2))
        lax.fori_loop(0, n_ops, lambda i, c: (single_op(phase, i), c)[1], 0)

        @pl.when(phase == 0)
        def _():
            x_rest.wait()
            attention_input(1, res_v[slot(0)])
            lax.fori_loop(LAG, LAG + PRE, precomputed_step, 0)
            lax.fori_loop(LAG + PRE, n_seg, paired_step, 0)

        return carry

    lax.fori_loop(0, 2, phase_body, 0)
    pltpu.make_async_copy(o_v, out_hbm, out_sem).wait()


@functools.partial(jax.jit, static_argnames=("A_seg_len",))
def pallas_interleave_layers__memory_aug_recurrent_mem_tr__glu_gated_geglu__prompt_kernel(
    A_x, A_mem0, A_Wq, A_Wk, A_Wv, A_Wo, A_seg_len, B_x, B_w_gate, B_w_up, B_w_down,
):
    del B_x
    B, S, D = A_x.shape
    _, H, Dh = A_Wq.shape
    M = A_mem0.shape[1]
    SEG = int(A_seg_len)
    DF = B_w_gate.shape[1]
    assert B == 1 and S % SEG == 0 and Dh == 128 and 2 * (M + SEG) <= 128
    R = 2 * (M + SEG)
    hbm = pl.BlockSpec(memory_space=pl.ANY)
    out = pl.pallas_call(
        functools.partial(_kernel, S=S, D=D, H=H, Dh=Dh, M=M, SEG=SEG, DF=DF),
        out_shape=jax.ShapeDtypeStruct((S, D), A_x.dtype),
        in_specs=[hbm, pl.BlockSpec(memory_space=pltpu.VMEM)] + [hbm] * 7,
        out_specs=hbm,
        scratch_shapes=[
            pltpu.VMEM((S, D), BF16),
            pltpu.VMEM((S, D), BF16),
            pltpu.VMEM((6 * D, H // 2, Dh), BF16),
            pltpu.VMEM((3, H // HG, D // 2, HG * Dh), jnp.int32),
            pltpu.VMEM((H * Dh, D), BF16),
            pltpu.VMEM((D, DF), BF16),
            pltpu.VMEM((D, DF), BF16),
            pltpu.VMEM((DF, D), BF16),
            pltpu.VMEM((RING, SEG, D), F32),
            pltpu.VMEM((R, D), BF16),
            pltpu.VMEM((R, D), F32),
            pltpu.VMEM((2 * SEG, D), BF16),
            pltpu.VMEM((2 * SEG, D), F32),
            pltpu.VMEM((R, 128), F32),
            pltpu.VMEM((2, R - SEG, 128), F32),
            pltpu.VMEM((PRE * SEG, D), BF16),
            pltpu.VMEM((3, H // HG, PRE * SEG, HG * Dh), BF16),
            pltpu.SemaphoreType.DMA((8 * (D // RB),)),
            pltpu.SemaphoreType.DMA((5,)),
            pltpu.SemaphoreType.DMA(()),
        ],
        compiler_params=pltpu.CompilerParams(vmem_limit_bytes=120 * 2**20),
    )(A_x.reshape(S, D), A_mem0.reshape(M, D),
      A_Wq, A_Wk, A_Wv,
      A_Wo.reshape(H * Dh, D), B_w_gate, B_w_up, B_w_down)
    return out.reshape(B, S, D)
```

```python
import functools
import math

import jax
import jax.numpy as jnp
import numpy as np
from jax import lax
from jax.experimental import pallas as pl
from jax.experimental.pallas import tpu as pltpu

F32 = jnp.float32
BF16 = jnp.bfloat16

HG = 2
FC = 512
LAG = 4
WINDOW = 4
PRE = 6
PRE_PARTS = 2
ATT_PARTS = 2
FFN_PARTS = 2
RING = 8
RB = 256
PRE_ROWS = 96
ORDER = "usdqao"
FFN_START = 24


def _step_order(n_grp, n_fc):
    at = [(c * (n_grp - 1)) // n_fc for c in range(n_fc)]
    order = [("q", 0), ("i", 0), ("q", 1), ("s", 0)]
    for g in range(n_grp):
        items = {
            "q": [("q", g + 2)] * (g + 2 < n_grp) + [("n", 0)] * (g + 2 == n_grp),
            "s": [("s", g + 1)] * (g + 1 < n_grp),
            "u": [("u", c) for c in range(n_fc) if at[c] == g],
            "d": [("d", c) for c in range(n_fc - 1) if at[c] + 1 == g],
            "a": [("a", g)],
            "o": [("o", g - 1)] * (g >= 1),
        }
        for kind in ORDER:
            order += items[kind]
    return order + [("o", n_grp - 1), ("d", n_fc - 1)]


def _layernorm(x):
    m = jnp.mean(x, axis=-1, keepdims=True)
    c = x - m
    v = jnp.mean(c * c, axis=-1, keepdims=True)
    return c * lax.rsqrt(v + 1e-5)


def _gelu(x):
    c0 = math.sqrt(2.0 / math.pi)
    inner = x * (c0 + (c0 * 0.044715) * (x * x))
    return (0.5 * x) * (1.0 + jnp.tanh(inner))


def _dot(a, b):
    return jnp.dot(a, b, preferred_element_type=F32)


def _kernel(x_hbm, mem0_ref, wq_hbm, wk_hbm, wv_hbm, wo_hbm, wg_hbm, wu_hbm, wd_hbm,
            out_hbm,
            x_v, o_v, raw_v, wqkv_v, wo_v, wg_v, wu_v, wd_v,
            res_v, lhs_a, lhs_next, acc_o, lhs_f, acc_f, fill_v, fill_s, pre_in, pre_v,
            chunk_sem, w_sem, out_sem,
            *, S, D, H, Dh, M, SEG, DF):
    n_seg = S // SEG
    MM = 2 * M
    R2 = MM + 2 * SEG
    R1 = MM + SEG
    n_grp = H // HG
    n_fc = DF // FC
    GW = HG * Dh
    scale = Dh ** -0.5
    exp_c = scale * math.log2(math.e)

    n_rb = D // RB
    n_raw = 6 * n_rb
    n_chunk = 8 * n_rb
    HH = H // 2

    def raw_copy(w_hbm, i):
        unit, r = lax.div(i, n_rb), lax.rem(i, n_rb)
        heads = pl.ds(pl.multiple_of(lax.div(unit, 3) * HH, HH), HH)
        return pltpu.make_async_copy(
            w_hbm.at[pl.ds(pl.multiple_of(r * RB, RB), RB), heads],
            raw_v.at[pl.ds(pl.multiple_of(i * RB, RB), RB)], chunk_sem.at[i])

    def wo_copy(i):
        n = H * Dh // (2 * n_rb)
        rows = pl.ds(pl.multiple_of((i - n_raw) * n, n), n)
        return pltpu.make_async_copy(wo_hbm.at[rows], wo_v.at[rows], chunk_sem.at[i])

    def start_chunk(i, carry=None):
        for m, w_hbm in enumerate((wq_hbm, wk_hbm, wv_hbm)):
            @pl.when(jnp.logical_and(i < n_raw, lax.rem(lax.div(i, n_rb), 3) == m))
            def _():
                raw_copy(w_hbm, i).start()

        @pl.when(i >= n_raw)
        def _():
            wo_copy(i).start()

        return carry

    head_rows = (LAG + PRE + 1) * SEG
    x_head, wg_copy, wu_copy, wd_copy, x_rest = [
        pltpu.make_async_copy(s, d, w_sem.at[i]) for i, (s, d) in enumerate((
            (x_hbm.at[pl.ds(0, head_rows)], x_v.at[pl.ds(0, head_rows)]),
            (wg_hbm, wg_v), (wu_hbm, wu_v), (wd_hbm, wd_v),
            (x_hbm.at[pl.ds(head_rows, S - head_rows)],
             x_v.at[pl.ds(head_rows, S - head_rows)])))]
    x_head.start()
    lax.fori_loop(0, WINDOW, start_chunk, None)

    def make_fill(rows, mem_lo, layer_of):
        row = lax.broadcasted_iota(jnp.int32, (rows, 128), 0)
        col = lax.broadcasted_iota(jnp.int32, (rows, 128), 1)

        def is_mem(i):
            return (i >= mem_lo) & (i < mem_lo + MM)

        keep = is_mem(row) | is_mem(col) | (row >= col)
        return jnp.where(layer_of(row) == layer_of(col),
                         jnp.where(keep, 0.0, -1e9 / scale), -jnp.inf).astype(F32)

    fill_v[...] = make_fill(
        R2, SEG, lambda i: jnp.where(i < SEG + M, 0, jnp.where(i < R2, 1, 2)))
    for layer in range(2):
        fill_s[layer] = make_fill(R1, 0, lambda i: jnp.where(
            i < M, 0, jnp.where(i < MM, 1, jnp.where(i < R1, layer, 2))))

    grp_half = n_grp // 2

    def relayout(i):
        unit, r = lax.div(i, n_rb), lax.rem(i, n_rb)
        half, m = lax.div(unit, 3), lax.rem(unit, 3)
        for t in range(RB // 16):
            x = raw_v[pl.ds(pl.multiple_of(i * RB + t * 16, 16), 16)].reshape(16 * HH, Dh)
            x = pltpu.bitcast(x, jnp.int32).reshape(8, 2, HH // 2, Dh)
            ev, od = x[:, 0], x[:, 1]
            lo = jnp.swapaxes((ev & 0xFFFF) | (od << 16), 0, 1)
            hi = jnp.swapaxes(lax.shift_right_logical(ev, 16) | (od & -65536), 0, 1)
            rows = pl.ds(pl.multiple_of(r * (RB // 2) + t * 8, 8), 8)
            for j in range(HH // 2):
                g, c = divmod(2 * j, HG)
                wqkv_v[m, half * grp_half + g, rows, pl.ds(c * Dh, Dh)] = lo[j]
                wqkv_v[m, half * grp_half + g, rows, pl.ds((c + 1) * Dh, Dh)] = hi[j]

    def precompute(i):
        unit, r = lax.div(i, n_rb), lax.rem(i, n_rb)
        half, m = lax.div(unit, 3), lax.rem(unit, 3)
        for j in range(grp_half // n_rb):
            g = half * grp_half + r * (grp_half // n_rb) + j
            w = pltpu.bitcast(wqkv_v[m, g], BF16)
            for lo in range(0, PRE * SEG, PRE_ROWS):
                rows = pl.ds(lo, min(PRE_ROWS, PRE * SEG - lo))
                pre_v[m, g, rows, :] = _dot(pre_in[rows, :], w).astype(BF16)

    x_head.wait()
    for s in range(LAG, LAG + PRE):
        x0 = x_v[pl.ds(s * SEG, SEG), :].astype(F32)
        pre_in[pl.ds((s - LAG) * SEG, SEG), :] = _layernorm(x0).astype(BF16)

    def load_body(i, carry):
        @pl.when(i < n_raw)
        def _():
            raw_copy(wq_hbm, i).wait()
            relayout(i)

        @pl.when(i >= n_raw)
        def _():
            wo_copy(i).wait()

        def started(n):
            return jnp.minimum(WINDOW + n + lax.div(jnp.maximum(n - n_rb, 0), 3), n_chunk)

        lax.fori_loop(started(i), started(i + 1), start_chunk, None)

        @pl.when(i == FFN_START)
        def _():
            wg_copy.start()

        @pl.when(jnp.logical_and(i >= n_rb, i < n_raw + n_rb))
        def _():
            precompute(i - n_rb)

        return carry

    lax.fori_loop(0, n_chunk, load_body, 0)
    wu_copy.start()
    wd_copy.start()

    def seg_rows(s):
        return pl.ds(pl.multiple_of(s * SEG, SEG), SEG)

    def slot(s):
        return s & (RING - 1)

    def load_segment(s):
        x0 = x_v[seg_rows(s), :].astype(F32)
        res_v[slot(s)] = x0
        return x0

    mem0 = mem0_ref[...].astype(F32)
    lhs_a[pl.ds(SEG, MM), :] = jnp.concatenate([mem0, mem0], axis=0).astype(BF16)
    for s in range(LAG + 1):
        load_segment(s)

    def qkv(g, rows):
        h = lhs_a[pl.ds(R2 - rows, rows), :]
        return jnp.concatenate(
            [_dot(h, pltpu.bitcast(wqkv_v[m, g], BF16)).astype(BF16) for m in range(3)],
            axis=1)

    def padded(a):
        return jnp.concatenate([a, jnp.zeros((128 - a.shape[0], Dh), BF16)], axis=0)

    def scores(p):
        return [lax.dot_general(p[:, i * Dh:(i + 1) * Dh],
                                padded(p[:, GW + i * Dh:GW + (i + 1) * Dh]),
                                (((1,), (1,)), ((), ())), preferred_element_type=F32)
                for i in range(HG)]

    def attend(p, ss, fill_ref):
        out = []
        for i in range(HG):
            fill = fill_ref[...]
            s = jnp.where(fill == 0.0, ss[i], fill)
            e = jnp.exp2((s - jnp.max(s, axis=-1, keepdims=True)) * exp_c)
            inv = 1.0 / jnp.sum(e, axis=-1, keepdims=True)
            v = padded(p[:, 2 * GW + i * Dh:2 * GW + (i + 1) * Dh])
            out.append((_dot(e.astype(BF16), v) * inv).astype(BF16))
        return jnp.concatenate(out, axis=1)

    def project(g, o, segs):
        rows = o.shape[0]
        y = _dot(o, wo_v[pl.ds(g * GW, GW), :])
        blocks = (0, SEG + MM) if len(segs) == 2 else (MM,)
        mem_lo = rows - R1
        if g == 0:
            acc_o[pl.ds(mem_lo, MM), :] = y[mem_lo:mem_lo + MM]
            for lo, s in zip(blocks, segs):
                acc_o[pl.ds(lo, SEG), :] = res_v[slot(s)] + y[lo:lo + SEG]
        elif g < n_grp - 1:
            acc_o[pl.ds(0, rows), :] += y
        else:
            y = acc_o[pl.ds(0, rows), :] + y
            for lo, s in zip(blocks, segs):
                res_v[slot(s)] = y[lo:lo + SEG]
            return y[mem_lo:mem_lo + MM]

    def ffn_input(segs):
        for n, s in enumerate(segs):
            x = res_v[slot(s)]
            acc_f[pl.ds(n * SEG, SEG), :] = x
            lhs_f[pl.ds(n * SEG, SEG), :] = _layernorm(x).astype(BF16)

    def ffn_up(c):
        h = lhs_f[...]
        gate = _dot(h, wg_v[:, pl.ds(c * FC, FC)])
        up = _dot(h, wu_v[:, pl.ds(c * FC, FC)])
        return (_gelu(gate) * up).astype(BF16)

    def ffn_down(c, a, segs):
        y = _dot(a, wd_v[pl.ds(c * FC, FC), :])
        if c < n_fc - 1:
            acc_f[...] += y
        else:
            y = acc_f[...] + y
            for n, s in enumerate(segs):
                r = y[n * SEG:(n + 1) * SEG]
                res_v[slot(s)] = r
                o_v[seg_rows(s), :] = r.astype(BF16)

    def out_copy(s):
        return pltpu.make_async_copy(o_v.at[seg_rows(s)], out_hbm.at[seg_rows(s)], out_sem)

    def attention_input(n, x):
        lhs_a[pl.ds(n * (SEG + MM), SEG), :] = _layernorm(x).astype(BF16)

    def ffn_cuts(parts):
        width = DF // parts
        cuts = list(range(0, width, FC)) + [width]
        return [(width, lo, hi - lo) for lo, hi in zip(cuts, cuts[1:])]

    def ffn_piece(op, k, cut, act):
        width, lo, n = cut
        cols = pl.ds(pl.multiple_of(k * width + lo, 128), n)
        if op == "u":
            h = lhs_f[...]
            return (_gelu(_dot(h, wg_v[:, cols])) * _dot(h, wu_v[:, cols])).astype(BF16)
        acc_f[...] += _dot(act, wd_v[cols, :])

    def project_piece(g, o):
        acc_o[pl.ds(0, o.shape[0]), :] += _dot(
            o, wo_v[pl.ds(pl.multiple_of(g * GW, GW), GW), :])

    def ffn_output(segs):
        for n, s in enumerate(segs):
            r = acc_f[pl.ds(n * SEG, SEG), :]
            res_v[slot(s)] = r
            o_v[seg_rows(s), :] = r.astype(BF16)

    def single_attention(layer, s):
        attention_input(1, res_v[slot(s)])
        acc_o[pl.ds(0, MM), :] = jnp.zeros((MM, D), F32)
        acc_o[pl.ds(MM, SEG), :] = res_v[slot(s)]
        gs = n_grp // ATT_PARTS

        def part(k, c):
            p, ss, o = {}, {}, {}
            for op, n in _step_order(gs, 1):
                g = k * gs + n
                if op == "q":
                    p[n] = qkv(g, R1)
                elif op == "s":
                    ss[n] = scores(p[n])
                elif op == "a":
                    o[n] = attend(p[n], ss[n], fill_s.at[layer])
                elif op == "o":
                    project_piece(g, o[n])
            return c

        lax.fori_loop(0, ATT_PARTS, part, 0)
        res_v[slot(s)] = acc_o[pl.ds(MM, SEG), :]
        own = jnp.where(lax.broadcasted_iota(jnp.int32, (MM, D), 0) < M, 0, 1) == layer
        lhs_a[pl.ds(SEG, MM), :] = jnp.where(
            own, acc_o[pl.ds(0, MM), :], lhs_a[pl.ds(SEG, MM), :].astype(F32)).astype(BF16)

    def single_ffn(segs):
        ffn_input(segs)
        cuts = ffn_cuts(FFN_PARTS)

        def part(k, c):
            a = {0: ffn_piece("u", k, cuts[0], None)}
            for n, cut in enumerate(cuts):
                if n + 1 < len(cuts):
                    a[n + 1] = ffn_piece("u", k, cuts[n + 1], None)
                ffn_piece("d", k, cut, a[n])
            return c

        lax.fori_loop(0, FFN_PARTS, part, 0)
        ffn_output(segs)

    def step_segments(t):
        return (t, t - LAG), (t - 1, jnp.where(t == LAG, t - 2, t - LAG - 1))

    def next_attention_input(t):
        attention_input(0, load_segment(jnp.minimum(t + 1, n_seg - 1)))
        attention_input(1, res_v[slot(t + 1 - LAG)])

    def paired_step(t, carry):
        att, ffn = step_segments(t)
        p, ss, o, a = {}, {}, {}, {}
        for op, n in _step_order(n_grp, n_fc):
            if op == "q":
                p[n] = qkv(n, R2)
            elif op == "s":
                ss[n] = scores(p[n])
            elif op == "a":
                o[n] = attend(p[n], ss[n], fill_v)
            elif op == "o":
                mem = project(n, o[n], att)
                if n == n_grp - 1:
                    lhs_a[pl.ds(SEG, MM), :] = mem.astype(BF16)
            elif op == "i":
                ffn_input(ffn)
            elif op == "u":
                a[n] = ffn_up(n)
            elif op == "d":
                ffn_down(n, a[n], ffn)
            else:
                next_attention_input(t)
        out_copy(t - LAG - 1).start()
        return carry

    def precomputed_step(t, carry):
        att, ffn = step_segments(t)
        pre_rows = pl.ds(pl.multiple_of((t - LAG) * SEG, SEG), SEG)
        gs, cuts = n_grp // PRE_PARTS, ffn_cuts(PRE_PARTS)
        acc_o[pl.ds(0, SEG), :] = res_v[slot(att[0])]
        acc_o[pl.ds(SEG, MM), :] = jnp.zeros((MM, D), F32)
        acc_o[pl.ds(SEG + MM, SEG), :] = res_v[slot(att[1])]
        for n, s in enumerate(ffn):
            acc_f[pl.ds(n * SEG, SEG), :] = res_v[slot(s)]

        def part(k, c):
            p, ss, o, a = {}, {}, {}, {}
            for op, n in _step_order(gs, len(cuts)):
                g = k * gs + n
                if op == "q":
                    p[n] = jnp.concatenate(
                        [jnp.concatenate([pre_v[m, g, pre_rows, :] for m in range(3)], axis=1),
                         qkv(g, R1)], axis=0)
                elif op == "s":
                    ss[n] = scores(p[n])
                elif op == "a":
                    o[n] = attend(p[n], ss[n], fill_v)
                elif op == "o":
                    project_piece(g, o[n])
                elif op == "i":
                    for j, s in enumerate(ffn):
                        lhs_f[pl.ds(j * SEG, SEG), :] = _layernorm(res_v[slot(s)]).astype(BF16)
                elif op == "n":
                    lhs_next[pl.ds(0, SEG), :] = _layernorm(load_segment(t + 1)).astype(BF16)
                    lhs_next[pl.ds(SEG, SEG), :] = _layernorm(
                        res_v[slot(t + 1 - LAG)]).astype(BF16)
                else:
                    a[n] = ffn_piece(op, k, cuts[n], a.get(n))
            return c

        lax.fori_loop(0, PRE_PARTS, part, 0)
        lhs_a[pl.ds(0, SEG), :] = lhs_next[pl.ds(0, SEG), :]
        lhs_a[pl.ds(SEG, MM), :] = acc_o[pl.ds(SEG, MM), :].astype(BF16)
        lhs_a[pl.ds(SEG + MM, SEG), :] = lhs_next[pl.ds(SEG, SEG), :]
        res_v[slot(att[0])] = acc_o[pl.ds(0, SEG), :]
        res_v[slot(att[1])] = acc_o[pl.ds(SEG + MM, SEG), :]
        ffn_output(ffn)

        @pl.when(t > LAG)
        def _():
            out_copy(t - LAG - 1).start()

        return carry

    def single_op(phase, i):
        is_head = phase == 0
        j = i - 1
        tail_ffn = lax.rem(i, 3) == 0
        is_ffn = jnp.where(is_head, i == LAG, tail_ffn)
        first = n_seg - LAG + 2 * lax.div(jnp.maximum(j, 0), 3)

        @pl.when(jnp.logical_not(is_ffn))
        def _():
            single_attention(phase, jnp.where(is_head, i, first + lax.rem(j, 3)))

        @pl.when(is_ffn)
        def _():
            @pl.when(is_head)
            def _():
                for c in (wg_copy, wu_copy, wd_copy):
                    c.wait()
                x_rest.start()

            s0 = jnp.where(is_head, 0, jnp.where(i == 0, n_seg - 1, first))
            s1 = jnp.where(is_head, 1, jnp.where(i == 0, n_seg - LAG - 1, first + 1))
            single_ffn((s0, s1))

            @pl.when(jnp.logical_not(is_head))
            def _():
                out_copy(s1).start()

                @pl.when(i > 0)
                def _():
                    out_copy(s0).start()

    def phase_body(phase, carry):
        n_ops = jnp.where(phase == 0, LAG + 1, 1 + 3 * (LAG // 2))
        lax.fori_loop(0, n_ops, lambda i, c: (single_op(phase, i), c)[1], 0)

        @pl.when(phase == 0)
        def _():
            x_rest.wait()
            attention_input(1, res_v[slot(0)])
            lax.fori_loop(LAG, LAG + PRE, precomputed_step, 0)
            lax.fori_loop(LAG + PRE, n_seg, paired_step, 0)

        return carry

    lax.fori_loop(0, 2, phase_body, 0)
    pltpu.make_async_copy(o_v, out_hbm, out_sem).wait()


@functools.partial(jax.jit, static_argnames=("A_seg_len",))
def pallas_interleave_layers__memory_aug_recurrent_mem_tr__glu_gated_geglu__prompt_kernel(
    A_x, A_mem0, A_Wq, A_Wk, A_Wv, A_Wo, A_seg_len, B_x, B_w_gate, B_w_up, B_w_down,
):
    del B_x
    B, S, D = A_x.shape
    _, H, Dh = A_Wq.shape
    M = A_mem0.shape[1]
    SEG = int(A_seg_len)
    DF = B_w_gate.shape[1]
    assert B == 1 and S % SEG == 0 and Dh == 128 and 2 * (M + SEG) <= 128
    R = 2 * (M + SEG)
    hbm = pl.BlockSpec(memory_space=pl.ANY)
    out = pl.pallas_call(
        functools.partial(_kernel, S=S, D=D, H=H, Dh=Dh, M=M, SEG=SEG, DF=DF),
        out_shape=jax.ShapeDtypeStruct((S, D), A_x.dtype),
        in_specs=[hbm, pl.BlockSpec(memory_space=pltpu.VMEM)] + [hbm] * 7,
        out_specs=hbm,
        scratch_shapes=[
            pltpu.VMEM((S, D), BF16),
            pltpu.VMEM((S, D), BF16),
            pltpu.VMEM((6 * D, H // 2, Dh), BF16),
            pltpu.VMEM((3, H // HG, D // 2, HG * Dh), jnp.int32),
            pltpu.VMEM((H * Dh, D), BF16),
            pltpu.VMEM((D, DF), BF16),
            pltpu.VMEM((D, DF), BF16),
            pltpu.VMEM((DF, D), BF16),
            pltpu.VMEM((RING, SEG, D), F32),
            pltpu.VMEM((R, D), BF16),
            pltpu.VMEM((2 * SEG, D), BF16),
            pltpu.VMEM((R, D), F32),
            pltpu.VMEM((2 * SEG, D), BF16),
            pltpu.VMEM((2 * SEG, D), F32),
            pltpu.VMEM((R, 128), F32),
            pltpu.VMEM((2, R - SEG, 128), F32),
            pltpu.VMEM((PRE * SEG, D), BF16),
            pltpu.VMEM((3, H // HG, PRE * SEG, HG * Dh), BF16),
            pltpu.SemaphoreType.DMA((8 * (D // RB),)),
            pltpu.SemaphoreType.DMA((5,)),
            pltpu.SemaphoreType.DMA(()),
        ],
        compiler_params=pltpu.CompilerParams(vmem_limit_bytes=120 * 2**20),
    )(A_x.reshape(S, D), A_mem0.reshape(M, D),
      A_Wq, A_Wk, A_Wv,
      A_Wo.reshape(H * Dh, D), B_w_gate, B_w_up, B_w_down)
    return out.reshape(B, S, D)
```

```python
import functools
import math

import jax
import jax.numpy as jnp
import numpy as np
from jax import lax
from jax.experimental import pallas as pl
from jax.experimental.pallas import tpu as pltpu

F32 = jnp.float32
BF16 = jnp.bfloat16

HG = 2
FC = 512
LAG = 4
WINDOW = 6
PRE = 7
PRE_PARTS = 2
ATT_PARTS = 2
FFN_PARTS = 2
RING = 8
RB = 256
PRE_ROWS = 112
ORDER = "usdqao"
FFN_START = 24


def _step_order(n_grp, n_fc):
    at = [(c * (n_grp - 1)) // n_fc for c in range(n_fc)]
    order = [("q", 0), ("i", 0), ("q", 1), ("s", 0)]
    for g in range(n_grp):
        items = {
            "q": [("q", g + 2)] * (g + 2 < n_grp) + [("n", 0)] * (g + 2 == n_grp),
            "s": [("s", g + 1)] * (g + 1 < n_grp),
            "u": [("u", c) for c in range(n_fc) if at[c] == g],
            "d": [("d", c) for c in range(n_fc - 1) if at[c] + 1 == g],
            "a": [("a", g)],
            "o": [("o", g - 1)] * (g >= 1),
        }
        for kind in ORDER:
            order += items[kind]
    return order + [("o", n_grp - 1), ("d", n_fc - 1)]


def _layernorm(x):
    m = jnp.mean(x, axis=-1, keepdims=True)
    c = x - m
    v = jnp.mean(c * c, axis=-1, keepdims=True)
    return c * lax.rsqrt(v + 1e-5)


def _gelu(x):
    c0 = math.sqrt(2.0 / math.pi)
    inner = x * (c0 + (c0 * 0.044715) * (x * x))
    return (0.5 * x) * (1.0 + jnp.tanh(inner))


def _dot(a, b):
    return jnp.dot(a, b, preferred_element_type=F32)


def _kernel(x_hbm, mem0_ref, wq_hbm, wk_hbm, wv_hbm, wo_hbm, wg_hbm, wu_hbm, wd_hbm,
            out_hbm,
            x_v, o_v, raw_v, wqkv_v, wo_v, wg_v, wu_v, wd_v,
            res_v, lhs_a, lhs_next, acc_o, lhs_f, acc_f, fill_v, fill_s, pre_in, pre_v,
            chunk_sem, w_sem, out_sem,
            *, S, D, H, Dh, M, SEG, DF):
    n_seg = S // SEG
    MM = 2 * M
    R2 = MM + 2 * SEG
    R1 = MM + SEG
    n_grp = H // HG
    n_fc = DF // FC
    GW = HG * Dh
    scale = Dh ** -0.5
    exp_c = scale * math.log2(math.e)

    n_rb = D // RB
    n_raw = 6 * n_rb
    n_chunk = 8 * n_rb
    HH = H // 2

    def raw_copy(w_hbm, i):
        unit, r = lax.div(i, n_rb), lax.rem(i, n_rb)
        heads = pl.ds(pl.multiple_of(lax.div(unit, 3) * HH, HH), HH)
        return pltpu.make_async_copy(
            w_hbm.at[pl.ds(pl.multiple_of(r * RB, RB), RB), heads],
            raw_v.at[pl.ds(pl.multiple_of(i * RB, RB), RB)], chunk_sem.at[i])

    def wo_copy(i):
        n = H * Dh // (2 * n_rb)
        rows = pl.ds(pl.multiple_of((i - n_raw) * n, n), n)
        return pltpu.make_async_copy(wo_hbm.at[rows], wo_v.at[rows], chunk_sem.at[i])

    def start_chunk(i, carry=None):
        for m, w_hbm in enumerate((wq_hbm, wk_hbm, wv_hbm)):
            @pl.when(jnp.logical_and(i < n_raw, lax.rem(lax.div(i, n_rb), 3) == m))
            def _():
                raw_copy(w_hbm, i).start()

        @pl.when(i >= n_raw)
        def _():
            wo_copy(i).start()

        return carry

    head_rows = (LAG + PRE + 1) * SEG
    x_head, wg_copy, wu_copy, wd_copy, x_rest = [
        pltpu.make_async_copy(s, d, w_sem.at[i]) for i, (s, d) in enumerate((
            (x_hbm.at[pl.ds(0, head_rows)], x_v.at[pl.ds(0, head_rows)]),
            (wg_hbm, wg_v), (wu_hbm, wu_v), (wd_hbm, wd_v),
            (x_hbm.at[pl.ds(head_rows, S - head_rows)],
             x_v.at[pl.ds(head_rows, S - head_rows)])))]
    x_head.start()
    lax.fori_loop(0, WINDOW, start_chunk, None)

    def make_fill(rows, mem_lo, layer_of):
        row = lax.broadcasted_iota(jnp.int32, (rows, 128), 0)
        col = lax.broadcasted_iota(jnp.int32, (rows, 128), 1)

        def is_mem(i):
            return (i >= mem_lo) & (i < mem_lo + MM)

        keep = is_mem(row) | is_mem(col) | (row >= col)
        return jnp.where(layer_of(row) == layer_of(col),
                         jnp.where(keep, 0.0, -1e9 / scale), -jnp.inf).astype(F32)

    fill_v[...] = make_fill(
        R2, SEG, lambda i: jnp.where(i < SEG + M, 0, jnp.where(i < R2, 1, 2)))
    for layer in range(2):
        fill_s[layer] = make_fill(R1, 0, lambda i: jnp.where(
            i < M, 0, jnp.where(i < MM, 1, jnp.where(i < R1, layer, 2))))

    grp_half = n_grp // 2

    def relayout(i, ts):
        unit, r = lax.div(i, n_rb), lax.rem(i, n_rb)
        half, m = lax.div(unit, 3), lax.rem(unit, 3)
        for t in ts:
            x = raw_v[pl.ds(pl.multiple_of(i * RB + t * 16, 16), 16)].reshape(16 * HH, Dh)
            x = pltpu.bitcast(x, jnp.int32).reshape(8, 2, HH // 2, Dh)
            ev, od = x[:, 0], x[:, 1]
            lo = jnp.swapaxes((ev & 0xFFFF) | (od << 16), 0, 1)
            hi = jnp.swapaxes(lax.shift_right_logical(ev, 16) | (od & -65536), 0, 1)
            rows = pl.ds(pl.multiple_of(r * (RB // 2) + t * 8, 8), 8)
            for j in range(HH // 2):
                g, c = divmod(2 * j, HG)
                wqkv_v[m, half * grp_half + g, rows, pl.ds(c * Dh, Dh)] = lo[j]
                wqkv_v[m, half * grp_half + g, rows, pl.ds((c + 1) * Dh, Dh)] = hi[j]

    pieces = [(j, lo) for j in range(grp_half // n_rb) for lo in range(0, PRE * SEG, PRE_ROWS)]

    def precompute(i, j, lo):
        unit, r = lax.div(i, n_rb), lax.rem(i, n_rb)
        half, m = lax.div(unit, 3), lax.rem(unit, 3)
        g = half * grp_half + r * (grp_half // n_rb) + j
        rows = pl.ds(lo, min(PRE_ROWS, PRE * SEG - lo))
        pre_v[m, g, rows, :] = _dot(
            pre_in[rows, :], pltpu.bitcast(wqkv_v[m, g], BF16)).astype(BF16)

    x_head.wait()
    for s in range(LAG, LAG + PRE):
        x0 = x_v[pl.ds(s * SEG, SEG), :].astype(F32)
        pre_in[pl.ds((s - LAG) * SEG, SEG), :] = _layernorm(x0).astype(BF16)

    def load_body(i, carry):
        @pl.when(i < n_raw)
        def _():
            raw_copy(wq_hbm, i).wait()

        @pl.when(i >= n_raw)
        def _():
            wo_copy(i).wait()

        def started(n):
            return jnp.minimum(WINDOW + n + lax.div(jnp.maximum(n - n_rb, 0), 3), n_chunk)

        lax.fori_loop(started(i), started(i + 1), start_chunk, None)

        @pl.when(i == FFN_START)
        def _():
            wg_copy.start()

        @pl.when(i < n_rb)
        def _():
            relayout(i, range(RB // 16))

        @pl.when(jnp.logical_and(i >= n_rb, i < n_raw))
        def _():
            per = RB // 16 // len(pieces)
            for n, piece in enumerate(pieces):
                precompute(i - n_rb, *piece)
                relayout(i, range(n * per, (n + 1) * per))

        @pl.when(jnp.logical_and(i >= n_raw, i < n_raw + n_rb))
        def _():
            for piece in pieces:
                precompute(i - n_rb, *piece)

        return carry

    lax.fori_loop(0, n_chunk, load_body, 0)
    wu_copy.start()
    wd_copy.start()

    def seg_rows(s):
        return pl.ds(pl.multiple_of(s * SEG, SEG), SEG)

    def slot(s):
        return s & (RING - 1)

    def load_segment(s):
        x0 = x_v[seg_rows(s), :].astype(F32)
        res_v[slot(s)] = x0
        return x0

    mem0 = mem0_ref[...].astype(F32)
    lhs_a[pl.ds(SEG, MM), :] = jnp.concatenate([mem0, mem0], axis=0).astype(BF16)
    for s in range(LAG + 1):
        load_segment(s)

    def qkv(g, rows):
        h = lhs_a[pl.ds(R2 - rows, rows), :]
        return jnp.concatenate(
            [_dot(h, pltpu.bitcast(wqkv_v[m, g], BF16)).astype(BF16) for m in range(3)],
            axis=1)

    def padded(a):
        return jnp.concatenate([a, jnp.zeros((128 - a.shape[0], Dh), BF16)], axis=0)

    def scores(p):
        return [lax.dot_general(p[:, i * Dh:(i + 1) * Dh],
                                padded(p[:, GW + i * Dh:GW + (i + 1) * Dh]),
                                (((1,), (1,)), ((), ())), preferred_element_type=F32)
                for i in range(HG)]

    def attend(p, ss, fill_ref):
        out = []
        for i in range(HG):
            fill = fill_ref[...]
            s = jnp.where(fill == 0.0, ss[i], fill)
            e = jnp.exp2((s - jnp.max(s, axis=-1, keepdims=True)) * exp_c)
            inv = 1.0 / jnp.sum(e, axis=-1, keepdims=True)
            v = padded(p[:, 2 * GW + i * Dh:2 * GW + (i + 1) * Dh])
            out.append((_dot(e.astype(BF16), v) * inv).astype(BF16))
        return jnp.concatenate(out, axis=1)

    def project(g, o, segs):
        rows = o.shape[0]
        y = _dot(o, wo_v[pl.ds(g * GW, GW), :])
        blocks = (0, SEG + MM) if len(segs) == 2 else (MM,)
        mem_lo = rows - R1
        if g == 0:
            acc_o[pl.ds(mem_lo, MM), :] = y[mem_lo:mem_lo + MM]
            for lo, s in zip(blocks, segs):
                acc_o[pl.ds(lo, SEG), :] = res_v[slot(s)] + y[lo:lo + SEG]
        elif g < n_grp - 1:
            acc_o[pl.ds(0, rows), :] += y
        else:
            y = acc_o[pl.ds(0, rows), :] + y
            for lo, s in zip(blocks, segs):
                res_v[slot(s)] = y[lo:lo + SEG]
            return y[mem_lo:mem_lo + MM]

    def ffn_input(segs):
        for n, s in enumerate(segs):
            x = res_v[slot(s)]
            acc_f[pl.ds(n * SEG, SEG), :] = x
            lhs_f[pl.ds(n * SEG, SEG), :] = _layernorm(x).astype(BF16)

    def ffn_up(c):
        h = lhs_f[...]
        gate = _dot(h, wg_v[:, pl.ds(c * FC, FC)])
        up = _dot(h, wu_v[:, pl.ds(c * FC, FC)])
        return (_gelu(gate) * up).astype(BF16)

    def ffn_down(c, a, segs):
        y = _dot(a, wd_v[pl.ds(c * FC, FC), :])
        if c < n_fc - 1:
            acc_f[...] += y
        else:
            y = acc_f[...] + y
            for n, s in enumerate(segs):
                r = y[n * SEG:(n + 1) * SEG]
                res_v[slot(s)] = r
                o_v[seg_rows(s), :] = r.astype(BF16)

    def out_copy(s):
        return pltpu.make_async_copy(o_v.at[seg_rows(s)], out_hbm.at[seg_rows(s)], out_sem)

    def attention_input(n, x):
        lhs_a[pl.ds(n * (SEG + MM), SEG), :] = _layernorm(x).astype(BF16)

    def ffn_cuts(parts):
        width = DF // parts
        cuts = list(range(0, width, FC)) + [width]
        return [(width, lo, hi - lo) for lo, hi in zip(cuts, cuts[1:])]

    def ffn_piece(op, k, cut, act):
        width, lo, n = cut
        cols = pl.ds(pl.multiple_of(k * width + lo, 128), n)
        if op == "u":
            h = lhs_f[...]
            return (_gelu(_dot(h, wg_v[:, cols])) * _dot(h, wu_v[:, cols])).astype(BF16)
        acc_f[...] += _dot(act, wd_v[cols, :])

    def project_piece(g, o):
        acc_o[pl.ds(0, o.shape[0]), :] += _dot(
            o, wo_v[pl.ds(pl.multiple_of(g * GW, GW), GW), :])

    def ffn_output(segs):
        for n, s in enumerate(segs):
            r = acc_f[pl.ds(n * SEG, SEG), :]
            res_v[slot(s)] = r
            o_v[seg_rows(s), :] = r.astype(BF16)

    def single_attention(layer, s):
        attention_input(1, res_v[slot(s)])
        acc_o[pl.ds(0, MM), :] = jnp.zeros((MM, D), F32)
        acc_o[pl.ds(MM, SEG), :] = res_v[slot(s)]
        gs = n_grp // ATT_PARTS

        def part(k, c):
            p, ss, o = {}, {}, {}
            for op, n in _step_order(gs, 1):
                g = k * gs + n
                if op == "q":
                    p[n] = qkv(g, R1)
                elif op == "s":
                    ss[n] = scores(p[n])
                elif op == "a":
                    o[n] = attend(p[n], ss[n], fill_s.at[layer])
                elif op == "o":
                    project_piece(g, o[n])
            return c

        lax.fori_loop(0, ATT_PARTS, part, 0)
        res_v[slot(s)] = acc_o[pl.ds(MM, SEG), :]
        own = jnp.where(lax.broadcasted_iota(jnp.int32, (MM, D), 0) < M, 0, 1) == layer
        lhs_a[pl.ds(SEG, MM), :] = jnp.where(
            own, acc_o[pl.ds(0, MM), :], lhs_a[pl.ds(SEG, MM), :].astype(F32)).astype(BF16)

    def single_ffn(segs):
        ffn_input(segs)
        cuts = ffn_cuts(FFN_PARTS)

        def part(k, c):
            a = {0: ffn_piece("u", k, cuts[0], None)}
            for n, cut in enumerate(cuts):
                if n + 1 < len(cuts):
                    a[n + 1] = ffn_piece("u", k, cuts[n + 1], None)
                ffn_piece("d", k, cut, a[n])
            return c

        lax.fori_loop(0, FFN_PARTS, part, 0)
        ffn_output(segs)

    def step_segments(t):
        return (t, t - LAG), (t - 1, jnp.where(t == LAG, t - 2, t - LAG - 1))

    def next_attention_input(t):
        attention_input(0, load_segment(jnp.minimum(t + 1, n_seg - 1)))
        attention_input(1, res_v[slot(t + 1 - LAG)])

    def paired_step(t, carry):
        att, ffn = step_segments(t)
        p, ss, o, a = {}, {}, {}, {}
        for op, n in _step_order(n_grp, n_fc):
            if op == "q":
                p[n] = qkv(n, R2)
            elif op == "s":
                ss[n] = scores(p[n])
            elif op == "a":
                o[n] = attend(p[n], ss[n], fill_v)
            elif op == "o":
                mem = project(n, o[n], att)
                if n == n_grp - 1:
                    lhs_a[pl.ds(SEG, MM), :] = mem.astype(BF16)
            elif op == "i":
                ffn_input(ffn)
            elif op == "u":
                a[n] = ffn_up(n)
            elif op == "d":
                ffn_down(n, a[n], ffn)
            else:
                next_attention_input(t)
        out_copy(t - LAG - 1).start()
        return carry

    def precomputed_step(t, carry):
        att, ffn = step_segments(t)
        pre_rows = pl.ds(pl.multiple_of((t - LAG) * SEG, SEG), SEG)
        gs, cuts = n_grp // PRE_PARTS, ffn_cuts(PRE_PARTS)
        acc_o[pl.ds(0, SEG), :] = res_v[slot(att[0])]
        acc_o[pl.ds(SEG, MM), :] = jnp.zeros((MM, D), F32)
        acc_o[pl.ds(SEG + MM, SEG), :] = res_v[slot(att[1])]
        for n, s in enumerate(ffn):
            acc_f[pl.ds(n * SEG, SEG), :] = res_v[slot(s)]

        def part(k, c):
            p, ss, o, a = {}, {}, {}, {}
            for op, n in _step_order(gs, len(cuts)):
                g = k * gs + n
                if op == "q":
                    p[n] = jnp.concatenate(
                        [jnp.concatenate([pre_v[m, g, pre_rows, :] for m in range(3)], axis=1),
                         qkv(g, R1)], axis=0)
                elif op == "s":
                    ss[n] = scores(p[n])
                elif op == "a":
                    o[n] = attend(p[n], ss[n], fill_v)
                elif op == "o":
                    project_piece(g, o[n])
                elif op == "i":
                    for j, s in enumerate(ffn):
                        lhs_f[pl.ds(j * SEG, SEG), :] = _layernorm(res_v[slot(s)]).astype(BF16)
                elif op == "n":
                    lhs_next[pl.ds(0, SEG), :] = _layernorm(load_segment(t + 1)).astype(BF16)
                    lhs_next[pl.ds(SEG, SEG), :] = _layernorm(
                        res_v[slot(t + 1 - LAG)]).astype(BF16)
                else:
                    a[n] = ffn_piece(op, k, cuts[n], a.get(n))
            return c

        lax.fori_loop(0, PRE_PARTS, part, 0)
        lhs_a[pl.ds(0, SEG), :] = lhs_next[pl.ds(0, SEG), :]
        lhs_a[pl.ds(SEG, MM), :] = acc_o[pl.ds(SEG, MM), :].astype(BF16)
        lhs_a[pl.ds(SEG + MM, SEG), :] = lhs_next[pl.ds(SEG, SEG), :]
        res_v[slot(att[0])] = acc_o[pl.ds(0, SEG), :]
        res_v[slot(att[1])] = acc_o[pl.ds(SEG + MM, SEG), :]
        ffn_output(ffn)

        @pl.when(t > LAG)
        def _():
            out_copy(t - LAG - 1).start()

        return carry

    def single_op(phase, i):
        is_head = phase == 0
        j = i - 1
        tail_ffn = lax.rem(i, 3) == 0
        is_ffn = jnp.where(is_head, i == LAG, tail_ffn)
        first = n_seg - LAG + 2 * lax.div(jnp.maximum(j, 0), 3)

        @pl.when(jnp.logical_not(is_ffn))
        def _():
            single_attention(phase, jnp.where(is_head, i, first + lax.rem(j, 3)))

        @pl.when(is_ffn)
        def _():
            @pl.when(is_head)
            def _():
                for c in (wg_copy, wu_copy, wd_copy):
                    c.wait()
                x_rest.start()

            s0 = jnp.where(is_head, 0, jnp.where(i == 0, n_seg - 1, first))
            s1 = jnp.where(is_head, 1, jnp.where(i == 0, n_seg - LAG - 1, first + 1))
            single_ffn((s0, s1))

            @pl.when(jnp.logical_not(is_head))
            def _():
                out_copy(s1).start()

                @pl.when(i > 0)
                def _():
                    out_copy(s0).start()

    def phase_body(phase, carry):
        n_ops = jnp.where(phase == 0, LAG + 1, 1 + 3 * (LAG // 2))
        lax.fori_loop(0, n_ops, lambda i, c: (single_op(phase, i), c)[1], 0)

        @pl.when(phase == 0)
        def _():
            x_rest.wait()
            attention_input(1, res_v[slot(0)])
            lax.fori_loop(LAG, LAG + PRE, precomputed_step, 0)
            lax.fori_loop(LAG + PRE, n_seg, paired_step, 0)

        return carry

    lax.fori_loop(0, 2, phase_body, 0)
    pltpu.make_async_copy(o_v, out_hbm, out_sem).wait()


@functools.partial(jax.jit, static_argnames=("A_seg_len",))
def pallas_interleave_layers__memory_aug_recurrent_mem_tr__glu_gated_geglu__prompt_kernel(
    A_x, A_mem0, A_Wq, A_Wk, A_Wv, A_Wo, A_seg_len, B_x, B_w_gate, B_w_up, B_w_down,
):
    del B_x
    B, S, D = A_x.shape
    _, H, Dh = A_Wq.shape
    M = A_mem0.shape[1]
    SEG = int(A_seg_len)
    DF = B_w_gate.shape[1]
    assert B == 1 and S % SEG == 0 and Dh == 128 and 2 * (M + SEG) <= 128
    R = 2 * (M + SEG)
    hbm = pl.BlockSpec(memory_space=pl.ANY)
    out = pl.pallas_call(
        functools.partial(_kernel, S=S, D=D, H=H, Dh=Dh, M=M, SEG=SEG, DF=DF),
        out_shape=jax.ShapeDtypeStruct((S, D), A_x.dtype),
        in_specs=[hbm, pl.BlockSpec(memory_space=pltpu.VMEM)] + [hbm] * 7,
        out_specs=hbm,
        scratch_shapes=[
            pltpu.VMEM((S, D), BF16),
            pltpu.VMEM((S, D), BF16),
            pltpu.VMEM((6 * D, H // 2, Dh), BF16),
            pltpu.VMEM((3, H // HG, D // 2, HG * Dh), jnp.int32),
            pltpu.VMEM((H * Dh, D), BF16),
            pltpu.VMEM((D, DF), BF16),
            pltpu.VMEM((D, DF), BF16),
            pltpu.VMEM((DF, D), BF16),
            pltpu.VMEM((RING, SEG, D), F32),
            pltpu.VMEM((R, D), BF16),
            pltpu.VMEM((2 * SEG, D), BF16),
            pltpu.VMEM((R, D), F32),
            pltpu.VMEM((2 * SEG, D), BF16),
            pltpu.VMEM((2 * SEG, D), F32),
            pltpu.VMEM((R, 128), F32),
            pltpu.VMEM((2, R - SEG, 128), F32),
            pltpu.VMEM((PRE * SEG, D), BF16),
            pltpu.VMEM((3, H // HG, PRE * SEG, HG * Dh), BF16),
            pltpu.SemaphoreType.DMA((8 * (D // RB),)),
            pltpu.SemaphoreType.DMA((5,)),
            pltpu.SemaphoreType.DMA(()),
        ],
        compiler_params=pltpu.CompilerParams(vmem_limit_bytes=120 * 2**20),
    )(A_x.reshape(S, D), A_mem0.reshape(M, D),
      A_Wq, A_Wk, A_Wv,
      A_Wo.reshape(H * Dh, D), B_w_gate, B_w_up, B_w_down)
    return out.reshape(B, S, D)
```

```python
import functools
import math

import jax
import jax.numpy as jnp
import numpy as np
from jax import lax
from jax.experimental import pallas as pl
from jax.experimental.pallas import tpu as pltpu

F32 = jnp.float32
BF16 = jnp.bfloat16

HG = 2
FC = 512
LAG = 4
WINDOW = 6
PRE = 7
PRE_PARTS = 2
ATT_PARTS = 2
FFN_PARTS = 2
RING = 8
RB = 256
PRE_ROWS = 112
ORDER = "usdqao"
FFN_START = 24


def _step_order(n_grp, n_fc):
    at = [(c * (n_grp - 1)) // n_fc for c in range(n_fc)]
    order = [("q", 0), ("i", 0), ("q", 1), ("s", 0)]
    for g in range(n_grp):
        items = {
            "q": [("q", g + 2)] * (g + 2 < n_grp) + [("n", 0)] * (g + 2 == n_grp),
            "s": [("s", g + 1)] * (g + 1 < n_grp),
            "u": [("u", c) for c in range(n_fc) if at[c] == g],
            "d": [("d", c) for c in range(n_fc - 1) if at[c] + 1 == g],
            "a": [("a", g)],
            "o": [("o", g - 1)] * (g >= 1),
        }
        for kind in ORDER:
            order += items[kind]
    return order + [("o", n_grp - 1), ("d", n_fc - 1)]


def _layernorm(x):
    m = jnp.mean(x, axis=-1, keepdims=True)
    c = x - m
    v = jnp.mean(c * c, axis=-1, keepdims=True)
    return c * lax.rsqrt(v + 1e-5)


def _gelu(x):
    c0 = math.sqrt(2.0 / math.pi)
    inner = x * (c0 + (c0 * 0.044715) * (x * x))
    return (0.5 * x) * (1.0 + jnp.tanh(inner))


def _dot(a, b):
    return jnp.dot(a, b, preferred_element_type=F32)


def _kernel(x_hbm, mem0_ref, wq_hbm, wk_hbm, wv_hbm, wo_hbm, wg_hbm, wu_hbm, wd_hbm,
            out_hbm,
            x_v, o_v, raw_v, wqkv_v, wo_v, wg_v, wu_v, wd_v,
            res_v, lhs_a, lhs_next, acc_o, lhs_f, acc_f, fill_v, fill_s, pre_in, pre_v,
            chunk_sem, w_sem, out_sem,
            *, S, D, H, Dh, M, SEG, DF):
    n_seg = S // SEG
    MM = 2 * M
    R2 = MM + 2 * SEG
    R1 = MM + SEG
    n_grp = H // HG
    n_fc = DF // FC
    GW = HG * Dh
    scale = Dh ** -0.5
    exp_c = scale * math.log2(math.e)

    n_rb = D // RB
    n_raw = 6 * n_rb
    n_chunk = 8 * n_rb
    HH = H // 2

    def raw_copy(w_hbm, i):
        unit, r = lax.div(i, n_rb), lax.rem(i, n_rb)
        heads = pl.ds(pl.multiple_of(lax.div(unit, 3) * HH, HH), HH)
        return pltpu.make_async_copy(
            w_hbm.at[pl.ds(pl.multiple_of(r * RB, RB), RB), heads],
            raw_v.at[pl.ds(pl.multiple_of(i * RB, RB), RB)], chunk_sem.at[i])

    def wo_copy(i):
        n = H * Dh // (2 * n_rb)
        rows = pl.ds(pl.multiple_of((i - n_raw) * n, n), n)
        return pltpu.make_async_copy(wo_hbm.at[rows], wo_v.at[rows], chunk_sem.at[i])

    def chunk_op(op, i, carry=None):
        for m, w_hbm in enumerate((wq_hbm, wk_hbm, wv_hbm)):
            @pl.when(jnp.logical_and(i < n_raw, lax.rem(lax.div(i, n_rb), 3) == m))
            def _():
                op(raw_copy(w_hbm, i))

        @pl.when(i >= n_raw)
        def _():
            op(wo_copy(i))

        return carry

    start_chunk = functools.partial(chunk_op, lambda copy: copy.start())
    wait_chunk = functools.partial(chunk_op, lambda copy: copy.wait())

    head_rows = (LAG + PRE + 1) * SEG
    x_head, wg_copy, wu_copy, wd_copy, x_rest = [
        pltpu.make_async_copy(s, d, w_sem.at[i]) for i, (s, d) in enumerate((
            (x_hbm.at[pl.ds(0, head_rows)], x_v.at[pl.ds(0, head_rows)]),
            (wg_hbm, wg_v), (wu_hbm, wu_v), (wd_hbm, wd_v),
            (x_hbm.at[pl.ds(head_rows, S - head_rows)],
             x_v.at[pl.ds(head_rows, S - head_rows)])))]
    x_head.start()
    lax.fori_loop(0, WINDOW, start_chunk, None)

    def make_fill(rows, mem_lo, layer_of):
        row = lax.broadcasted_iota(jnp.int32, (rows, 128), 0)
        col = lax.broadcasted_iota(jnp.int32, (rows, 128), 1)

        def is_mem(i):
            return (i >= mem_lo) & (i < mem_lo + MM)

        keep = is_mem(row) | is_mem(col) | (row >= col)
        return jnp.where(layer_of(row) == layer_of(col),
                         jnp.where(keep, 0.0, -1e9 / scale), -jnp.inf).astype(F32)

    fill_v[...] = make_fill(
        R2, SEG, lambda i: jnp.where(i < SEG + M, 0, jnp.where(i < R2, 1, 2)))
    for layer in range(2):
        fill_s[layer] = make_fill(R1, 0, lambda i: jnp.where(
            i < M, 0, jnp.where(i < MM, 1, jnp.where(i < R1, layer, 2))))

    grp_half = n_grp // 2

    def relayout(i, ts):
        unit, r = lax.div(i, n_rb), lax.rem(i, n_rb)
        half, m = lax.div(unit, 3), lax.rem(unit, 3)
        for t in ts:
            x = raw_v[pl.ds(pl.multiple_of(i * RB + t * 16, 16), 16)].reshape(16 * HH, Dh)
            x = pltpu.bitcast(x, jnp.int32).reshape(8, 2, HH // 2, Dh)
            ev, od = x[:, 0], x[:, 1]
            lo = jnp.swapaxes((ev & 0xFFFF) | (od << 16), 0, 1)
            hi = jnp.swapaxes(lax.shift_right_logical(ev, 16) | (od & -65536), 0, 1)
            rows = pl.ds(pl.multiple_of(r * (RB // 2) + t * 8, 8), 8)
            for j in range(HH // 2):
                g, c = divmod(2 * j, HG)
                wqkv_v[m, half * grp_half + g, rows, pl.ds(c * Dh, Dh)] = lo[j]
                wqkv_v[m, half * grp_half + g, rows, pl.ds((c + 1) * Dh, Dh)] = hi[j]

    pieces = [(j, lo) for j in range(grp_half // n_rb) for lo in range(0, PRE * SEG, PRE_ROWS)]

    def precompute(i, j, lo):
        unit, r = lax.div(i, n_rb), lax.rem(i, n_rb)
        half, m = lax.div(unit, 3), lax.rem(unit, 3)
        g = half * grp_half + r * (grp_half // n_rb) + j
        rows = pl.ds(lo, min(PRE_ROWS, PRE * SEG - lo))
        pre_v[m, g, rows, :] = _dot(
            pre_in[rows, :], pltpu.bitcast(wqkv_v[m, g], BF16)).astype(BF16)

    def seg_rows(s):
        return pl.ds(pl.multiple_of(s * SEG, SEG), SEG)

    def slot(s):
        return s & (RING - 1)

    def load_segment(s):
        x0 = x_v[seg_rows(s), :].astype(F32)
        res_v[slot(s)] = x0
        return x0

    def attention_input(n, x):
        lhs_a[pl.ds(n * (SEG + MM), SEG), :] = _layernorm(x).astype(BF16)

    x_head.wait()
    mem0 = mem0_ref[...].astype(F32)
    lhs_a[pl.ds(SEG, MM), :] = jnp.concatenate([mem0, mem0], axis=0).astype(BF16)
    attention_input(1, load_segment(0))
    for s in range(1, LAG + 1):
        load_segment(s)

    for s in range(LAG, LAG + PRE):
        x0 = x_v[pl.ds(s * SEG, SEG), :].astype(F32)
        pre_in[pl.ds((s - LAG) * SEG, SEG), :] = _layernorm(x0).astype(BF16)

    def load_body(i, carry):
        wait_chunk(i)

        def started(n):
            return jnp.minimum(WINDOW + n + lax.div(jnp.maximum(n - n_rb, 0), 3), n_chunk)

        lax.fori_loop(started(i), started(i + 1), start_chunk, None)

        @pl.when(i == FFN_START)
        def _():
            wg_copy.start()

        @pl.when(i < n_rb)
        def _():
            relayout(i, range(RB // 16))

        @pl.when(jnp.logical_and(i >= n_rb, i < n_raw))
        def _():
            per = RB // 16 // len(pieces)
            for n, piece in enumerate(pieces):
                precompute(i - n_rb, *piece)
                relayout(i, range(n * per, (n + 1) * per))

        @pl.when(jnp.logical_and(i >= n_raw, i < n_raw + n_rb))
        def _():
            for piece in pieces:
                precompute(i - n_rb, *piece)

        return carry

    lax.fori_loop(0, n_chunk, load_body, 0)
    wu_copy.start()
    wd_copy.start()

    def qkv(g, rows):
        h = lhs_a[pl.ds(R2 - rows, rows), :]
        return jnp.concatenate(
            [_dot(h, pltpu.bitcast(wqkv_v[m, g], BF16)).astype(BF16) for m in range(3)],
            axis=1)

    def padded(a):
        return jnp.concatenate([a, jnp.zeros((128 - a.shape[0], Dh), BF16)], axis=0)

    def scores(p):
        return [lax.dot_general(p[:, i * Dh:(i + 1) * Dh],
                                padded(p[:, GW + i * Dh:GW + (i + 1) * Dh]),
                                (((1,), (1,)), ((), ())), preferred_element_type=F32)
                for i in range(HG)]

    def attend(p, ss, fill_ref):
        out = []
        for i in range(HG):
            fill = fill_ref[...]
            s = jnp.where(fill == 0.0, ss[i], fill)
            e = jnp.exp2((s - jnp.max(s, axis=-1, keepdims=True)) * exp_c)
            inv = 1.0 / jnp.sum(e, axis=-1, keepdims=True)
            v = padded(p[:, 2 * GW + i * Dh:2 * GW + (i + 1) * Dh])
            out.append((_dot(e.astype(BF16), v) * inv).astype(BF16))
        return jnp.concatenate(out, axis=1)

    def project(g, o, segs):
        rows = o.shape[0]
        y = _dot(o, wo_v[pl.ds(g * GW, GW), :])
        blocks = (0, SEG + MM) if len(segs) == 2 else (MM,)
        mem_lo = rows - R1
        if g == 0:
            acc_o[pl.ds(mem_lo, MM), :] = y[mem_lo:mem_lo + MM]
            for lo, s in zip(blocks, segs):
                acc_o[pl.ds(lo, SEG), :] = res_v[slot(s)] + y[lo:lo + SEG]
        elif g < n_grp - 1:
            acc_o[pl.ds(0, rows), :] += y
        else:
            y = acc_o[pl.ds(0, rows), :] + y
            for lo, s in zip(blocks, segs):
                res_v[slot(s)] = y[lo:lo + SEG]
            return y[mem_lo:mem_lo + MM]

    def ffn_input(segs):
        for n, s in enumerate(segs):
            x = res_v[slot(s)]
            acc_f[pl.ds(n * SEG, SEG), :] = x
            lhs_f[pl.ds(n * SEG, SEG), :] = _layernorm(x).astype(BF16)

    def ffn_up(c):
        h = lhs_f[...]
        gate = _dot(h, wg_v[:, pl.ds(c * FC, FC)])
        up = _dot(h, wu_v[:, pl.ds(c * FC, FC)])
        return (_gelu(gate) * up).astype(BF16)

    def ffn_down(c, a, segs):
        y = _dot(a, wd_v[pl.ds(c * FC, FC), :])
        if c < n_fc - 1:
            acc_f[...] += y
        else:
            y = acc_f[...] + y
            for n, s in enumerate(segs):
                r = y[n * SEG:(n + 1) * SEG]
                res_v[slot(s)] = r
                o_v[seg_rows(s), :] = r.astype(BF16)

    def out_copy(s):
        return pltpu.make_async_copy(o_v.at[seg_rows(s)], out_hbm.at[seg_rows(s)], out_sem)

    def ffn_cuts(parts):
        width = DF // parts
        cuts = list(range(0, width, FC)) + [width]
        return [(width, lo, hi - lo) for lo, hi in zip(cuts, cuts[1:])]

    def ffn_piece(op, k, cut, act):
        width, lo, n = cut
        cols = pl.ds(pl.multiple_of(k * width + lo, 128), n)
        if op == "u":
            h = lhs_f[...]
            return (_gelu(_dot(h, wg_v[:, cols])) * _dot(h, wu_v[:, cols])).astype(BF16)
        acc_f[...] += _dot(act, wd_v[cols, :])

    def project_piece(g, o):
        acc_o[pl.ds(0, o.shape[0]), :] += _dot(
            o, wo_v[pl.ds(pl.multiple_of(g * GW, GW), GW), :])

    def ffn_output(segs):
        for n, s in enumerate(segs):
            r = acc_f[pl.ds(n * SEG, SEG), :]
            res_v[slot(s)] = r
            o_v[seg_rows(s), :] = r.astype(BF16)

    def single_attention(layer, s):
        acc_o[pl.ds(0, MM), :] = jnp.zeros((MM, D), F32)
        acc_o[pl.ds(MM, SEG), :] = res_v[slot(s)]
        gs = n_grp // ATT_PARTS

        def part(k, c):
            p, ss, o = {}, {}, {}
            for op, n in _step_order(gs, 1):
                g = k * gs + n
                if op == "q":
                    p[n] = qkv(g, R1)
                elif op == "i":
                    lhs_next[pl.ds(0, SEG), :] = _layernorm(res_v[slot(s + 1)]).astype(BF16)
                elif op == "s":
                    ss[n] = scores(p[n])
                elif op == "a":
                    o[n] = attend(p[n], ss[n], fill_s.at[layer])
                elif op == "o":
                    project_piece(g, o[n])
            return c

        lax.fori_loop(0, ATT_PARTS, part, 0)
        lhs_a[pl.ds(SEG + MM, SEG), :] = lhs_next[pl.ds(0, SEG), :]
        res_v[slot(s)] = acc_o[pl.ds(MM, SEG), :]
        own = jnp.where(lax.broadcasted_iota(jnp.int32, (MM, D), 0) < M, 0, 1) == layer
        lhs_a[pl.ds(SEG, MM), :] = jnp.where(
            own, acc_o[pl.ds(0, MM), :], lhs_a[pl.ds(SEG, MM), :].astype(F32)).astype(BF16)

    def single_ffn(segs):
        ffn_input(segs)
        cuts = ffn_cuts(FFN_PARTS)

        def part(k, c):
            a = {0: ffn_piece("u", k, cuts[0], None)}
            for n, cut in enumerate(cuts):
                if n + 1 < len(cuts):
                    a[n + 1] = ffn_piece("u", k, cuts[n + 1], None)
                ffn_piece("d", k, cut, a[n])
            return c

        lax.fori_loop(0, FFN_PARTS, part, 0)
        ffn_output(segs)

    def step_segments(t):
        return (t, t - LAG), (t - 1, jnp.where(t == LAG, t - 2, t - LAG - 1))

    def next_attention_input(t):
        attention_input(0, load_segment(jnp.minimum(t + 1, n_seg - 1)))
        attention_input(1, res_v[slot(t + 1 - LAG)])

    def paired_step(t, carry):
        att, ffn = step_segments(t)
        p, ss, o, a = {}, {}, {}, {}
        for op, n in _step_order(n_grp, n_fc):
            if op == "q":
                p[n] = qkv(n, R2)
            elif op == "s":
                ss[n] = scores(p[n])
            elif op == "a":
                o[n] = attend(p[n], ss[n], fill_v)
            elif op == "o":
                mem = project(n, o[n], att)
                if n == n_grp - 1:
                    lhs_a[pl.ds(SEG, MM), :] = mem.astype(BF16)
            elif op == "i":
                ffn_input(ffn)
            elif op == "u":
                a[n] = ffn_up(n)
            elif op == "d":
                ffn_down(n, a[n], ffn)
            else:
                next_attention_input(t)
        out_copy(t - LAG - 1).start()
        return carry

    def precomputed_step(t, carry):
        att, ffn = step_segments(t)
        pre_rows = pl.ds(pl.multiple_of((t - LAG) * SEG, SEG), SEG)
        gs, cuts = n_grp // PRE_PARTS, ffn_cuts(PRE_PARTS)
        acc_o[pl.ds(0, SEG), :] = res_v[slot(att[0])]
        acc_o[pl.ds(SEG, MM), :] = jnp.zeros((MM, D), F32)
        acc_o[pl.ds(SEG + MM, SEG), :] = res_v[slot(att[1])]
        for n, s in enumerate(ffn):
            acc_f[pl.ds(n * SEG, SEG), :] = res_v[slot(s)]

        def part(k, c):
            p, ss, o, a = {}, {}, {}, {}
            for op, n in _step_order(gs, len(cuts)):
                g = k * gs + n
                if op == "q":
                    p[n] = jnp.concatenate(
                        [jnp.concatenate([pre_v[m, g, pre_rows, :] for m in range(3)], axis=1),
                         qkv(g, R1)], axis=0)
                elif op == "s":
                    ss[n] = scores(p[n])
                elif op == "a":
                    o[n] = attend(p[n], ss[n], fill_v)
                elif op == "o":
                    project_piece(g, o[n])
                elif op == "i":
                    for j, s in enumerate(ffn):
                        lhs_f[pl.ds(j * SEG, SEG), :] = _layernorm(res_v[slot(s)]).astype(BF16)
                elif op == "n":
                    lhs_next[pl.ds(0, SEG), :] = _layernorm(load_segment(t + 1)).astype(BF16)
                    lhs_next[pl.ds(SEG, SEG), :] = _layernorm(
                        res_v[slot(t + 1 - LAG)]).astype(BF16)
                else:
                    a[n] = ffn_piece(op, k, cuts[n], a.get(n))
            return c

        lax.fori_loop(0, PRE_PARTS, part, 0)
        lhs_a[pl.ds(0, SEG), :] = lhs_next[pl.ds(0, SEG), :]
        lhs_a[pl.ds(SEG, MM), :] = acc_o[pl.ds(SEG, MM), :].astype(BF16)
        lhs_a[pl.ds(SEG + MM, SEG), :] = lhs_next[pl.ds(SEG, SEG), :]
        res_v[slot(att[0])] = acc_o[pl.ds(0, SEG), :]
        res_v[slot(att[1])] = acc_o[pl.ds(SEG + MM, SEG), :]
        ffn_output(ffn)

        @pl.when(t > LAG)
        def _():
            out_copy(t - LAG - 1).start()

        return carry

    def single_op(phase, i):
        is_head = phase == 0
        j = i - 1
        tail_ffn = lax.rem(i, 3) == 0
        is_ffn = jnp.where(is_head, i == LAG, tail_ffn)
        first = n_seg - LAG + 2 * lax.div(jnp.maximum(j, 0), 3)

        @pl.when(jnp.logical_not(is_ffn))
        def _():
            single_attention(phase, jnp.where(is_head, i, first + lax.rem(j, 3)))

        @pl.when(is_ffn)
        def _():
            @pl.when(is_head)
            def _():
                for c in (wg_copy, wu_copy, wd_copy):
                    c.wait()
                x_rest.start()

            s0 = jnp.where(is_head, 0, jnp.where(i == 0, n_seg - 1, first))
            s1 = jnp.where(is_head, 1, jnp.where(i == 0, n_seg - LAG - 1, first + 1))
            single_ffn((s0, s1))

            @pl.when(jnp.logical_not(is_head))
            def _():
                out_copy(s1).start()

                @pl.when(i > 0)
                def _():
                    out_copy(s0).start()

    def phase_body(phase, carry):
        n_ops = jnp.where(phase == 0, LAG + 1, 1 + 3 * (LAG // 2))
        lax.fori_loop(0, n_ops, lambda i, c: (single_op(phase, i), c)[1], 0)

        @pl.when(phase == 0)
        def _():
            x_rest.wait()
            attention_input(1, res_v[slot(0)])
            lax.fori_loop(LAG, LAG + PRE, precomputed_step, 0)
            lax.fori_loop(LAG + PRE, n_seg, paired_step, 0)

        return carry

    lax.fori_loop(0, 2, phase_body, 0)
    pltpu.make_async_copy(o_v, out_hbm, out_sem).wait()


@functools.partial(jax.jit, static_argnames=("A_seg_len",))
def pallas_interleave_layers__memory_aug_recurrent_mem_tr__glu_gated_geglu__prompt_kernel(
    A_x, A_mem0, A_Wq, A_Wk, A_Wv, A_Wo, A_seg_len, B_x, B_w_gate, B_w_up, B_w_down,
):
    del B_x
    B, S, D = A_x.shape
    _, H, Dh = A_Wq.shape
    M = A_mem0.shape[1]
    SEG = int(A_seg_len)
    DF = B_w_gate.shape[1]
    assert B == 1 and S % SEG == 0 and Dh == 128 and 2 * (M + SEG) <= 128
    R = 2 * (M + SEG)
    hbm = pl.BlockSpec(memory_space=pl.ANY)
    out = pl.pallas_call(
        functools.partial(_kernel, S=S, D=D, H=H, Dh=Dh, M=M, SEG=SEG, DF=DF),
        out_shape=jax.ShapeDtypeStruct((S, D), A_x.dtype),
        in_specs=[hbm, pl.BlockSpec(memory_space=pltpu.VMEM)] + [hbm] * 7,
        out_specs=hbm,
        scratch_shapes=[
            pltpu.VMEM((S, D), BF16),
            pltpu.VMEM((S, D), BF16),
            pltpu.VMEM((6 * D, H // 2, Dh), BF16),
            pltpu.VMEM((3, H // HG, D // 2, HG * Dh), jnp.int32),
            pltpu.VMEM((H * Dh, D), BF16),
            pltpu.VMEM((D, DF), BF16),
            pltpu.VMEM((D, DF), BF16),
            pltpu.VMEM((DF, D), BF16),
            pltpu.VMEM((RING, SEG, D), F32),
            pltpu.VMEM((R, D), BF16),
            pltpu.VMEM((2 * SEG, D), BF16),
            pltpu.VMEM((R, D), F32),
            pltpu.VMEM((2 * SEG, D), BF16),
            pltpu.VMEM((2 * SEG, D), F32),
            pltpu.VMEM((R, 128), F32),
            pltpu.VMEM((2, R - SEG, 128), F32),
            pltpu.VMEM((PRE * SEG, D), BF16),
            pltpu.VMEM((3, H // HG, PRE * SEG, HG * Dh), BF16),
            pltpu.SemaphoreType.DMA((8 * (D // RB),)),
            pltpu.SemaphoreType.DMA((5,)),
            pltpu.SemaphoreType.DMA(()),
        ],
        compiler_params=pltpu.CompilerParams(vmem_limit_bytes=120 * 2**20),
    )(A_x.reshape(S, D), A_mem0.reshape(M, D),
      A_Wq, A_Wk, A_Wv,
      A_Wo.reshape(H * Dh, D), B_w_gate, B_w_up, B_w_down)
    return out.reshape(B, S, D)
```

```python
import functools
import math

import jax
import jax.numpy as jnp
import numpy as np
from jax import lax
from jax.experimental import pallas as pl
from jax.experimental.pallas import tpu as pltpu

F32 = jnp.float32
BF16 = jnp.bfloat16

HG = 2
FC = 512
LAG = 4
WINDOW = 8
PRE = 7
PRE_PARTS = 2
ATT_PARTS = 2
FFN_PARTS = 2
RING = 8
RB = 256
PRE_ROWS = 112
CUTS = (0, 7, 12, 16, 16)
ORDER = "usdqao"
FFN_START = 27


def _step_order(n_grp, n_fc):
    at = [(c * (n_grp - 1)) // n_fc for c in range(n_fc)]
    order = [("q", 0), ("i", 0), ("q", 1), ("s", 0)]
    for g in range(n_grp):
        items = {
            "q": [("q", g + 2)] * (g + 2 < n_grp) + [("n", 0)] * (g + 2 == n_grp),
            "s": [("s", g + 1)] * (g + 1 < n_grp),
            "u": [("u", c) for c in range(n_fc) if at[c] == g],
            "d": [("d", c) for c in range(n_fc - 1) if at[c] + 1 == g],
            "a": [("a", g)],
            "o": [("o", g - 1)] * (g >= 1),
        }
        for kind in ORDER:
            order += items[kind]
    return order + [("o", n_grp - 1), ("d", n_fc - 1)]


def _layernorm(x):
    m = jnp.mean(x, axis=-1, keepdims=True)
    c = x - m
    v = jnp.mean(c * c, axis=-1, keepdims=True)
    return c * lax.rsqrt(v + 1e-5)


def _gelu(x):
    c0 = math.sqrt(2.0 / math.pi)
    inner = x * (c0 + (c0 * 0.044715) * (x * x))
    return (0.5 * x) * (1.0 + jnp.tanh(inner))


def _dot(a, b):
    return jnp.dot(a, b, preferred_element_type=F32)


def _kernel(x_hbm, mem0_ref, wq_hbm, wk_hbm, wv_hbm, wo_hbm, wg_hbm, wu_hbm, wd_hbm,
            out_hbm,
            x_v, o_v, raw_v, wqkv_v, wo_v, wg_v, wu_v, wd_v,
            res_v, lhs_a, lhs_next, acc_o, lhs_f, acc_f, fill_v, fill_s, pre_in, pre_v,
            chunk_sem, w_sem, out_sem,
            *, S, D, H, Dh, M, SEG, DF):
    n_seg = S // SEG
    MM = 2 * M
    R2 = MM + 2 * SEG
    R1 = MM + SEG
    n_grp = H // HG
    n_fc = DF // FC
    GW = HG * Dh
    scale = Dh ** -0.5
    exp_c = scale * math.log2(math.e)

    n_rb = D // RB
    n_raw = 6 * n_rb
    n_chunk = 8 * n_rb
    HH = H // 2

    def raw_copy(w_hbm, i):
        unit, r = lax.div(i, n_rb), lax.rem(i, n_rb)
        heads = pl.ds(pl.multiple_of(lax.div(unit, 3) * HH, HH), HH)
        return pltpu.make_async_copy(
            w_hbm.at[pl.ds(pl.multiple_of(r * RB, RB), RB), heads],
            raw_v.at[pl.ds(pl.multiple_of(i * RB, RB), RB)], chunk_sem.at[i])

    def wo_copy(i):
        n = H * Dh // (2 * n_rb)
        rows = pl.ds(pl.multiple_of((i - n_raw) * n, n), n)
        return pltpu.make_async_copy(wo_hbm.at[rows], wo_v.at[rows], chunk_sem.at[i])

    def start_chunk(i, carry):
        for m, w_hbm in enumerate((wq_hbm, wk_hbm, wv_hbm)):
            @pl.when(jnp.logical_and(i < n_raw, lax.rem(lax.div(i, n_rb), 3) == m))
            def _():
                raw_copy(w_hbm, i).start()

        @pl.when(i >= n_raw)
        def _():
            wo_copy(i).start()

        return carry

    def wait_raw(i):
        dst = raw_v.at[pl.ds(pl.multiple_of(i * RB, RB), RB)]
        pltpu.make_async_copy(dst, dst, chunk_sem.at[i]).wait()

    head_rows = (LAG + PRE + 1) * SEG
    x_head, wg_copy, wu_copy, wd_copy, x_rest = [
        pltpu.make_async_copy(s, d, w_sem.at[i]) for i, (s, d) in enumerate((
            (x_hbm.at[pl.ds(0, head_rows)], x_v.at[pl.ds(0, head_rows)]),
            (wg_hbm, wg_v), (wu_hbm, wu_v), (wd_hbm, wd_v),
            (x_hbm.at[pl.ds(head_rows, S - head_rows)],
             x_v.at[pl.ds(head_rows, S - head_rows)])))]
    x_head.start()
    lax.fori_loop(0, WINDOW, start_chunk, None)

    def make_fill(rows, mem_lo, layer_of):
        row = lax.broadcasted_iota(jnp.int32, (rows, 128), 0)
        col = lax.broadcasted_iota(jnp.int32, (rows, 128), 1)

        def is_mem(i):
            return (i >= mem_lo) & (i < mem_lo + MM)

        keep = is_mem(row) | is_mem(col) | (row >= col)
        return jnp.where(layer_of(row) == layer_of(col),
                         jnp.where(keep, 0.0, -1e9 / scale), -jnp.inf).astype(F32)

    fill_v[...] = make_fill(
        R2, SEG, lambda i: jnp.where(i < SEG + M, 0, jnp.where(i < R2, 1, 2)))
    for layer in range(2):
        fill_s[layer] = make_fill(R1, 0, lambda i: jnp.where(
            i < M, 0, jnp.where(i < MM, 1, jnp.where(i < R1, layer, 2))))

    grp_half = n_grp // 2

    def relayout(i, ts):
        unit, r = lax.div(i, n_rb), lax.rem(i, n_rb)
        half, m = lax.div(unit, 3), lax.rem(unit, 3)
        for t in ts:
            x = raw_v[pl.ds(pl.multiple_of(i * RB + t * 16, 16), 16)].reshape(16 * HH, Dh)
            x = pltpu.bitcast(x, jnp.int32).reshape(8, 2, HH // 2, Dh)
            ev, od = x[:, 0], x[:, 1]
            lo = jnp.swapaxes((ev & 0xFFFF) | (od << 16), 0, 1)
            hi = jnp.swapaxes(lax.shift_right_logical(ev, 16) | (od & -65536), 0, 1)
            rows = pl.ds(pl.multiple_of(r * (RB // 2) + t * 8, 8), 8)
            for j in range(HH // 2):
                g, c = divmod(2 * j, HG)
                wqkv_v[m, half * grp_half + g, rows, pl.ds(c * Dh, Dh)] = lo[j]
                wqkv_v[m, half * grp_half + g, rows, pl.ds((c + 1) * Dh, Dh)] = hi[j]

    pieces = [(j, lo) for j in range(grp_half // n_rb) for lo in range(0, PRE * SEG, PRE_ROWS)]

    def precompute(i, j, lo):
        unit, r = lax.div(i, n_rb), lax.rem(i, n_rb)
        half, m = lax.div(unit, 3), lax.rem(unit, 3)
        g = half * grp_half + r * (grp_half // n_rb) + j
        rows = pl.ds(lo, min(PRE_ROWS, PRE * SEG - lo))
        pre_v[m, g, rows, :] = _dot(
            pre_in[rows, :], pltpu.bitcast(wqkv_v[m, g], BF16)).astype(BF16)

    def seg_rows(s):
        return pl.ds(pl.multiple_of(s * SEG, SEG), SEG)

    def slot(s):
        return s & (RING - 1)

    def load_segment(s):
        x0 = x_v[seg_rows(s), :].astype(F32)
        res_v[slot(s)] = x0
        return x0

    def attention_input(n, x):
        lhs_a[pl.ds(n * (SEG + MM), SEG), :] = _layernorm(x).astype(BF16)

    x_head.wait()
    mem0 = mem0_ref[...].astype(F32)
    lhs_a[pl.ds(SEG, MM), :] = jnp.concatenate([mem0, mem0], axis=0).astype(BF16)
    attention_input(1, load_segment(0))
    for s in range(1, LAG + 1):
        load_segment(s)

    for s in range(LAG, LAG + PRE):
        x0 = x_v[pl.ds(s * SEG, SEG), :].astype(F32)
        pre_in[pl.ds((s - LAG) * SEG, SEG), :] = _layernorm(x0).astype(BF16)

    def started(n):
        return jnp.minimum(WINDOW + n + lax.div(jnp.maximum(n - n_rb, 0), 3), n_chunk)

    def load_body(i, carry):
        lax.fori_loop(started(i), started(i + 1), start_chunk, None)

        @pl.when(i == FFN_START)
        def _():
            wg_copy.start()

        @pl.when(i < n_rb)
        def _():
            wait_raw(i)
            relayout(i, range(RB // 16))

        @pl.when(jnp.logical_and(i >= n_rb, i < n_raw))
        def _():
            wait_raw(i)
            for piece, (lo, hi) in zip(pieces, zip(CUTS, CUTS[1:])):
                precompute(i - n_rb, *piece)
                relayout(i, range(lo, hi))

        @pl.when(i >= n_raw)
        def _():
            wo_copy(i).wait()
            for piece in pieces:
                precompute(i - n_rb, *piece)

        return carry

    lax.fori_loop(0, n_chunk - n_rb, load_body, 0)
    lax.fori_loop(started(n_chunk - n_rb), n_chunk, start_chunk, None)

    def finish_loads():
        for i in range(n_chunk - n_rb, n_chunk):
            wo_copy(i).wait()
        wu_copy.start()
        wd_copy.start()

    def qkv(g, rows):
        h = lhs_a[pl.ds(R2 - rows, rows), :]
        return jnp.concatenate(
            [_dot(h, pltpu.bitcast(wqkv_v[m, g], BF16)).astype(BF16) for m in range(3)],
            axis=1)

    def padded(a):
        return jnp.concatenate([a, jnp.zeros((128 - a.shape[0], Dh), BF16)], axis=0)

    def scores(p):
        return [lax.dot_general(p[:, i * Dh:(i + 1) * Dh],
                                padded(p[:, GW + i * Dh:GW + (i + 1) * Dh]),
                                (((1,), (1,)), ((), ())), preferred_element_type=F32)
                for i in range(HG)]

    def attend(p, ss, fill_ref):
        out = []
        for i in range(HG):
            fill = fill_ref[...]
            s = jnp.where(fill == 0.0, ss[i], fill)
            e = jnp.exp2((s - jnp.max(s, axis=-1, keepdims=True)) * exp_c)
            inv = 1.0 / jnp.sum(e, axis=-1, keepdims=True)
            v = padded(p[:, 2 * GW + i * Dh:2 * GW + (i + 1) * Dh])
            out.append((_dot(e.astype(BF16), v) * inv).astype(BF16))
        return jnp.concatenate(out, axis=1)

    def project(g, o, segs):
        rows = o.shape[0]
        y = _dot(o, wo_v[pl.ds(g * GW, GW), :])
        blocks = (0, SEG + MM) if len(segs) == 2 else (MM,)
        mem_lo = rows - R1
        if g == 0:
            acc_o[pl.ds(mem_lo, MM), :] = y[mem_lo:mem_lo + MM]
            for lo, s in zip(blocks, segs):
                acc_o[pl.ds(lo, SEG), :] = res_v[slot(s)] + y[lo:lo + SEG]
        elif g < n_grp - 1:
            acc_o[pl.ds(0, rows), :] += y
        else:
            y = acc_o[pl.ds(0, rows), :] + y
            for lo, s in zip(blocks, segs):
                res_v[slot(s)] = y[lo:lo + SEG]
            return y[mem_lo:mem_lo + MM]

    def ffn_input(segs):
        for n, s in enumerate(segs):
            x = res_v[slot(s)]
            acc_f[pl.ds(n * SEG, SEG), :] = x
            lhs_f[pl.ds(n * SEG, SEG), :] = _layernorm(x).astype(BF16)

    def ffn_up(c):
        h = lhs_f[...]
        gate = _dot(h, wg_v[:, pl.ds(c * FC, FC)])
        up = _dot(h, wu_v[:, pl.ds(c * FC, FC)])
        return (_gelu(gate) * up).astype(BF16)

    def ffn_down(c, a, segs):
        y = _dot(a, wd_v[pl.ds(c * FC, FC), :])
        if c < n_fc - 1:
            acc_f[...] += y
        else:
            y = acc_f[...] + y
            for n, s in enumerate(segs):
                r = y[n * SEG:(n + 1) * SEG]
                res_v[slot(s)] = r
                o_v[seg_rows(s), :] = r.astype(BF16)

    def out_copy(s):
        return pltpu.make_async_copy(o_v.at[seg_rows(s)], out_hbm.at[seg_rows(s)], out_sem)

    def ffn_cuts(parts):
        width = DF // parts
        cuts = list(range(0, width, FC)) + [width]
        return [(width, lo, hi - lo) for lo, hi in zip(cuts, cuts[1:])]

    def ffn_piece(op, k, cut, act):
        width, lo, n = cut
        cols = pl.ds(pl.multiple_of(k * width + lo, 128), n)
        if op == "u":
            h = lhs_f[...]
            return (_gelu(_dot(h, wg_v[:, cols])) * _dot(h, wu_v[:, cols])).astype(BF16)
        acc_f[...] += _dot(act, wd_v[cols, :])

    def project_piece(g, o):
        acc_o[pl.ds(0, o.shape[0]), :] += _dot(
            o, wo_v[pl.ds(pl.multiple_of(g * GW, GW), GW), :])

    def ffn_output(segs):
        for n, s in enumerate(segs):
            r = acc_f[pl.ds(n * SEG, SEG), :]
            res_v[slot(s)] = r
            o_v[seg_rows(s), :] = r.astype(BF16)

    def single_attention(layer, s):
        acc_o[pl.ds(0, MM), :] = jnp.zeros((MM, D), F32)
        acc_o[pl.ds(MM, SEG), :] = res_v[slot(s)]
        gs = n_grp // ATT_PARTS

        def part(k, c):
            pl.when(jnp.logical_and(jnp.logical_and(layer == 0, s == 0), k == ATT_PARTS // 2))(
                finish_loads)
            p, ss, o = {}, {}, {}
            for op, n in _step_order(gs, 1):
                g = k * gs + n
                if op == "q":
                    p[n] = qkv(g, R1)
                elif op == "i":
                    lhs_next[pl.ds(0, SEG), :] = _layernorm(res_v[slot(s + 1)]).astype(BF16)
                elif op == "s":
                    ss[n] = scores(p[n])
                elif op == "a":
                    o[n] = attend(p[n], ss[n], fill_s.at[layer])
                elif op == "o":
                    project_piece(g, o[n])
            return c

        lax.fori_loop(0, ATT_PARTS, part, 0)
        lhs_a[pl.ds(SEG + MM, SEG), :] = lhs_next[pl.ds(0, SEG), :]
        res_v[slot(s)] = acc_o[pl.ds(MM, SEG), :]
        own = jnp.where(lax.broadcasted_iota(jnp.int32, (MM, D), 0) < M, 0, 1) == layer
        lhs_a[pl.ds(SEG, MM), :] = jnp.where(
            own, acc_o[pl.ds(0, MM), :], lhs_a[pl.ds(SEG, MM), :].astype(F32)).astype(BF16)

    def single_ffn(segs):
        ffn_input(segs)
        cuts = ffn_cuts(FFN_PARTS)

        def part(k, c):
            a = {0: ffn_piece("u", k, cuts[0], None)}
            for n, cut in enumerate(cuts):
                if n + 1 < len(cuts):
                    a[n + 1] = ffn_piece("u", k, cuts[n + 1], None)
                ffn_piece("d", k, cut, a[n])
            return c

        lax.fori_loop(0, FFN_PARTS, part, 0)
        ffn_output(segs)

    def step_segments(t):
        return (t, t - LAG), (t - 1, jnp.where(t == LAG, t - 2, t - LAG - 1))

    def next_attention_input(t):
        attention_input(0, load_segment(jnp.minimum(t + 1, n_seg - 1)))
        attention_input(1, res_v[slot(t + 1 - LAG)])

    def paired_step(t, carry):
        att, ffn = step_segments(t)
        p, ss, o, a = {}, {}, {}, {}
        for op, n in _step_order(n_grp, n_fc):
            if op == "q":
                p[n] = qkv(n, R2)
            elif op == "s":
                ss[n] = scores(p[n])
            elif op == "a":
                o[n] = attend(p[n], ss[n], fill_v)
            elif op == "o":
                mem = project(n, o[n], att)
                if n == n_grp - 1:
                    lhs_a[pl.ds(SEG, MM), :] = mem.astype(BF16)
            elif op == "i":
                ffn_input(ffn)
            elif op == "u":
                a[n] = ffn_up(n)
            elif op == "d":
                ffn_down(n, a[n], ffn)
            else:
                next_attention_input(t)
        out_copy(t - LAG - 1).start()
        return carry

    def precomputed_step(t, carry):
        att, ffn = step_segments(t)
        pre_rows = pl.ds(pl.multiple_of((t - LAG) * SEG, SEG), SEG)
        gs, cuts = n_grp // PRE_PARTS, ffn_cuts(PRE_PARTS)
        acc_o[pl.ds(0, SEG), :] = res_v[slot(att[0])]
        acc_o[pl.ds(SEG, MM), :] = jnp.zeros((MM, D), F32)
        acc_o[pl.ds(SEG + MM, SEG), :] = res_v[slot(att[1])]
        for n, s in enumerate(ffn):
            acc_f[pl.ds(n * SEG, SEG), :] = res_v[slot(s)]

        def part(k, c):
            p, ss, o, a = {}, {}, {}, {}
            for op, n in _step_order(gs, len(cuts)):
                g = k * gs + n
                if op == "q":
                    p[n] = jnp.concatenate(
                        [jnp.concatenate([pre_v[m, g, pre_rows, :] for m in range(3)], axis=1),
                         qkv(g, R1)], axis=0)
                elif op == "s":
                    ss[n] = scores(p[n])
                elif op == "a":
                    o[n] = attend(p[n], ss[n], fill_v)
                elif op == "o":
                    project_piece(g, o[n])
                elif op == "i":
                    for j, s in enumerate(ffn):
                        lhs_f[pl.ds(j * SEG, SEG), :] = _layernorm(res_v[slot(s)]).astype(BF16)
                elif op == "n":
                    lhs_next[pl.ds(0, SEG), :] = _layernorm(load_segment(t + 1)).astype(BF16)
                    lhs_next[pl.ds(SEG, SEG), :] = _layernorm(
                        res_v[slot(t + 1 - LAG)]).astype(BF16)
                else:
                    a[n] = ffn_piece(op, k, cuts[n], a.get(n))
            return c

        lax.fori_loop(0, PRE_PARTS, part, 0)
        lhs_a[pl.ds(0, SEG), :] = lhs_next[pl.ds(0, SEG), :]
        lhs_a[pl.ds(SEG, MM), :] = acc_o[pl.ds(SEG, MM), :].astype(BF16)
        lhs_a[pl.ds(SEG + MM, SEG), :] = lhs_next[pl.ds(SEG, SEG), :]
        res_v[slot(att[0])] = acc_o[pl.ds(0, SEG), :]
        res_v[slot(att[1])] = acc_o[pl.ds(SEG + MM, SEG), :]
        ffn_output(ffn)

        @pl.when(t > LAG)
        def _():
            out_copy(t - LAG - 1).start()

        return carry

    def single_op(phase, i):
        is_head = phase == 0
        j = i - 1
        tail_ffn = lax.rem(i, 3) == 0
        is_ffn = jnp.where(is_head, i == LAG, tail_ffn)
        first = n_seg - LAG + 2 * lax.div(jnp.maximum(j, 0), 3)

        @pl.when(jnp.logical_not(is_ffn))
        def _():
            single_attention(phase, jnp.where(is_head, i, first + lax.rem(j, 3)))

        @pl.when(is_ffn)
        def _():
            @pl.when(is_head)
            def _():
                for c in (wg_copy, wu_copy, wd_copy):
                    c.wait()
                x_rest.start()

            s0 = jnp.where(is_head, 0, jnp.where(i == 0, n_seg - 1, first))
            s1 = jnp.where(is_head, 1, jnp.where(i == 0, n_seg - LAG - 1, first + 1))
            single_ffn((s0, s1))

            @pl.when(jnp.logical_not(is_head))
            def _():
                out_copy(s1).start()

                @pl.when(i > 0)
                def _():
                    out_copy(s0).start()

    def phase_body(phase, carry):
        n_ops = jnp.where(phase == 0, LAG + 1, 1 + 3 * (LAG // 2))
        lax.fori_loop(0, n_ops, lambda i, c: (single_op(phase, i), c)[1], 0)

        @pl.when(phase == 0)
        def _():
            x_rest.wait()
            attention_input(1, res_v[slot(0)])
            lax.fori_loop(LAG, LAG + PRE, precomputed_step, 0)
            lax.fori_loop(LAG + PRE, n_seg, paired_step, 0)

        return carry

    lax.fori_loop(0, 2, phase_body, 0)
    pltpu.make_async_copy(o_v, out_hbm, out_sem).wait()


@functools.partial(jax.jit, static_argnames=("A_seg_len",))
def pallas_interleave_layers__memory_aug_recurrent_mem_tr__glu_gated_geglu__prompt_kernel(
    A_x, A_mem0, A_Wq, A_Wk, A_Wv, A_Wo, A_seg_len, B_x, B_w_gate, B_w_up, B_w_down,
):
    del B_x
    B, S, D = A_x.shape
    _, H, Dh = A_Wq.shape
    M = A_mem0.shape[1]
    SEG = int(A_seg_len)
    DF = B_w_gate.shape[1]
    assert B == 1 and S % SEG == 0 and Dh == 128 and 2 * (M + SEG) <= 128
    R = 2 * (M + SEG)
    hbm = pl.BlockSpec(memory_space=pl.ANY)
    out = pl.pallas_call(
        functools.partial(_kernel, S=S, D=D, H=H, Dh=Dh, M=M, SEG=SEG, DF=DF),
        out_shape=jax.ShapeDtypeStruct((S, D), A_x.dtype),
        in_specs=[hbm, pl.BlockSpec(memory_space=pltpu.VMEM)] + [hbm] * 7,
        out_specs=hbm,
        scratch_shapes=[
            pltpu.VMEM((S, D), BF16),
            pltpu.VMEM((S, D), BF16),
            pltpu.VMEM((6 * D, H // 2, Dh), BF16),
            pltpu.VMEM((3, H // HG, D // 2, HG * Dh), jnp.int32),
            pltpu.VMEM((H * Dh, D), BF16),
            pltpu.VMEM((D, DF), BF16),
            pltpu.VMEM((D, DF), BF16),
            pltpu.VMEM((DF, D), BF16),
            pltpu.VMEM((RING, SEG, D), F32),
            pltpu.VMEM((R, D), BF16),
            pltpu.VMEM((2 * SEG, D), BF16),
            pltpu.VMEM((R, D), F32),
            pltpu.VMEM((2 * SEG, D), BF16),
            pltpu.VMEM((2 * SEG, D), F32),
            pltpu.VMEM((R, 128), F32),
            pltpu.VMEM((2, R - SEG, 128), F32),
            pltpu.VMEM((PRE * SEG, D), BF16),
            pltpu.VMEM((3, H // HG, PRE * SEG, HG * Dh), BF16),
            pltpu.SemaphoreType.DMA((8 * (D // RB),)),
            pltpu.SemaphoreType.DMA((5,)),
            pltpu.SemaphoreType.DMA(()),
        ],
        compiler_params=pltpu.CompilerParams(vmem_limit_bytes=120 * 2**20),
    )(A_x.reshape(S, D), A_mem0.reshape(M, D),
      A_Wq, A_Wk, A_Wv,
      A_Wo.reshape(H * Dh, D), B_w_gate, B_w_up, B_w_down)
    return out.reshape(B, S, D)
```

```python
import functools
import math

import jax
import jax.numpy as jnp
from jax import lax
from jax.experimental import pallas as pl
from jax.experimental.pallas import tpu as pltpu

F32 = jnp.float32
BF16 = jnp.bfloat16

HG = 2
FC = 512
LAG = 4
RING = 8
ORDER = "usdqao"

RB = 256
WINDOW = 8
CATCH_UP = 3
FFN_START = 27
PRE = 7
PRE_ROWS = 112
CUTS = (0, 7, 12, 16, 16)

PRE_PARTS = 2
ATT_PARTS = 2
FFN_PARTS = 2


def _step_order(n_grp, n_fc):
    at = [(c * (n_grp - 1)) // n_fc for c in range(n_fc)]
    order = [("q", 0), ("i", 0), ("q", 1), ("s", 0)]
    for g in range(n_grp):
        items = {
            "q": [("q", g + 2)] * (g + 2 < n_grp) + [("n", 0)] * (g + 2 == n_grp),
            "s": [("s", g + 1)] * (g + 1 < n_grp),
            "u": [("u", c) for c in range(n_fc) if at[c] == g],
            "d": [("d", c) for c in range(n_fc - 1) if at[c] + 1 == g],
            "a": [("a", g)],
            "o": [("o", g - 1)] * (g >= 1),
        }
        for kind in ORDER:
            order += items[kind]
    return order + [("o", n_grp - 1), ("d", n_fc - 1)]


def _layernorm(x):
    m = jnp.mean(x, axis=-1, keepdims=True)
    c = x - m
    v = jnp.mean(c * c, axis=-1, keepdims=True)
    return c * lax.rsqrt(v + 1e-5)


def _gelu(x):
    c0 = math.sqrt(2.0 / math.pi)
    inner = x * (c0 + (c0 * 0.044715) * (x * x))
    return (0.5 * x) * (1.0 + jnp.tanh(inner))


def _dot(a, b):
    return jnp.dot(a, b, preferred_element_type=F32)


def _kernel(x_hbm, mem0_ref, wq_hbm, wk_hbm, wv_hbm, wo_hbm, wg_hbm, wu_hbm, wd_hbm,
            out_hbm,
            x_v, o_v, raw_v, wqkv_v, wo_v, wg_v, wu_v, wd_v,
            res_v, lhs_a, lhs_next, acc_o, lhs_f, acc_f, fill_v, fill_s, pre_in, pre_v,
            chunk_sem, w_sem, out_sem,
            *, S, D, H, Dh, M, SEG, DF):
    n_seg = S // SEG
    MM = 2 * M
    R2 = MM + 2 * SEG
    R1 = MM + SEG
    n_grp = H // HG
    n_fc = DF // FC
    GW = HG * Dh
    scale = Dh ** -0.5
    exp_c = scale * math.log2(math.e)

    n_rb = D // RB
    n_raw = 6 * n_rb
    n_chunk = 8 * n_rb
    HH = H // 2

    def raw_copy(w_hbm, i):
        unit, r = lax.div(i, n_rb), lax.rem(i, n_rb)
        heads = pl.ds(pl.multiple_of(lax.div(unit, 3) * HH, HH), HH)
        return pltpu.make_async_copy(
            w_hbm.at[pl.ds(pl.multiple_of(r * RB, RB), RB), heads],
            raw_v.at[pl.ds(pl.multiple_of(i * RB, RB), RB)], chunk_sem.at[i])

    def wo_copy(i):
        n = H * Dh // (2 * n_rb)
        rows = pl.ds(pl.multiple_of((i - n_raw) * n, n), n)
        return pltpu.make_async_copy(wo_hbm.at[rows], wo_v.at[rows], chunk_sem.at[i])

    def start_chunk(i, carry):
        for m, w_hbm in enumerate((wq_hbm, wk_hbm, wv_hbm)):
            @pl.when(jnp.logical_and(i < n_raw, lax.rem(lax.div(i, n_rb), 3) == m))
            def _():
                raw_copy(w_hbm, i).start()

        @pl.when(i >= n_raw)
        def _():
            wo_copy(i).start()

        return carry

    def wait_raw(i):
        dst = raw_v.at[pl.ds(pl.multiple_of(i * RB, RB), RB)]
        pltpu.make_async_copy(dst, dst, chunk_sem.at[i]).wait()

    head_rows = (LAG + PRE + 1) * SEG
    x_head, wg_copy, wu_copy, wd_copy, x_rest = [
        pltpu.make_async_copy(s, d, w_sem.at[i]) for i, (s, d) in enumerate((
            (x_hbm.at[pl.ds(0, head_rows)], x_v.at[pl.ds(0, head_rows)]),
            (wg_hbm, wg_v), (wu_hbm, wu_v), (wd_hbm, wd_v),
            (x_hbm.at[pl.ds(head_rows, S - head_rows)],
             x_v.at[pl.ds(head_rows, S - head_rows)])))]
    x_head.start()
    lax.fori_loop(0, WINDOW, start_chunk, None)

    def make_fill(rows, mem_lo, layer_of):
        row = lax.broadcasted_iota(jnp.int32, (rows, 128), 0)
        col = lax.broadcasted_iota(jnp.int32, (rows, 128), 1)

        def is_mem(i):
            return (i >= mem_lo) & (i < mem_lo + MM)

        keep = is_mem(row) | is_mem(col) | (row >= col)
        return jnp.where(layer_of(row) == layer_of(col),
                         jnp.where(keep, 0.0, -1e9 / scale), -jnp.inf).astype(F32)

    fill_v[...] = make_fill(
        R2, SEG, lambda i: jnp.where(i < SEG + M, 0, jnp.where(i < R2, 1, 2)))
    for layer in range(2):
        fill_s[layer] = make_fill(R1, 0, lambda i: jnp.where(
            i < M, 0, jnp.where(i < MM, 1, jnp.where(i < R1, layer, 2))))

    grp_half = n_grp // 2

    def relayout(i, ts):
        unit, r = lax.div(i, n_rb), lax.rem(i, n_rb)
        half, m = lax.div(unit, 3), lax.rem(unit, 3)
        for t in ts:
            x = raw_v[pl.ds(pl.multiple_of(i * RB + t * 16, 16), 16)].reshape(16 * HH, Dh)
            x = pltpu.bitcast(x, jnp.int32).reshape(8, 2, HH // 2, Dh)
            ev, od = x[:, 0], x[:, 1]
            lo = jnp.swapaxes((ev & 0xFFFF) | (od << 16), 0, 1)
            hi = jnp.swapaxes(lax.shift_right_logical(ev, 16) | (od & -65536), 0, 1)
            rows = pl.ds(pl.multiple_of(r * (RB // 2) + t * 8, 8), 8)
            for j in range(HH // 2):
                g, c = divmod(2 * j, HG)
                wqkv_v[m, half * grp_half + g, rows, pl.ds(c * Dh, Dh)] = lo[j]
                wqkv_v[m, half * grp_half + g, rows, pl.ds((c + 1) * Dh, Dh)] = hi[j]

    pieces = [(j, lo) for j in range(grp_half // n_rb) for lo in range(0, PRE * SEG, PRE_ROWS)]

    def precompute(i, j, lo):
        unit, r = lax.div(i, n_rb), lax.rem(i, n_rb)
        half, m = lax.div(unit, 3), lax.rem(unit, 3)
        g = half * grp_half + r * (grp_half // n_rb) + j
        rows = pl.ds(lo, min(PRE_ROWS, PRE * SEG - lo))
        pre_v[m, g, rows, :] = _dot(
            pre_in[rows, :], pltpu.bitcast(wqkv_v[m, g], BF16)).astype(BF16)

    def seg_rows(s):
        return pl.ds(pl.multiple_of(s * SEG, SEG), SEG)

    def slot(s):
        return s & (RING - 1)

    def load_segment(s):
        x0 = x_v[seg_rows(s), :].astype(F32)
        res_v[slot(s)] = x0
        return x0

    def attention_input(n, x):
        lhs_a[pl.ds(n * (SEG + MM), SEG), :] = _layernorm(x).astype(BF16)

    x_head.wait()
    mem0 = mem0_ref[...].astype(F32)
    lhs_a[pl.ds(SEG, MM), :] = jnp.concatenate([mem0, mem0], axis=0).astype(BF16)
    attention_input(1, load_segment(0))
    for s in range(1, LAG + 1):
        load_segment(s)

    for s in range(LAG, LAG + PRE):
        x0 = x_v[pl.ds(s * SEG, SEG), :].astype(F32)
        pre_in[pl.ds((s - LAG) * SEG, SEG), :] = _layernorm(x0).astype(BF16)

    def started(n):
        return jnp.minimum(WINDOW + n + lax.div(jnp.maximum(n - n_rb, 0), CATCH_UP), n_chunk)

    def load_body(i, carry):
        lax.fori_loop(started(i), started(i + 1), start_chunk, None)

        @pl.when(i == FFN_START)
        def _():
            wg_copy.start()

        @pl.when(i < n_rb)
        def _():
            wait_raw(i)
            relayout(i, range(RB // 16))

        @pl.when(jnp.logical_and(i >= n_rb, i < n_raw))
        def _():
            wait_raw(i)
            for piece, (lo, hi) in zip(pieces, zip(CUTS, CUTS[1:])):
                precompute(i - n_rb, *piece)
                relayout(i, range(lo, hi))

        @pl.when(i >= n_raw)
        def _():
            wo_copy(i).wait()
            for piece in pieces:
                precompute(i - n_rb, *piece)

        return carry

    lax.fori_loop(0, n_chunk - n_rb, load_body, 0)
    lax.fori_loop(started(n_chunk - n_rb), n_chunk, start_chunk, None)

    def finish_loads():
        for i in range(n_chunk - n_rb, n_chunk):
            wo_copy(i).wait()
        wu_copy.start()
        wd_copy.start()

    def qkv(g, rows):
        h = lhs_a[pl.ds(R2 - rows, rows), :]
        return jnp.concatenate(
            [_dot(h, pltpu.bitcast(wqkv_v[m, g], BF16)).astype(BF16) for m in range(3)],
            axis=1)

    def padded(a):
        return jnp.concatenate([a, jnp.zeros((128 - a.shape[0], Dh), BF16)], axis=0)

    def scores(p):
        return [lax.dot_general(p[:, i * Dh:(i + 1) * Dh],
                                padded(p[:, GW + i * Dh:GW + (i + 1) * Dh]),
                                (((1,), (1,)), ((), ())), preferred_element_type=F32)
                for i in range(HG)]

    def attend(p, ss, fill_ref):
        out = []
        for i in range(HG):
            fill = fill_ref[...]
            s = jnp.where(fill == 0.0, ss[i], fill)
            e = jnp.exp2((s - jnp.max(s, axis=-1, keepdims=True)) * exp_c)
            inv = 1.0 / jnp.sum(e, axis=-1, keepdims=True)
            v = padded(p[:, 2 * GW + i * Dh:2 * GW + (i + 1) * Dh])
            out.append((_dot(e.astype(BF16), v) * inv).astype(BF16))
        return jnp.concatenate(out, axis=1)

    def project(g, o, segs):
        rows = o.shape[0]
        y = _dot(o, wo_v[pl.ds(g * GW, GW), :])
        blocks = (0, SEG + MM) if len(segs) == 2 else (MM,)
        mem_lo = rows - R1
        if g == 0:
            acc_o[pl.ds(mem_lo, MM), :] = y[mem_lo:mem_lo + MM]
            for lo, s in zip(blocks, segs):
                acc_o[pl.ds(lo, SEG), :] = res_v[slot(s)] + y[lo:lo + SEG]
        elif g < n_grp - 1:
            acc_o[pl.ds(0, rows), :] += y
        else:
            y = acc_o[pl.ds(0, rows), :] + y
            for lo, s in zip(blocks, segs):
                res_v[slot(s)] = y[lo:lo + SEG]
            return y[mem_lo:mem_lo + MM]

    def ffn_input(segs):
        for n, s in enumerate(segs):
            x = res_v[slot(s)]
            acc_f[pl.ds(n * SEG, SEG), :] = x
            lhs_f[pl.ds(n * SEG, SEG), :] = _layernorm(x).astype(BF16)

    def ffn_up(c):
        return ffn_piece("u", 0, (DF, c * FC, FC), None)

    def ffn_down(c, a, segs):
        y = _dot(a, wd_v[pl.ds(c * FC, FC), :])
        if c < n_fc - 1:
            acc_f[...] += y
        else:
            y = acc_f[...] + y
            for n, s in enumerate(segs):
                r = y[n * SEG:(n + 1) * SEG]
                res_v[slot(s)] = r
                o_v[seg_rows(s), :] = r.astype(BF16)

    def out_copy(s):
        return pltpu.make_async_copy(o_v.at[seg_rows(s)], out_hbm.at[seg_rows(s)], out_sem)

    def ffn_cuts(parts):
        width = DF // parts
        cuts = list(range(0, width, FC)) + [width]
        return [(width, lo, hi - lo) for lo, hi in zip(cuts, cuts[1:])]

    def ffn_piece(op, k, cut, act):
        width, lo, n = cut
        cols = pl.ds(pl.multiple_of(k * width + lo, 128), n)
        if op == "u":
            h = lhs_f[...]
            return (_gelu(_dot(h, wg_v[:, cols])) * _dot(h, wu_v[:, cols])).astype(BF16)
        acc_f[...] += _dot(act, wd_v[cols, :])

    def project_piece(g, o):
        acc_o[pl.ds(0, o.shape[0]), :] += _dot(
            o, wo_v[pl.ds(pl.multiple_of(g * GW, GW), GW), :])

    def ffn_output(segs):
        for n, s in enumerate(segs):
            r = acc_f[pl.ds(n * SEG, SEG), :]
            res_v[slot(s)] = r
            o_v[seg_rows(s), :] = r.astype(BF16)

    def single_attention(layer, s):
        acc_o[pl.ds(0, MM), :] = jnp.zeros((MM, D), F32)
        acc_o[pl.ds(MM, SEG), :] = res_v[slot(s)]
        gs = n_grp // ATT_PARTS

        def part(k, c):
            pl.when(jnp.logical_and(jnp.logical_and(layer == 0, s == 0), k == ATT_PARTS // 2))(
                finish_loads)
            p, ss, o = {}, {}, {}
            for op, n in _step_order(gs, 1):
                g = k * gs + n
                if op == "q":
                    p[n] = qkv(g, R1)
                elif op == "i":
                    lhs_next[pl.ds(0, SEG), :] = _layernorm(res_v[slot(s + 1)]).astype(BF16)
                elif op == "s":
                    ss[n] = scores(p[n])
                elif op == "a":
                    o[n] = attend(p[n], ss[n], fill_s.at[layer])
                elif op == "o":
                    project_piece(g, o[n])
            return c

        lax.fori_loop(0, ATT_PARTS, part, 0)
        lhs_a[pl.ds(SEG + MM, SEG), :] = lhs_next[pl.ds(0, SEG), :]
        res_v[slot(s)] = acc_o[pl.ds(MM, SEG), :]
        own = jnp.where(lax.broadcasted_iota(jnp.int32, (MM, D), 0) < M, 0, 1) == layer
        lhs_a[pl.ds(SEG, MM), :] = jnp.where(
            own, acc_o[pl.ds(0, MM), :], lhs_a[pl.ds(SEG, MM), :].astype(F32)).astype(BF16)

    def single_ffn(segs):
        ffn_input(segs)
        cuts = ffn_cuts(FFN_PARTS)

        def part(k, c):
            a = {0: ffn_piece("u", k, cuts[0], None)}
            for n, cut in enumerate(cuts):
                if n + 1 < len(cuts):
                    a[n + 1] = ffn_piece("u", k, cuts[n + 1], None)
                ffn_piece("d", k, cut, a[n])
            return c

        lax.fori_loop(0, FFN_PARTS, part, 0)
        ffn_output(segs)

    def step_segments(t):
        return (t, t - LAG), (t - 1, jnp.where(t == LAG, t - 2, t - LAG - 1))

    def next_attention_input(t):
        attention_input(0, load_segment(jnp.minimum(t + 1, n_seg - 1)))
        attention_input(1, res_v[slot(t + 1 - LAG)])

    def paired_step(t, carry):
        att, ffn = step_segments(t)
        p, ss, o, a = {}, {}, {}, {}
        for op, n in _step_order(n_grp, n_fc):
            if op == "q":
                p[n] = qkv(n, R2)
            elif op == "s":
                ss[n] = scores(p[n])
            elif op == "a":
                o[n] = attend(p[n], ss[n], fill_v)
            elif op == "o":
                mem = project(n, o[n], att)
                if n == n_grp - 1:
                    lhs_a[pl.ds(SEG, MM), :] = mem.astype(BF16)
            elif op == "i":
                ffn_input(ffn)
            elif op == "u":
                a[n] = ffn_up(n)
            elif op == "d":
                ffn_down(n, a[n], ffn)
            else:
                next_attention_input(t)
        out_copy(t - LAG - 1).start()
        return carry

    def precomputed_step(t, carry):
        att, ffn = step_segments(t)
        pre_rows = pl.ds(pl.multiple_of((t - LAG) * SEG, SEG), SEG)
        gs, cuts = n_grp // PRE_PARTS, ffn_cuts(PRE_PARTS)
        acc_o[pl.ds(0, SEG), :] = res_v[slot(att[0])]
        acc_o[pl.ds(SEG, MM), :] = jnp.zeros((MM, D), F32)
        acc_o[pl.ds(SEG + MM, SEG), :] = res_v[slot(att[1])]
        for n, s in enumerate(ffn):
            acc_f[pl.ds(n * SEG, SEG), :] = res_v[slot(s)]

        def part(k, c):
            p, ss, o, a = {}, {}, {}, {}
            for op, n in _step_order(gs, len(cuts)):
                g = k * gs + n
                if op == "q":
                    p[n] = jnp.concatenate(
                        [jnp.concatenate([pre_v[m, g, pre_rows, :] for m in range(3)], axis=1),
                         qkv(g, R1)], axis=0)
                elif op == "s":
                    ss[n] = scores(p[n])
                elif op == "a":
                    o[n] = attend(p[n], ss[n], fill_v)
                elif op == "o":
                    project_piece(g, o[n])
                elif op == "i":
                    for j, s in enumerate(ffn):
                        lhs_f[pl.ds(j * SEG, SEG), :] = _layernorm(res_v[slot(s)]).astype(BF16)
                elif op == "n":
                    lhs_next[pl.ds(0, SEG), :] = _layernorm(load_segment(t + 1)).astype(BF16)
                    lhs_next[pl.ds(SEG, SEG), :] = _layernorm(
                        res_v[slot(t + 1 - LAG)]).astype(BF16)
                else:
                    a[n] = ffn_piece(op, k, cuts[n], a.get(n))
            return c

        lax.fori_loop(0, PRE_PARTS, part, 0)
        lhs_a[pl.ds(0, SEG), :] = lhs_next[pl.ds(0, SEG), :]
        lhs_a[pl.ds(SEG, MM), :] = acc_o[pl.ds(SEG, MM), :].astype(BF16)
        lhs_a[pl.ds(SEG + MM, SEG), :] = lhs_next[pl.ds(SEG, SEG), :]
        res_v[slot(att[0])] = acc_o[pl.ds(0, SEG), :]
        res_v[slot(att[1])] = acc_o[pl.ds(SEG + MM, SEG), :]
        ffn_output(ffn)

        @pl.when(t > LAG)
        def _():
            out_copy(t - LAG - 1).start()

        return carry

    def single_op(phase, i):
        is_head = phase == 0
        j = i - 1
        tail_ffn = lax.rem(i, 3) == 0
        is_ffn = jnp.where(is_head, i == LAG, tail_ffn)
        first = n_seg - LAG + 2 * lax.div(jnp.maximum(j, 0), 3)

        @pl.when(jnp.logical_not(is_ffn))
        def _():
            single_attention(phase, jnp.where(is_head, i, first + lax.rem(j, 3)))

        @pl.when(is_ffn)
        def _():
            @pl.when(is_head)
            def _():
                for c in (wg_copy, wu_copy, wd_copy):
                    c.wait()
                x_rest.start()

            s0 = jnp.where(is_head, 0, jnp.where(i == 0, n_seg - 1, first))
            s1 = jnp.where(is_head, 1, jnp.where(i == 0, n_seg - LAG - 1, first + 1))
            single_ffn((s0, s1))

            @pl.when(jnp.logical_not(is_head))
            def _():
                out_copy(s1).start()

                @pl.when(i > 0)
                def _():
                    out_copy(s0).start()

    def phase_body(phase, carry):
        n_ops = jnp.where(phase == 0, LAG + 1, 1 + 3 * (LAG // 2))
        lax.fori_loop(0, n_ops, lambda i, c: (single_op(phase, i), c)[1], 0)

        @pl.when(phase == 0)
        def _():
            x_rest.wait()
            attention_input(1, res_v[slot(0)])
            lax.fori_loop(LAG, LAG + PRE, precomputed_step, 0)
            lax.fori_loop(LAG + PRE, n_seg, paired_step, 0)

        return carry

    lax.fori_loop(0, 2, phase_body, 0)
    pltpu.make_async_copy(o_v, out_hbm, out_sem).wait()


@functools.partial(jax.jit, static_argnames=("A_seg_len",))
def pallas_interleave_layers__memory_aug_recurrent_mem_tr__glu_gated_geglu__prompt_kernel(
    A_x, A_mem0, A_Wq, A_Wk, A_Wv, A_Wo, A_seg_len, B_x, B_w_gate, B_w_up, B_w_down,
):
    del B_x
    B, S, D = A_x.shape
    _, H, Dh = A_Wq.shape
    M = A_mem0.shape[1]
    SEG = int(A_seg_len)
    DF = B_w_gate.shape[1]
    assert B == 1 and Dh == 128 and (M, SEG, H) == (8, 32, 32) and S // SEG >= LAG + PRE + 1
    R = 2 * (M + SEG)
    hbm = pl.BlockSpec(memory_space=pl.ANY)
    out = pl.pallas_call(
        functools.partial(_kernel, S=S, D=D, H=H, Dh=Dh, M=M, SEG=SEG, DF=DF),
        out_shape=jax.ShapeDtypeStruct((S, D), A_x.dtype),
        in_specs=[hbm, pl.BlockSpec(memory_space=pltpu.VMEM)] + [hbm] * 7,
        out_specs=hbm,
        scratch_shapes=[
            pltpu.VMEM((S, D), BF16),
            pltpu.VMEM((S, D), BF16),
            pltpu.VMEM((6 * D, H // 2, Dh), BF16),
            pltpu.VMEM((3, H // HG, D // 2, HG * Dh), jnp.int32),
            pltpu.VMEM((H * Dh, D), BF16),
            pltpu.VMEM((D, DF), BF16),
            pltpu.VMEM((D, DF), BF16),
            pltpu.VMEM((DF, D), BF16),
            pltpu.VMEM((RING, SEG, D), F32),
            pltpu.VMEM((R, D), BF16),
            pltpu.VMEM((2 * SEG, D), BF16),
            pltpu.VMEM((R, D), F32),
            pltpu.VMEM((2 * SEG, D), BF16),
            pltpu.VMEM((2 * SEG, D), F32),
            pltpu.VMEM((R, 128), F32),
            pltpu.VMEM((2, R - SEG, 128), F32),
            pltpu.VMEM((PRE * SEG, D), BF16),
            pltpu.VMEM((3, H // HG, PRE * SEG, HG * Dh), BF16),
            pltpu.SemaphoreType.DMA((8 * (D // RB),)),
            pltpu.SemaphoreType.DMA((5,)),
            pltpu.SemaphoreType.DMA(()),
        ],
        compiler_params=pltpu.CompilerParams(vmem_limit_bytes=120 * 2**20),
    )(A_x.reshape(S, D), A_mem0.reshape(M, D),
      A_Wq, A_Wk, A_Wv,
      A_Wo.reshape(H * Dh, D), B_w_gate, B_w_up, B_w_down)
    return out.reshape(B, S, D)
```

```python
import functools
import math

import jax
import jax.numpy as jnp
from jax import lax
from jax.experimental import pallas as pl
from jax.experimental.pallas import tpu as pltpu

F32 = jnp.float32
BF16 = jnp.bfloat16

HG = 2
FC = 512
LAG = 4
RING = 8
ORDER = "usdqao"

RB = 256
WINDOW = 8
FFN_START = 27
PRE = 7
PRE_ROWS = 112
CUTS = (0, 7, 12, 16, 16)

PRE_PARTS = 2
ATT_PARTS = 2
FFN_PARTS = 2


def _step_order(n_grp, n_fc):
    at = [(c * (n_grp - 1)) // n_fc for c in range(n_fc)]
    order = [("q", 0), ("i", 0), ("q", 1), ("s", 0)]
    for g in range(n_grp):
        items = {
            "q": [("q", g + 2)] * (g + 2 < n_grp) + [("n", 0)] * (g + 2 == n_grp),
            "s": [("s", g + 1)] * (g + 1 < n_grp),
            "u": [("u", c) for c in range(n_fc) if at[c] == g],
            "d": [("d", c) for c in range(n_fc - 1) if at[c] + 1 == g],
            "a": [("a", g)],
            "o": [("o", g - 1)] * (g >= 1),
        }
        for kind in ORDER:
            order += items[kind]
    return order + [("o", n_grp - 1), ("d", n_fc - 1)]


def _layernorm(x):
    m = jnp.mean(x, axis=-1, keepdims=True)
    c = x - m
    v = jnp.mean(c * c, axis=-1, keepdims=True)
    return c * lax.rsqrt(v + 1e-5)


def _gelu(x):
    c0 = math.sqrt(2.0 / math.pi)
    inner = x * (c0 + (c0 * 0.044715) * (x * x))
    return (0.5 * x) * (1.0 + jnp.tanh(inner))


def _dot(a, b):
    return jnp.dot(a, b, preferred_element_type=F32)


def _kernel(x_hbm, mem0_ref, wq_hbm, wk_hbm, wv_hbm, wo_hbm, wg_hbm, wu_hbm, wd_hbm,
            out_hbm,
            x_v, o_v, raw_v, wqkv_v, wo_v, wg_v, wu_v, wd_v,
            res_v, lhs_a, lhs_next, acc_o, lhs_f, acc_f, fill_v, fill_s, pre_in, pre_v,
            chunk_sem, w_sem, out_sem,
            *, S, D, H, Dh, M, SEG, DF):
    n_seg = S // SEG
    MM = 2 * M
    R2 = MM + 2 * SEG
    R1 = MM + SEG
    n_grp = H // HG
    n_fc = DF // FC
    GW = HG * Dh
    scale = Dh ** -0.5
    exp_c = scale * math.log2(math.e)

    n_rb = D // RB
    n_raw = 6 * n_rb
    n_chunk = 8 * n_rb
    assert WINDOW >= n_rb
    HH = H // 2

    def raw_copy(w_hbm, i):
        unit, r = lax.div(i, n_rb), lax.rem(i, n_rb)
        heads = pl.ds(pl.multiple_of(lax.div(unit, 3) * HH, HH), HH)
        return pltpu.make_async_copy(
            w_hbm.at[pl.ds(pl.multiple_of(r * RB, RB), RB), heads],
            raw_v.at[pl.ds(pl.multiple_of(i * RB, RB), RB)], chunk_sem.at[i])

    def wo_copy(i):
        n = H * Dh // (2 * n_rb)
        rows = pl.ds(pl.multiple_of((i - n_raw) * n, n), n)
        return pltpu.make_async_copy(wo_hbm.at[rows], wo_v.at[rows], chunk_sem.at[i])

    def start_chunk(i, carry):
        for m, w_hbm in enumerate((wq_hbm, wk_hbm, wv_hbm)):
            @pl.when(jnp.logical_and(i < n_raw, lax.rem(lax.div(i, n_rb), 3) == m))
            def _():
                raw_copy(w_hbm, i).start()

        @pl.when(i >= n_raw)
        def _():
            wo_copy(i).start()

        return carry

    def wait_raw(i):
        dst = raw_v.at[pl.ds(pl.multiple_of(i * RB, RB), RB)]
        pltpu.make_async_copy(dst, dst, chunk_sem.at[i]).wait()

    head_rows = (LAG + PRE + 1) * SEG
    x_head, wg_copy, wu_copy, wd_copy, x_rest = [
        pltpu.make_async_copy(s, d, w_sem.at[i]) for i, (s, d) in enumerate((
            (x_hbm.at[pl.ds(0, head_rows)], x_v.at[pl.ds(0, head_rows)]),
            (wg_hbm, wg_v), (wu_hbm, wu_v), (wd_hbm, wd_v),
            (x_hbm.at[pl.ds(head_rows, S - head_rows)],
             x_v.at[pl.ds(head_rows, S - head_rows)])))]
    x_head.start()
    lax.fori_loop(0, WINDOW, start_chunk, None)

    def make_fill(rows, mem_lo, layer_of):
        row = lax.broadcasted_iota(jnp.int32, (rows, 128), 0)
        col = lax.broadcasted_iota(jnp.int32, (rows, 128), 1)

        def is_mem(i):
            return (i >= mem_lo) & (i < mem_lo + MM)

        keep = is_mem(row) | is_mem(col) | (row >= col)
        return jnp.where(layer_of(row) == layer_of(col),
                         jnp.where(keep, 0.0, -1e9 / scale), -jnp.inf).astype(F32)

    fill_v[...] = make_fill(
        R2, SEG, lambda i: jnp.where(i < SEG + M, 0, jnp.where(i < R2, 1, 2)))
    for layer in range(2):
        fill_s[layer] = make_fill(R1, 0, lambda i: jnp.where(
            i < M, 0, jnp.where(i < MM, 1, jnp.where(i < R1, layer, 2))))

    grp_half = n_grp // 2

    def relayout(i, ts):
        unit, r = lax.div(i, n_rb), lax.rem(i, n_rb)
        half, m = lax.div(unit, 3), lax.rem(unit, 3)
        for t in ts:
            x = raw_v[pl.ds(pl.multiple_of(i * RB + t * 16, 16), 16)].reshape(16 * HH, Dh)
            x = pltpu.bitcast(x, jnp.int32).reshape(8, 2, HH // 2, Dh)
            ev, od = x[:, 0], x[:, 1]
            lo = jnp.swapaxes((ev & 0xFFFF) | (od << 16), 0, 1)
            hi = jnp.swapaxes(lax.shift_right_logical(ev, 16) | (od & -65536), 0, 1)
            rows = pl.ds(pl.multiple_of(r * (RB // 2) + t * 8, 8), 8)
            for j in range(HH // 2):
                g, c = divmod(2 * j, HG)
                wqkv_v[m, half * grp_half + g, rows, pl.ds(c * Dh, Dh)] = lo[j]
                wqkv_v[m, half * grp_half + g, rows, pl.ds((c + 1) * Dh, Dh)] = hi[j]

    pieces = [(j, lo) for j in range(grp_half // n_rb) for lo in range(0, PRE * SEG, PRE_ROWS)]

    def precompute(i, j, lo):
        unit, r = lax.div(i, n_rb), lax.rem(i, n_rb)
        half, m = lax.div(unit, 3), lax.rem(unit, 3)
        g = half * grp_half + r * (grp_half // n_rb) + j
        rows = pl.ds(lo, min(PRE_ROWS, PRE * SEG - lo))
        pre_v[m, g, rows, :] = _dot(
            pre_in[rows, :], pltpu.bitcast(wqkv_v[m, g], BF16)).astype(BF16)

    def seg_rows(s):
        return pl.ds(pl.multiple_of(s * SEG, SEG), SEG)

    def slot(s):
        return s & (RING - 1)

    def load_segment(s):
        x0 = x_v[seg_rows(s), :].astype(F32)
        res_v[slot(s)] = x0
        return x0

    def attention_input(n, x):
        lhs_a[pl.ds(n * (SEG + MM), SEG), :] = _layernorm(x).astype(BF16)

    x_head.wait()
    mem0 = mem0_ref[...].astype(F32)
    lhs_a[pl.ds(SEG, MM), :] = jnp.concatenate([mem0, mem0], axis=0).astype(BF16)
    attention_input(1, load_segment(0))
    for s in range(1, LAG + 1):
        load_segment(s)

    for s in range(LAG, LAG + PRE):
        x0 = x_v[pl.ds(s * SEG, SEG), :].astype(F32)
        pre_in[pl.ds((s - LAG) * SEG, SEG), :] = _layernorm(x0).astype(BF16)

    def load_body(i, carry):
        @pl.when(i + WINDOW < n_chunk)
        def _():
            start_chunk(i + WINDOW, None)

        @pl.when(i == FFN_START)
        def _():
            wg_copy.start()

        @pl.when(i < n_rb)
        def _():
            wait_raw(i)
            relayout(i, range(RB // 16))

        @pl.when(jnp.logical_and(i >= n_rb, i < n_raw))
        def _():
            wait_raw(i)
            for piece, (lo, hi) in zip(pieces, zip(CUTS, CUTS[1:])):
                precompute(i - n_rb, *piece)
                relayout(i, range(lo, hi))

        @pl.when(i >= n_raw)
        def _():
            wo_copy(i).wait()
            for piece in pieces:
                precompute(i - n_rb, *piece)

        return carry

    lax.fori_loop(0, n_chunk - n_rb, load_body, 0)

    def finish_loads():
        for i in range(n_chunk - n_rb, n_chunk):
            wo_copy(i).wait()
        wu_copy.start()
        wd_copy.start()

    def qkv(g, rows):
        h = lhs_a[pl.ds(R2 - rows, rows), :]
        return jnp.concatenate(
            [_dot(h, pltpu.bitcast(wqkv_v[m, g], BF16)).astype(BF16) for m in range(3)],
            axis=1)

    def padded(a):
        return jnp.concatenate([a, jnp.zeros((128 - a.shape[0], Dh), BF16)], axis=0)

    def scores(p):
        return [lax.dot_general(p[:, i * Dh:(i + 1) * Dh],
                                padded(p[:, GW + i * Dh:GW + (i + 1) * Dh]),
                                (((1,), (1,)), ((), ())), preferred_element_type=F32)
                for i in range(HG)]

    def attend(p, ss, fill_ref):
        out = []
        for i in range(HG):
            fill = fill_ref[...]
            s = jnp.where(fill == 0.0, ss[i], fill)
            e = jnp.exp2((s - jnp.max(s, axis=-1, keepdims=True)) * exp_c)
            inv = 1.0 / jnp.sum(e, axis=-1, keepdims=True)
            v = padded(p[:, 2 * GW + i * Dh:2 * GW + (i + 1) * Dh])
            out.append((_dot(e.astype(BF16), v) * inv).astype(BF16))
        return jnp.concatenate(out, axis=1)

    def project(g, o, segs):
        rows = o.shape[0]
        y = _dot(o, wo_v[pl.ds(g * GW, GW), :])
        blocks = (0, SEG + MM) if len(segs) == 2 else (MM,)
        mem_lo = rows - R1
        if g == 0:
            acc_o[pl.ds(mem_lo, MM), :] = y[mem_lo:mem_lo + MM]
            for lo, s in zip(blocks, segs):
                acc_o[pl.ds(lo, SEG), :] = res_v[slot(s)] + y[lo:lo + SEG]
        elif g < n_grp - 1:
            acc_o[pl.ds(0, rows), :] += y
        else:
            y = acc_o[pl.ds(0, rows), :] + y
            for lo, s in zip(blocks, segs):
                res_v[slot(s)] = y[lo:lo + SEG]
            return y[mem_lo:mem_lo + MM]

    def ffn_input(segs):
        for n, s in enumerate(segs):
            x = res_v[slot(s)]
            acc_f[pl.ds(n * SEG, SEG), :] = x
            lhs_f[pl.ds(n * SEG, SEG), :] = _layernorm(x).astype(BF16)

    def ffn_up(c):
        return ffn_piece("u", 0, (DF, c * FC, FC), None)

    def ffn_down(c, a, segs):
        y = _dot(a, wd_v[pl.ds(c * FC, FC), :])
        if c < n_fc - 1:
            acc_f[...] += y
        else:
            y = acc_f[...] + y
            for n, s in enumerate(segs):
                r = y[n * SEG:(n + 1) * SEG]
                res_v[slot(s)] = r
                o_v[seg_rows(s), :] = r.astype(BF16)

    def out_copy(s):
        return pltpu.make_async_copy(o_v.at[seg_rows(s)], out_hbm.at[seg_rows(s)], out_sem)

    def ffn_cuts(parts):
        width = DF // parts
        cuts = list(range(0, width, FC)) + [width]
        return [(width, lo, hi - lo) for lo, hi in zip(cuts, cuts[1:])]

    def ffn_piece(op, k, cut, act):
        width, lo, n = cut
        cols = pl.ds(pl.multiple_of(k * width + lo, 128), n)
        if op == "u":
            h = lhs_f[...]
            return (_gelu(_dot(h, wg_v[:, cols])) * _dot(h, wu_v[:, cols])).astype(BF16)
        acc_f[...] += _dot(act, wd_v[cols, :])

    def project_piece(g, o):
        acc_o[pl.ds(0, o.shape[0]), :] += _dot(
            o, wo_v[pl.ds(pl.multiple_of(g * GW, GW), GW), :])

    def ffn_output(segs):
        for n, s in enumerate(segs):
            r = acc_f[pl.ds(n * SEG, SEG), :]
            res_v[slot(s)] = r
            o_v[seg_rows(s), :] = r.astype(BF16)

    def single_attention(layer, s):
        acc_o[pl.ds(0, MM), :] = jnp.zeros((MM, D), F32)
        acc_o[pl.ds(MM, SEG), :] = res_v[slot(s)]
        gs = n_grp // ATT_PARTS

        def part(k, c):
            pl.when(jnp.logical_and(jnp.logical_and(layer == 0, s == 0), k == ATT_PARTS // 2))(
                finish_loads)
            p, ss, o = {}, {}, {}
            for op, n in _step_order(gs, 1):
                g = k * gs + n
                if op == "q":
                    p[n] = qkv(g, R1)
                elif op == "i":
                    lhs_next[pl.ds(0, SEG), :] = _layernorm(res_v[slot(s + 1)]).astype(BF16)
                elif op == "s":
                    ss[n] = scores(p[n])
                elif op == "a":
                    o[n] = attend(p[n], ss[n], fill_s.at[layer])
                elif op == "o":
                    project_piece(g, o[n])
            return c

        lax.fori_loop(0, ATT_PARTS, part, 0)
        lhs_a[pl.ds(SEG + MM, SEG), :] = lhs_next[pl.ds(0, SEG), :]
        res_v[slot(s)] = acc_o[pl.ds(MM, SEG), :]
        own = jnp.where(lax.broadcasted_iota(jnp.int32, (MM, D), 0) < M, 0, 1) == layer
        lhs_a[pl.ds(SEG, MM), :] = jnp.where(
            own, acc_o[pl.ds(0, MM), :], lhs_a[pl.ds(SEG, MM), :].astype(F32)).astype(BF16)

    def single_ffn(segs):
        ffn_input(segs)
        cuts = ffn_cuts(FFN_PARTS)

        def part(k, c):
            a = {0: ffn_piece("u", k, cuts[0], None)}
            for n, cut in enumerate(cuts):
                if n + 1 < len(cuts):
                    a[n + 1] = ffn_piece("u", k, cuts[n + 1], None)
                ffn_piece("d", k, cut, a[n])
            return c

        lax.fori_loop(0, FFN_PARTS, part, 0)
        ffn_output(segs)

    def step_segments(t):
        return (t, t - LAG), (t - 1, jnp.where(t == LAG, t - 2, t - LAG - 1))

    def next_attention_input(t):
        attention_input(0, load_segment(jnp.minimum(t + 1, n_seg - 1)))
        attention_input(1, res_v[slot(t + 1 - LAG)])

    def paired_step(t, carry):
        att, ffn = step_segments(t)
        p, ss, o, a = {}, {}, {}, {}
        for op, n in _step_order(n_grp, n_fc):
            if op == "q":
                p[n] = qkv(n, R2)
            elif op == "s":
                ss[n] = scores(p[n])
            elif op == "a":
                o[n] = attend(p[n], ss[n], fill_v)
            elif op == "o":
                mem = project(n, o[n], att)
                if n == n_grp - 1:
                    lhs_a[pl.ds(SEG, MM), :] = mem.astype(BF16)
            elif op == "i":
                ffn_input(ffn)
            elif op == "u":
                a[n] = ffn_up(n)
            elif op == "d":
                ffn_down(n, a[n], ffn)
            else:
                next_attention_input(t)
        out_copy(t - LAG - 1).start()
        return carry

    def precomputed_step(t, carry):
        att, ffn = step_segments(t)
        pre_rows = pl.ds(pl.multiple_of((t - LAG) * SEG, SEG), SEG)
        gs, cuts = n_grp // PRE_PARTS, ffn_cuts(PRE_PARTS)
        acc_o[pl.ds(0, SEG), :] = res_v[slot(att[0])]
        acc_o[pl.ds(SEG, MM), :] = jnp.zeros((MM, D), F32)
        acc_o[pl.ds(SEG + MM, SEG), :] = res_v[slot(att[1])]
        for n, s in enumerate(ffn):
            acc_f[pl.ds(n * SEG, SEG), :] = res_v[slot(s)]

        def part(k, c):
            p, ss, o, a = {}, {}, {}, {}
            for op, n in _step_order(gs, len(cuts)):
                g = k * gs + n
                if op == "q":
                    p[n] = jnp.concatenate(
                        [jnp.concatenate([pre_v[m, g, pre_rows, :] for m in range(3)], axis=1),
                         qkv(g, R1)], axis=0)
                elif op == "s":
                    ss[n] = scores(p[n])
                elif op == "a":
                    o[n] = attend(p[n], ss[n], fill_v)
                elif op == "o":
                    project_piece(g, o[n])
                elif op == "i":
                    for j, s in enumerate(ffn):
                        lhs_f[pl.ds(j * SEG, SEG), :] = _layernorm(res_v[slot(s)]).astype(BF16)
                elif op == "n":
                    lhs_next[pl.ds(0, SEG), :] = _layernorm(load_segment(t + 1)).astype(BF16)
                    lhs_next[pl.ds(SEG, SEG), :] = _layernorm(
                        res_v[slot(t + 1 - LAG)]).astype(BF16)
                else:
                    a[n] = ffn_piece(op, k, cuts[n], a.get(n))
            return c

        lax.fori_loop(0, PRE_PARTS, part, 0)
        lhs_a[pl.ds(0, SEG), :] = lhs_next[pl.ds(0, SEG), :]
        lhs_a[pl.ds(SEG, MM), :] = acc_o[pl.ds(SEG, MM), :].astype(BF16)
        lhs_a[pl.ds(SEG + MM, SEG), :] = lhs_next[pl.ds(SEG, SEG), :]
        res_v[slot(att[0])] = acc_o[pl.ds(0, SEG), :]
        res_v[slot(att[1])] = acc_o[pl.ds(SEG + MM, SEG), :]
        ffn_output(ffn)

        @pl.when(t > LAG)
        def _():
            out_copy(t - LAG - 1).start()

        return carry

    def single_op(phase, i):
        is_head = phase == 0
        j = i - 1
        tail_ffn = lax.rem(i, 3) == 0
        is_ffn = jnp.where(is_head, i == LAG, tail_ffn)
        first = n_seg - LAG + 2 * lax.div(jnp.maximum(j, 0), 3)

        @pl.when(jnp.logical_not(is_ffn))
        def _():
            single_attention(phase, jnp.where(is_head, i, first + lax.rem(j, 3)))

        @pl.when(is_ffn)
        def _():
            @pl.when(is_head)
            def _():
                for c in (wg_copy, wu_copy, wd_copy):
                    c.wait()
                x_rest.start()

            s0 = jnp.where(is_head, 0, jnp.where(i == 0, n_seg - 1, first))
            s1 = jnp.where(is_head, 1, jnp.where(i == 0, n_seg - LAG - 1, first + 1))
            single_ffn((s0, s1))

            @pl.when(jnp.logical_not(is_head))
            def _():
                out_copy(s1).start()

                @pl.when(i > 0)
                def _():
                    out_copy(s0).start()

    def phase_body(phase, carry):
        n_ops = jnp.where(phase == 0, LAG + 1, 1 + 3 * (LAG // 2))
        lax.fori_loop(0, n_ops, lambda i, c: (single_op(phase, i), c)[1], 0)

        @pl.when(phase == 0)
        def _():
            x_rest.wait()
            attention_input(1, res_v[slot(0)])
            lax.fori_loop(LAG, LAG + PRE, precomputed_step, 0)
            lax.fori_loop(LAG + PRE, n_seg, paired_step, 0)

        return carry

    lax.fori_loop(0, 2, phase_body, 0)
    pltpu.make_async_copy(o_v, out_hbm, out_sem).wait()


@functools.partial(jax.jit, static_argnames=("A_seg_len",))
def pallas_interleave_layers__memory_aug_recurrent_mem_tr__glu_gated_geglu__prompt_kernel(
    A_x, A_mem0, A_Wq, A_Wk, A_Wv, A_Wo, A_seg_len, B_x, B_w_gate, B_w_up, B_w_down,
):
    del B_x
    B, S, D = A_x.shape
    _, H, Dh = A_Wq.shape
    M = A_mem0.shape[1]
    SEG = int(A_seg_len)
    DF = B_w_gate.shape[1]
    assert B == 1 and Dh == 128 and (M, SEG, H) == (8, 32, 32) and S // SEG >= LAG + PRE + 1
    R = 2 * (M + SEG)
    hbm = pl.BlockSpec(memory_space=pl.ANY)
    out = pl.pallas_call(
        functools.partial(_kernel, S=S, D=D, H=H, Dh=Dh, M=M, SEG=SEG, DF=DF),
        out_shape=jax.ShapeDtypeStruct((S, D), A_x.dtype),
        in_specs=[hbm, pl.BlockSpec(memory_space=pltpu.VMEM)] + [hbm] * 7,
        out_specs=hbm,
        scratch_shapes=[
            pltpu.VMEM((S, D), BF16),
            pltpu.VMEM((S, D), BF16),
            pltpu.VMEM((6 * D, H // 2, Dh), BF16),
            pltpu.VMEM((3, H // HG, D // 2, HG * Dh), jnp.int32),
            pltpu.VMEM((H * Dh, D), BF16),
            pltpu.VMEM((D, DF), BF16),
            pltpu.VMEM((D, DF), BF16),
            pltpu.VMEM((DF, D), BF16),
            pltpu.VMEM((RING, SEG, D), F32),
            pltpu.VMEM((R, D), BF16),
            pltpu.VMEM((2 * SEG, D), BF16),
            pltpu.VMEM((R, D), F32),
            pltpu.VMEM((2 * SEG, D), BF16),
            pltpu.VMEM((2 * SEG, D), F32),
            pltpu.VMEM((R, 128), F32),
            pltpu.VMEM((2, R - SEG, 128), F32),
            pltpu.VMEM((PRE * SEG, D), BF16),
            pltpu.VMEM((3, H // HG, PRE * SEG, HG * Dh), BF16),
            pltpu.SemaphoreType.DMA((8 * (D // RB),)),
            pltpu.SemaphoreType.DMA((5,)),
            pltpu.SemaphoreType.DMA(()),
        ],
        compiler_params=pltpu.CompilerParams(vmem_limit_bytes=120 * 2**20),
    )(A_x.reshape(S, D), A_mem0.reshape(M, D),
      A_Wq, A_Wk, A_Wv,
      A_Wo.reshape(H * Dh, D), B_w_gate, B_w_up, B_w_down)
    return out.reshape(B, S, D)
```

```python
import functools
import math

import jax
import jax.numpy as jnp
from jax import lax
from jax.experimental import pallas as pl
from jax.experimental.pallas import tpu as pltpu

F32 = jnp.float32
BF16 = jnp.bfloat16

HG = 2
FC = 512
LAG = 4
RING = 8
ORDER = "usdqao"

RB = 256
WINDOW = 8
FFN_START = 27
PRE = 7
PRE_ROWS = 112
CUTS = (0, 7, 12, 16, 16)

PRE_PARTS = 2
ATT_PARTS = 2
FFN_PARTS = 2


def _step_order(n_grp, n_fc):
    at = [(c * (n_grp - 1)) // n_fc for c in range(n_fc)]
    order = [("q", 0), ("i", 0), ("q", 1), ("s", 0)]
    for g in range(n_grp):
        items = {
            "q": [("q", g + 2)] * (g + 2 < n_grp) + [("n", 0)] * (g + 2 == n_grp),
            "s": [("s", g + 1)] * (g + 1 < n_grp),
            "u": [("u", c) for c in range(n_fc) if at[c] == g],
            "d": [("d", c) for c in range(n_fc - 1) if at[c] + 1 == g],
            "a": [("a", g)],
            "o": [("o", g - 1)] * (g >= 1),
        }
        for kind in ORDER:
            order += items[kind]
    return order + [("o", n_grp - 1), ("d", n_fc - 1)]


def _layernorm(x):
    m = jnp.mean(x, axis=-1, keepdims=True)
    c = x - m
    v = jnp.mean(c * c, axis=-1, keepdims=True)
    return c * lax.rsqrt(v + 1e-5)


def _gelu(x):
    c0 = math.sqrt(2.0 / math.pi)
    inner = x * (c0 + (c0 * 0.044715) * (x * x))
    return (0.5 * x) * (1.0 + jnp.tanh(inner))


def _dot(a, b):
    return jnp.dot(a, b, preferred_element_type=F32)


def _kernel(x_hbm, mem0_ref, wq_hbm, wk_hbm, wv_hbm, wo_hbm, wg_hbm, wu_hbm, wd_hbm,
            out_hbm,
            x_v, o_v, raw_v, wqkv_v, wo_v, wg_v, wu_v, wd_v,
            res_v, lhs_a, lhs_next, acc_o, lhs_f, acc_f, fill_v, fill_s, pre_in, pre_v,
            chunk_sem, w_sem, out_sem,
            *, S, D, H, Dh, M, SEG, DF):
    n_seg = S // SEG
    MM = 2 * M
    R2 = MM + 2 * SEG
    R1 = MM + SEG
    n_grp = H // HG
    n_fc = DF // FC
    GW = HG * Dh
    scale = Dh ** -0.5
    exp_c = scale * math.log2(math.e)

    n_rb = D // RB
    n_raw = 6 * n_rb
    n_chunk = 8 * n_rb
    assert WINDOW >= n_rb
    HH = H // 2

    def raw_copy(w_hbm, i):
        unit, r = lax.div(i, n_rb), lax.rem(i, n_rb)
        heads = pl.ds(pl.multiple_of(lax.div(unit, 3) * HH, HH), HH)
        return pltpu.make_async_copy(
            w_hbm.at[pl.ds(pl.multiple_of(r * RB, RB), RB), heads],
            raw_v.at[pl.ds(pl.multiple_of(i * RB, RB), RB)], chunk_sem.at[i])

    def wo_copy(i):
        n = H * Dh // (2 * n_rb)
        rows = pl.ds(pl.multiple_of((i - n_raw) * n, n), n)
        return pltpu.make_async_copy(wo_hbm.at[rows], wo_v.at[rows], chunk_sem.at[i])

    def start_chunk(i, carry):
        for m, w_hbm in enumerate((wq_hbm, wk_hbm, wv_hbm)):
            @pl.when(jnp.logical_and(i < n_raw, lax.rem(lax.div(i, n_rb), 3) == m))
            def _():
                raw_copy(w_hbm, i).start()

        @pl.when(i >= n_raw)
        def _():
            wo_copy(i).start()

        return carry

    def wait_raw(i):
        dst = raw_v.at[pl.ds(pl.multiple_of(i * RB, RB), RB)]
        pltpu.make_async_copy(dst, dst, chunk_sem.at[i]).wait()

    head_rows = (LAG + PRE + 1) * SEG
    x_head, wg_copy, wu_copy, wd_copy, x_rest = [
        pltpu.make_async_copy(s, d, w_sem.at[i]) for i, (s, d) in enumerate((
            (x_hbm.at[pl.ds(0, head_rows)], x_v.at[pl.ds(0, head_rows)]),
            (wg_hbm, wg_v), (wu_hbm, wu_v), (wd_hbm, wd_v),
            (x_hbm.at[pl.ds(head_rows, S - head_rows)],
             x_v.at[pl.ds(head_rows, S - head_rows)])))]
    x_head.start()
    lax.fori_loop(0, WINDOW, start_chunk, None)

    def make_fill(rows, mem_lo, layer_of):
        row = lax.broadcasted_iota(jnp.int32, (rows, 128), 0)
        col = lax.broadcasted_iota(jnp.int32, (rows, 128), 1)

        def is_mem(i):
            return (i >= mem_lo) & (i < mem_lo + MM)

        keep = is_mem(row) | is_mem(col) | (row >= col)
        return jnp.where(layer_of(row) == layer_of(col),
                         jnp.where(keep, 0.0, -1e9 / scale), -jnp.inf).astype(F32)

    fill_v[...] = make_fill(
        R2, SEG, lambda i: jnp.where(i < SEG + M, 0, jnp.where(i < R2, 1, 2)))
    for layer in range(2):
        fill_s[layer] = make_fill(R1, 0, lambda i: jnp.where(
            i < M, 0, jnp.where(i < MM, 1, jnp.where(i < R1, layer, 2))))

    grp_half = n_grp // 2

    def relayout(i, ts):
        unit, r = lax.div(i, n_rb), lax.rem(i, n_rb)
        half, m = lax.div(unit, 3), lax.rem(unit, 3)
        for t in ts:
            x = raw_v[pl.ds(pl.multiple_of(i * RB + t * 16, 16), 16)].reshape(16 * HH, Dh)
            x = pltpu.bitcast(x, jnp.int32).reshape(8, 2, HH // 2, Dh)
            ev, od = x[:, 0], x[:, 1]
            lo = jnp.swapaxes((ev & 0xFFFF) | (od << 16), 0, 1)
            hi = jnp.swapaxes(lax.shift_right_logical(ev, 16) | (od & -65536), 0, 1)
            rows = pl.ds(pl.multiple_of(r * (RB // 2) + t * 8, 8), 8)
            for j in range(HH // 2):
                g, c = divmod(2 * j, HG)
                wqkv_v[m, half * grp_half + g, rows, pl.ds(c * Dh, Dh)] = lo[j]
                wqkv_v[m, half * grp_half + g, rows, pl.ds((c + 1) * Dh, Dh)] = hi[j]

    pieces = [(j, lo) for j in range(grp_half // n_rb) for lo in range(0, PRE * SEG, PRE_ROWS)]

    def precompute(i, j, lo):
        unit, r = lax.div(i, n_rb), lax.rem(i, n_rb)
        half, m = lax.div(unit, 3), lax.rem(unit, 3)
        g = half * grp_half + r * (grp_half // n_rb) + j
        rows = pl.ds(lo, min(PRE_ROWS, PRE * SEG - lo))
        pre_v[m, g, rows, :] = _dot(
            pre_in[rows, :], pltpu.bitcast(wqkv_v[m, g], BF16)).astype(BF16)

    def seg_rows(s):
        return pl.ds(pl.multiple_of(s * SEG, SEG), SEG)

    def slot(s):
        return s & (RING - 1)

    def load_segment(s):
        x0 = x_v[seg_rows(s), :].astype(F32)
        res_v[slot(s)] = x0
        return x0

    def attention_input(n, x):
        lhs_a[pl.ds(n * (SEG + MM), SEG), :] = _layernorm(x).astype(BF16)

    x_head.wait()
    mem0 = mem0_ref[...].astype(F32)
    lhs_a[pl.ds(SEG, MM), :] = jnp.concatenate([mem0, mem0], axis=0).astype(BF16)
    attention_input(1, load_segment(0))
    for s in range(1, LAG + 1):
        load_segment(s)

    for s in range(LAG, LAG + PRE):
        x0 = x_v[pl.ds(s * SEG, SEG), :].astype(F32)
        pre_in[pl.ds((s - LAG) * SEG, SEG), :] = _layernorm(x0).astype(BF16)

    def load_body(i, carry):
        @pl.when(i + WINDOW < n_chunk)
        def _():
            start_chunk(i + WINDOW, None)

        @pl.when(i == FFN_START)
        def _():
            wg_copy.start()

        @pl.when(i < n_rb)
        def _():
            wait_raw(i)
            relayout(i, range(RB // 16))

        @pl.when(jnp.logical_and(i >= n_rb, i < n_raw))
        def _():
            wait_raw(i)
            for piece, (lo, hi) in zip(pieces, zip(CUTS, CUTS[1:])):
                precompute(i - n_rb, *piece)
                relayout(i, range(lo, hi))

        @pl.when(i >= n_raw)
        def _():
            wo_copy(i).wait()
            for piece in pieces:
                precompute(i - n_rb, *piece)

        return carry

    lax.fori_loop(0, n_chunk - n_rb, load_body, 0)

    def finish_loads():
        for i in range(n_chunk - n_rb, n_chunk):
            wo_copy(i).wait()
        wu_copy.start()
        wd_copy.start()

    def qkv(g, rows):
        h = lhs_a[pl.ds(R2 - rows, rows), :]
        return jnp.concatenate(
            [_dot(h, pltpu.bitcast(wqkv_v[m, g], BF16)).astype(BF16) for m in range(3)],
            axis=1)

    def padded(a):
        return jnp.concatenate([a, jnp.zeros((128 - a.shape[0], Dh), BF16)], axis=0)

    def scores(p):
        return [lax.dot_general(p[:, i * Dh:(i + 1) * Dh],
                                padded(p[:, GW + i * Dh:GW + (i + 1) * Dh]),
                                (((1,), (1,)), ((), ())), preferred_element_type=F32)
                for i in range(HG)]

    def attend(p, ss, fill_ref):
        out = []
        for i in range(HG):
            fill = fill_ref[...]
            s = jnp.where(fill == 0.0, ss[i], fill)
            e = jnp.exp2((s - jnp.max(s, axis=-1, keepdims=True)) * exp_c)
            inv = 1.0 / jnp.sum(e, axis=-1, keepdims=True)
            v = padded(p[:, 2 * GW + i * Dh:2 * GW + (i + 1) * Dh])
            out.append((_dot(e.astype(BF16), v) * inv).astype(BF16))
        return jnp.concatenate(out, axis=1)

    def project(g, o, segs):
        rows = o.shape[0]
        y = _dot(o, wo_v[pl.ds(g * GW, GW), :])
        blocks = (0, SEG + MM) if len(segs) == 2 else (MM,)
        mem_lo = rows - R1
        if g == 0:
            acc_o[pl.ds(mem_lo, MM), :] = y[mem_lo:mem_lo + MM]
            for lo, s in zip(blocks, segs):
                acc_o[pl.ds(lo, SEG), :] = res_v[slot(s)] + y[lo:lo + SEG]
        elif g < n_grp - 1:
            acc_o[pl.ds(0, rows), :] += y
        else:
            y = acc_o[pl.ds(0, rows), :] + y
            for lo, s in zip(blocks, segs):
                res_v[slot(s)] = y[lo:lo + SEG]
            return y[mem_lo:mem_lo + MM]

    def ffn_input(segs):
        for n, s in enumerate(segs):
            x = res_v[slot(s)]
            acc_f[pl.ds(n * SEG, SEG), :] = x
            lhs_f[pl.ds(n * SEG, SEG), :] = _layernorm(x).astype(BF16)

    def ffn_up(c):
        return ffn_piece("u", 0, (DF, c * FC, FC), None)

    def ffn_down(c, a, segs):
        y = _dot(a, wd_v[pl.ds(c * FC, FC), :])
        if c < n_fc - 1:
            acc_f[...] += y
        else:
            y = acc_f[...] + y
            for n, s in enumerate(segs):
                r = y[n * SEG:(n + 1) * SEG]
                res_v[slot(s)] = r
                o_v[seg_rows(s), :] = r.astype(BF16)

    def out_copy(s):
        return pltpu.make_async_copy(o_v.at[seg_rows(s)], out_hbm.at[seg_rows(s)], out_sem)

    def ffn_cuts(parts):
        width = DF // parts
        cuts = list(range(0, width, FC)) + [width]
        return [(width, lo, hi - lo) for lo, hi in zip(cuts, cuts[1:])]

    def ffn_piece(op, k, cut, act):
        width, lo, n = cut
        cols = pl.ds(pl.multiple_of(k * width + lo, 128), n)
        if op == "u":
            h = lhs_f[...]
            return (_gelu(_dot(h, wg_v[:, cols])) * _dot(h, wu_v[:, cols])).astype(BF16)
        acc_f[...] += _dot(act, wd_v[cols, :])

    def project_piece(g, o):
        acc_o[pl.ds(0, o.shape[0]), :] += _dot(
            o, wo_v[pl.ds(pl.multiple_of(g * GW, GW), GW), :])

    def ffn_output(segs):
        for n, s in enumerate(segs):
            r = acc_f[pl.ds(n * SEG, SEG), :]
            res_v[slot(s)] = r
            o_v[seg_rows(s), :] = r.astype(BF16)

    def single_attention(layer, s):
        acc_o[pl.ds(0, MM), :] = jnp.zeros((MM, D), F32)
        acc_o[pl.ds(MM, SEG), :] = res_v[slot(s)]
        gs = n_grp // ATT_PARTS

        def part(k, c):
            pl.when(jnp.logical_and(jnp.logical_and(layer == 0, s == 0), k == ATT_PARTS // 2))(
                finish_loads)
            p, ss, o = {}, {}, {}
            for op, n in _step_order(gs, 1):
                g = k * gs + n
                if op == "q":
                    p[n] = qkv(g, R1)
                elif op == "i":
                    lhs_next[pl.ds(0, SEG), :] = _layernorm(res_v[slot(s + 1)]).astype(BF16)
                elif op == "s":
                    ss[n] = scores(p[n])
                elif op == "a":
                    o[n] = attend(p[n], ss[n], fill_s.at[layer])
                elif op == "o":
                    project_piece(g, o[n])
            return c

        lax.fori_loop(0, ATT_PARTS, part, 0)
        lhs_a[pl.ds(SEG + MM, SEG), :] = lhs_next[pl.ds(0, SEG), :]
        res_v[slot(s)] = acc_o[pl.ds(MM, SEG), :]
        own = jnp.where(lax.broadcasted_iota(jnp.int32, (MM, D), 0) < M, 0, 1) == layer
        lhs_a[pl.ds(SEG, MM), :] = jnp.where(
            own, acc_o[pl.ds(0, MM), :], lhs_a[pl.ds(SEG, MM), :].astype(F32)).astype(BF16)

    def single_ffn(segs):
        ffn_input(segs)
        cuts = ffn_cuts(FFN_PARTS)

        def part(k, c):
            a = {0: ffn_piece("u", k, cuts[0], None)}
            for n, cut in enumerate(cuts):
                if n + 1 < len(cuts):
                    a[n + 1] = ffn_piece("u", k, cuts[n + 1], None)
                ffn_piece("d", k, cut, a[n])
            return c

        lax.fori_loop(0, FFN_PARTS, part, 0)
        ffn_output(segs)

    def step_segments(t):
        return (t, t - LAG), (t - 1, jnp.where(t == LAG, t - 2, t - LAG - 1))

    def next_attention_input(t):
        attention_input(0, load_segment(jnp.minimum(t + 1, n_seg - 1)))
        attention_input(1, res_v[slot(t + 1 - LAG)])

    def paired_step(t, carry):
        att, ffn = step_segments(t)
        out_copy(t - LAG - 2).start()
        p, ss, o, a = {}, {}, {}, {}
        for op, n in _step_order(n_grp, n_fc):
            if op == "q":
                p[n] = qkv(n, R2)
            elif op == "s":
                ss[n] = scores(p[n])
            elif op == "a":
                o[n] = attend(p[n], ss[n], fill_v)
            elif op == "o":
                mem = project(n, o[n], att)
                if n == n_grp - 1:
                    lhs_a[pl.ds(SEG, MM), :] = mem.astype(BF16)
            elif op == "i":
                ffn_input(ffn)
            elif op == "u":
                a[n] = ffn_up(n)
            elif op == "d":
                ffn_down(n, a[n], ffn)
            else:
                next_attention_input(t)
        return carry

    def precomputed_step(t, carry):
        att, ffn = step_segments(t)
        pre_rows = pl.ds(pl.multiple_of((t - LAG) * SEG, SEG), SEG)
        gs, cuts = n_grp // PRE_PARTS, ffn_cuts(PRE_PARTS)
        acc_o[pl.ds(0, SEG), :] = res_v[slot(att[0])]
        acc_o[pl.ds(SEG, MM), :] = jnp.zeros((MM, D), F32)
        acc_o[pl.ds(SEG + MM, SEG), :] = res_v[slot(att[1])]
        for n, s in enumerate(ffn):
            acc_f[pl.ds(n * SEG, SEG), :] = res_v[slot(s)]

        def part(k, c):
            p, ss, o, a = {}, {}, {}, {}
            for op, n in _step_order(gs, len(cuts)):
                g = k * gs + n
                if op == "q":
                    p[n] = jnp.concatenate(
                        [jnp.concatenate([pre_v[m, g, pre_rows, :] for m in range(3)], axis=1),
                         qkv(g, R1)], axis=0)
                elif op == "s":
                    ss[n] = scores(p[n])
                elif op == "a":
                    o[n] = attend(p[n], ss[n], fill_v)
                elif op == "o":
                    project_piece(g, o[n])
                elif op == "i":
                    for j, s in enumerate(ffn):
                        lhs_f[pl.ds(j * SEG, SEG), :] = _layernorm(res_v[slot(s)]).astype(BF16)
                elif op == "n":
                    lhs_next[pl.ds(0, SEG), :] = _layernorm(load_segment(t + 1)).astype(BF16)
                    lhs_next[pl.ds(SEG, SEG), :] = _layernorm(
                        res_v[slot(t + 1 - LAG)]).astype(BF16)
                else:
                    a[n] = ffn_piece(op, k, cuts[n], a.get(n))
            return c

        lax.fori_loop(0, PRE_PARTS, part, 0)
        lhs_a[pl.ds(0, SEG), :] = lhs_next[pl.ds(0, SEG), :]
        lhs_a[pl.ds(SEG, MM), :] = acc_o[pl.ds(SEG, MM), :].astype(BF16)
        lhs_a[pl.ds(SEG + MM, SEG), :] = lhs_next[pl.ds(SEG, SEG), :]
        res_v[slot(att[0])] = acc_o[pl.ds(0, SEG), :]
        res_v[slot(att[1])] = acc_o[pl.ds(SEG + MM, SEG), :]
        ffn_output(ffn)

        @pl.when(t > LAG + 1)
        def _():
            out_copy(t - LAG - 2).start()

        return carry

    def single_op(phase, i):
        is_head = phase == 0
        j = i - 1
        tail_ffn = lax.rem(i, 3) == 0
        is_ffn = jnp.where(is_head, i == LAG, tail_ffn)
        first = n_seg - LAG + 2 * lax.div(jnp.maximum(j, 0), 3)

        @pl.when(jnp.logical_not(is_ffn))
        def _():
            single_attention(phase, jnp.where(is_head, i, first + lax.rem(j, 3)))

        @pl.when(is_ffn)
        def _():
            @pl.when(is_head)
            def _():
                for c in (wg_copy, wu_copy, wd_copy):
                    c.wait()
                x_rest.start()

            s0 = jnp.where(is_head, 0, jnp.where(i == 0, n_seg - 1, first))
            s1 = jnp.where(is_head, 1, jnp.where(i == 0, n_seg - LAG - 1, first + 1))
            single_ffn((s0, s1))

            @pl.when(jnp.logical_not(is_head))
            def _():
                out_copy(s1).start()

                @pl.when(i > 0)
                def _():
                    out_copy(s0).start()

    def phase_body(phase, carry):
        n_ops = jnp.where(phase == 0, LAG + 1, 1 + 3 * (LAG // 2))
        lax.fori_loop(0, n_ops, lambda i, c: (single_op(phase, i), c)[1], 0)

        @pl.when(phase == 0)
        def _():
            x_rest.wait()
            attention_input(1, res_v[slot(0)])
            lax.fori_loop(LAG, LAG + PRE, precomputed_step, 0)
            lax.fori_loop(LAG + PRE, n_seg, paired_step, 0)
            out_copy(n_seg - LAG - 2).start()

        return carry

    lax.fori_loop(0, 2, phase_body, 0)
    pltpu.make_async_copy(o_v, out_hbm, out_sem).wait()


@functools.partial(jax.jit, static_argnames=("A_seg_len",))
def pallas_interleave_layers__memory_aug_recurrent_mem_tr__glu_gated_geglu__prompt_kernel(
    A_x, A_mem0, A_Wq, A_Wk, A_Wv, A_Wo, A_seg_len, B_x, B_w_gate, B_w_up, B_w_down,
):
    del B_x
    B, S, D = A_x.shape
    _, H, Dh = A_Wq.shape
    M = A_mem0.shape[1]
    SEG = int(A_seg_len)
    DF = B_w_gate.shape[1]
    assert B == 1 and Dh == 128 and (M, SEG, H) == (8, 32, 32) and S // SEG >= LAG + PRE + 1
    R = 2 * (M + SEG)
    hbm = pl.BlockSpec(memory_space=pl.ANY)
    out = pl.pallas_call(
        functools.partial(_kernel, S=S, D=D, H=H, Dh=Dh, M=M, SEG=SEG, DF=DF),
        out_shape=jax.ShapeDtypeStruct((S, D), A_x.dtype),
        in_specs=[hbm, pl.BlockSpec(memory_space=pltpu.VMEM)] + [hbm] * 7,
        out_specs=hbm,
        scratch_shapes=[
            pltpu.VMEM((S, D), BF16),
            pltpu.VMEM((S, D), BF16),
            pltpu.VMEM((6 * D, H // 2, Dh), BF16),
            pltpu.VMEM((3, H // HG, D // 2, HG * Dh), jnp.int32),
            pltpu.VMEM((H * Dh, D), BF16),
            pltpu.VMEM((D, DF), BF16),
            pltpu.VMEM((D, DF), BF16),
            pltpu.VMEM((DF, D), BF16),
            pltpu.VMEM((RING, SEG, D), F32),
            pltpu.VMEM((R, D), BF16),
            pltpu.VMEM((2 * SEG, D), BF16),
            pltpu.VMEM((R, D), F32),
            pltpu.VMEM((2 * SEG, D), BF16),
            pltpu.VMEM((2 * SEG, D), F32),
            pltpu.VMEM((R, 128), F32),
            pltpu.VMEM((2, R - SEG, 128), F32),
            pltpu.VMEM((PRE * SEG, D), BF16),
            pltpu.VMEM((3, H // HG, PRE * SEG, HG * Dh), BF16),
            pltpu.SemaphoreType.DMA((8 * (D // RB),)),
            pltpu.SemaphoreType.DMA((5,)),
            pltpu.SemaphoreType.DMA(()),
        ],
        compiler_params=pltpu.CompilerParams(vmem_limit_bytes=120 * 2**20),
    )(A_x.reshape(S, D), A_mem0.reshape(M, D),
      A_Wq, A_Wk, A_Wv,
      A_Wo.reshape(H * Dh, D), B_w_gate, B_w_up, B_w_down)
    return out.reshape(B, S, D)
```
